```python
import jax
import jax.numpy as jnp

def _softmax(x, axis=-1):
    return jax.nn.softmax(x, axis=axis)
def _gelu(x):
    return jax.nn.gelu(x, approximate=True)
def _silu(x):
    return jax.nn.silu(x)
def _sigmoid(x):
    return jax.nn.sigmoid(x)
def _layernorm(x, axis=-1, eps=1e-5):
    m = jnp.mean(x, axis=axis, keepdims=True)
    v = jnp.var(x, axis=axis, keepdims=True)
    return (x - m) / jnp.sqrt(v + eps)
def _scatter_add(tgt, idx, src, axis=0):
    return tgt.at[idx].add(src)
def _segment_sum(src, seg, n):
    return jax.ops.segment_sum(src, seg, n)
class _Rng:
    def __init__(self, key):
        self._k = key
    def _next(self):
        self._k, sub = jax.random.split(self._k)
        return sub
    def normal(self, shape):
        return jax.random.normal(self._next(), shape, dtype=jnp.bfloat16)
    def randint(self, lo, hi, shape):
        return jax.random.randint(self._next(), shape, lo, hi, dtype=jnp.int32)
    def uniform(self, shape, lo=0.0, hi=1.0):
        return jax.random.uniform(self._next(), shape, jnp.bfloat16, lo, hi)
    def permutation(self, n):
        return jax.random.permutation(self._next(), n)


kernel_name = 'concat_heads__sliding_block_cached__compressed_kv_cla__decode'

def setup_inputs():
    _rng = _Rng(jax.random.key(int.from_bytes(__import__("os").urandom(4), "little")))
    _w = (lambda a: (lambda t: t.astype(jnp.bfloat16) if jnp.issubdtype(t.dtype, jnp.floating) else t)(jnp.asarray(a)))
    def _A_setup():
        B, Sq, D = 4, 1, 512
        Hq, Hkv, Sk, Dh = 32, 32, 4096, 128
        assert Hq % Hkv == 0, (Hq, Hkv)
        return {
            "x": _w((lambda *s: _rng.normal(s) * 0.05)(B, Sq, D)),
            "k_cache": _w((lambda *s: _rng.normal(s) * 0.05)(B, Hkv, Sk, Dh)),
            "v_cache": _w((lambda *s: _rng.normal(s) * 0.05)(B, Hkv, Sk, Dh)),
            "wq": _w((lambda *s: _rng.normal(s) * 0.05)(D, Hq * Dh) * (D ** -0.5)),
            "wo": _w((lambda *s: _rng.normal(s) * 0.05)(Hq * Dh, D) * ((Hq * Dh) ** -0.5)),
        }
    _A_in = _A_setup()

    def _B_setup():
        B, H, Sq, Sk, D, M = 4, 32, 1, 4096, 128, 512
        Dc = 4 * D
        return {
            "x": _w((lambda *s: _rng.normal(s) * 0.05)(B, Sq, M)),
            "c_kv": _w((lambda *s: _rng.normal(s) * 0.05)(B, Sk, Dc)),
            "w_q": _w((lambda *s: _rng.normal(s) * 0.05)(M, H, D) * (M ** -0.5)),
            "w_uk": _w((lambda *s: _rng.normal(s) * 0.05)(Dc, H, D) * (Dc ** -0.5)),
            "w_uv": _w((lambda *s: _rng.normal(s) * 0.05)(Dc, H, D) * (Dc ** -0.5)),
            "w_o": _w((lambda *s: _rng.normal(s) * 0.05)(H, D, M) * ((H * D) ** -0.5)),
        }
    _B_in = _B_setup()

    return {
        "A_x": _A_in["x"],
        "A_k_cache": _A_in["k_cache"],
        "A_v_cache": _A_in["v_cache"],
        "A_wq": _A_in["wq"],
        "A_wo": _A_in["wo"],
        "B_x": _B_in["x"],
        "B_c_kv": _B_in["c_kv"],
        "B_w_q": _B_in["w_q"],
        "B_w_uk": _B_in["w_uk"],
        "B_w_uv": _B_in["w_uv"],
        "B_w_o": _B_in["w_o"],
    }

def reference(A_x, A_k_cache, A_v_cache, A_wq, A_wo, B_x, B_c_kv, B_w_q, B_w_uk, B_w_uv, B_w_o):
    def _A_ref(x, k_cache, v_cache, wq, wo):
        B, Sq, D = x.shape
        Hq, Dh = 32, 128
        Hkv, Sk = k_cache.shape[1], k_cache.shape[2]
        W = min(4096, max(256, Sk // 4))
        rep = Hq // Hkv
        q = (lambda x, *d: x.transpose(*d))((x @ wq).reshape(B, Sq, Hq, Dh), 0, 2, 1, 3)
        k = jnp.repeat(k_cache[:, :, Sk - W:, :], rep, axis=1)
        v = jnp.repeat(v_cache[:, :, Sk - W:, :], rep, axis=1)
        scores = jnp.einsum("bhqd,bhkd->bhqk", q, k) * (Dh ** -0.5)
        p = _softmax(scores, axis=-1)
        o = jnp.einsum("bhqk,bhkd->bhqd", p, v)
        return (lambda x, *d: x.transpose(*d))(o, 0, 2, 1, 3).reshape(B, Sq, Hq * Dh) @ wo

    def _B_ref(x, c_kv, w_q, w_uk, w_uv, w_o):
        B, Sq, M = x.shape[0], x.shape[1], x.shape[2]
        Sk = c_kv.shape[1]
        H, D = w_q.shape[1], w_q.shape[2]
        q = jnp.einsum("bqm,mhd->bhqd", x, w_q)
        k = jnp.einsum("bkc,chd->bhkd", c_kv, w_uk)
        v = jnp.einsum("bkc,chd->bhkd", c_kv, w_uv)
        scores = jnp.einsum("bhqd,bhkd->bhqk", q, k) * (D ** -0.5)
        off = Sk - Sq
        qi = jnp.arange(Sq)[:, None]
        kj = jnp.arange(Sk)[None, :]
        cmask = kj <= (qi + off)
        scores = jnp.where(cmask[None, None], scores, -1e9)
        p = _softmax(scores, axis=-1)
        ctx = jnp.einsum("bhqk,bhkd->bhqd", p, v)
        return jnp.einsum("bhqd,hdm->bqm", ctx, w_o)

    a = _A_ref(A_x, A_k_cache, A_v_cache, A_wq, A_wo)
    b = _B_ref(B_x, B_c_kv, B_w_q, B_w_uk, B_w_uv, B_w_o)
    return jnp.concatenate([a, b], axis=-1)
```

```python
import jax
import jax.numpy as jnp
from jax import lax
import jax.experimental.pallas as pl
import jax.experimental.pallas.tpu as pltpu

F32 = jnp.float32
BF16 = jnp.bfloat16

NB = 4
NH = 32
DH = 128
DM = 512
SK = 4096
WIN = 1024
CK = 256
NU = 32
NT = ((1,), (1,)), ((), ())

CFG = dict(compute=True, pre0=5, bwait=6)


def _mult(x, m):
    return x if isinstance(x, int) else pl.multiple_of(x, m)


def _kernel(xa_hbm, xb_hbm, k_hbm, v_hbm, wqa_hbm, woa_hbm, c_hbm, wqb_hbm, wuk_hbm,
            wuv_hbm, wob_hbm, o_ref,
            xa_buf, xb_buf, kbuf, vbuf, wqa_buf, woa_buf, cbuf, wqb_buf, wuk_buf,
            wuv_buf, wob_buf,
            xb_s, qa_t, oa_t, pa_s, la_s, qb_s, qabs_t, qabs_s, sb_s, pb_s, al_s,
            m_s, l_s, acc_s, cc_s, ctx_s, out_s,
            sem1, sem0, semx, semt):
    do_compute = CFG["compute"]
    scale = DH ** -0.5
    row4 = lax.broadcasted_iota(jnp.int32, (NB, DH), 0)

    def copy(piece, sem):
        return pltpu.make_async_copy(piece[0], piece[1], sem)

    def ticks(waits, starts1, starts0, comp):
        for t, (piece, sem) in enumerate(waits):
            copy(piece, sem).wait()
            for p, s in starts0.get(t, ()):
                copy(p, s).start(priority=0)
            for p, s in starts1.get(t, ()):
                copy(p, s).start(priority=1)
            for f in comp.get(t, ()):
                f()

    def unit_bh(u):
        return u & 3, (u >> 2) * 4

    def kv_pieces(hbm, buf, u):
        b, h0 = unit_bh(u)
        return [(hbm.at[b, pl.ds(h0, 4), pl.ds(SK - WIN + 64 * s, 64)],
                 buf.at[u & 1, :, pl.ds(64 * s, 64)]) for s in range(16)]

    def b_chunk(stage, i):
        if stage == "c":
            pcs = []
            for s in range(CK // 16):
                for b0 in (0, 2):
                    pcs.append((c_hbm.at[pl.ds(b0, 2), pl.ds(_mult(i * CK + 16 * s, 16), 16)],
                                cbuf.at[i & 1, pl.ds(b0, 2), pl.ds(16 * s, 16)]))
            return pcs, cbuf.at[i & 1]
        hbm, buf, rows = {"wq": (wqb_hbm, wqb_buf, 2), "wuk": (wuk_hbm, wuk_buf, 2),
                          "wuv": (wuv_hbm, wuv_buf, 2), "wo": (wob_hbm, wob_buf, 16)}[stage]
        pcs = []
        for s in range(32):
            idx = (pl.ds(2 * i, 2), pl.ds(rows * s, rows))
            pcs.append((hbm.at[idx], buf.at[idx]))
        return pcs, buf.at[pl.ds(2 * i, 2)]

    def wqa_piece(r0, nr, s):
        idx = (pl.ds(r0, nr), pl.ds(8 * (s // 4), 8), pl.ds(1024 * (s % 4), 1024))
        return wqa_hbm.at[idx], wqa_buf.at[idx]

    def woa_piece(r0, nr, s):
        idx = (pl.ds(r0, nr), pl.ds(16 * s, 16))
        return woa_hbm.at[idx], woa_buf.at[idx]

    def split_w(mk):
        p1 = [mk(0, 4, s) for s in range(32)] + [mk(4, 4, s) for s in range(16)]
        p0 = [mk(r, 2, s) for s0 in (16, 24) for r in (4, 6) for s in range(s0, s0 + 8)]
        return p1, p0

    def w3_block(buf, cb, hb):
        w = buf[pl.ds(2 * cb, 2), :, 8 * hb:8 * hb + 8, :]
        return w.reshape(128, 8, DH).reshape(128, 8 * DH)

    def wqb_comp(cb):
        def piece(hb):
            def f():
                r = jnp.dot(xb_s[cb].astype(BF16), w3_block(wqb_buf, cb, hb),
                            preferred_element_type=F32)
                qb_s[:, 1024 * hb:1024 * hb + 1024] += r
            return f
        return [piece(hb) for hb in range(4)]

    def wuk_comp(cb):
        def piece(hb):
            def f():
                w = w3_block(wuk_buf, cb, hb)
                for j in range(8):
                    h = 8 * hb + j
                    q = (qb_s[:, DH * h:DH * h + DH] * scale).astype(BF16)
                    r = lax.dot_general(q, w[:, DH * j:DH * j + DH], NT,
                                        preferred_element_type=F32)
                    qabs_t[cb, 8 * h:8 * h + NB, :] = r
            return f
        return [piece(hb) for hb in range(4)]

    def qabs_finish():
        for b in range(NB):
            for cb in range(4):
                qabs_s[b, :, 128 * cb:128 * cb + 128] = (
                    qabs_t[cb, pl.ds(b, NH, stride=8), :].astype(BF16))

    def c_comp(i):
        sl = i & 1

        def qk(bs):
            def f():
                for b in bs:
                    sb_s[b] = lax.dot_general(qabs_s[b], cbuf[sl, b], NT,
                                              preferred_element_type=F32)
            return f

        def sm():
            s = sb_s[...]
            m_old = m_s[...]
            m_new = jnp.maximum(m_old, jnp.max(s, axis=-1, keepdims=True))
            alpha = jnp.exp(m_old - m_new)
            p = jnp.exp(s - m_new)
            l_s[...] = alpha * l_s[...] + jnp.sum(p, axis=-1, keepdims=True)
            m_s[...] = m_new
            al_s[...] = alpha
            pb_s[...] = p.astype(BF16)

        def pv(bs):
            def f():
                for b in bs:
                    r = jnp.dot(pb_s[b], cbuf[sl, b], preferred_element_type=F32)
                    acc_s[b] = al_s[b] * acc_s[b] + r
            return f

        return [qk((0, 1)), qk((2, 3)), sm, pv((0, 1)), pv((2, 3))]

    def c_finish():
        for b in range(NB):
            cc = acc_s[b] / l_s[b]
            for cb in range(4):
                cc_s[cb, NH * b:NH * b + NH, :] = cc[:, 128 * cb:128 * cb + 128]

    def wuv_comp(cb):
        def piece(hb):
            def f():
                w = w3_block(wuv_buf, cb, hb)
                for j in range(8):
                    cc = cc_s[cb, pl.ds(8 * hb + j, NB, stride=NH), :].astype(BF16)
                    r = jnp.dot(cc, w[:, DH * j:DH * j + DH], preferred_element_type=F32)
                    ctx_s[hb, :, DH * j:DH * j + DH] += r
            return f
        return [piece(hb) for hb in range(4)]

    def wob_comp(g):
        def piece(half):
            def f():
                x = ctx_s[g, :, 512 * half:512 * half + 512].astype(BF16)
                out_s[1] += jnp.dot(x, wob_buf[2 * g + half], preferred_element_type=F32)
            return f
        return [piece(0), piece(1)]

    b_comp = {"wq": wqb_comp, "wuk": wuk_comp, "c": c_comp, "wuv": wuv_comp, "wo": wob_comp}
    b_finish = {"wuk": qabs_finish, "c": c_finish}

    def init():
        for cp in x_copies:
            cp.wait()
        if not do_compute:
            return
        xb = xb_buf[...].astype(F32)
        for cb in range(4):
            xb_s[cb] = xb[:, 128 * cb:128 * cb + 128]
        qb_s[...] = jnp.zeros(qb_s.shape, F32)
        ctx_s[...] = jnp.zeros(ctx_s.shape, F32)
        out_s[...] = jnp.zeros(out_s.shape, F32)
        m_s[...] = jnp.full(m_s.shape, -jnp.inf, F32)
        l_s[...] = jnp.zeros(l_s.shape, F32)
        acc_s[...] = jnp.zeros(acc_s.shape, F32)

    def wqa_comp(j):
        def f():
            w = wqa_buf[:, :, 1024 * j:1024 * j + 1024].reshape(DM, 1024)
            r = jnp.dot(xa_buf[...], w, preferred_element_type=F32) * scale
            for i in range(8):
                h = 8 * j + i
                qa_t[8 * h:8 * h + NB, :] = r[:, DH * i:DH * i + DH]
        return f

    def a_qk(u):
        b, h0 = unit_bh(u)
        st = {}

        def qk(js):
            def f():
                q4 = qa_t[pl.ds(8 * h0 + b, 4, stride=8), :]
                s = st.get("s")
                for j in js:
                    qm = jnp.where(row4 == j, q4, 0.0).astype(BF16)
                    sj = lax.dot_general(qm, kbuf[u & 1, j], NT, preferred_element_type=F32)
                    s = sj if s is None else s + sj
                st["s"] = s
            return f

        def sm():
            s = st["s"]
            p = jnp.exp(s - jnp.max(s, axis=-1, keepdims=True))
            la_s[...] = jnp.sum(p, axis=-1, keepdims=True)
            pa_s[...] = p

        return [qk((0, 1)), qk((2, 3)), sm]

    def a_pv(u):
        b, h0 = unit_bh(u)

        def f():
            p = pa_s[...].astype(BF16)
            o = None
            for j in range(4):
                oj = jnp.dot(p, vbuf[u & 1, j], preferred_element_type=F32)
                o = oj if o is None else jnp.where(row4 == j, oj, o)
            oa_t[pl.ds(8 * h0 + b, 4, stride=8), :] = o / la_s[...]
        return f

    def woa_comp(heads):
        def f():
            r = None
            for h in heads:
                o = oa_t[8 * h:8 * h + NB, :].astype(BF16)
                w = woa_buf[h // 4, 128 * (h % 4):128 * (h % 4) + 128, :]
                t = jnp.dot(o, w, preferred_element_type=F32)
                r = t if r is None else r + t
            out_s[0] += r
        return f

    def at(d, t, item):
        d.setdefault(t, []).append(item)

    def wait_all(pieces, sem):
        def f():
            for p in pieces:
                copy(p, sem).wait()
        return f

    D1 = 16
    pre0 = CFG["pre0"]
    bwait = CFG["bwait"]
    x_copies = [pltpu.make_async_copy(xa_hbm, xa_buf, semx.at[0]),
                pltpu.make_async_copy(xb_hbm, xb_buf, semx.at[1])]
    q1, q0 = split_w(wqa_piece)
    for j in range(D1):
        copy(q1[j], sem1.at[1]).start(priority=1)
        if j < pre0:
            copy(q0[j], sem0.at[1]).start(priority=0)
    for cp in x_copies:
        cp.start()
    s1, s0, cm = {}, {}, {}
    nxt = [(p, sem1.at[1]) for p in q1[D1:]] + [(p, sem1.at[0]) for p in kv_pieces(k_hbm, kbuf, 0)]
    for t, it in enumerate(nxt):
        at(s1, t, it)
    n0 = len(q0) - pre0
    for j in range(n0):
        at(s0, (j * len(q1)) // n0, (q0[pre0 + j], sem0.at[1]))
    at(cm, 4, init)
    ticks([(p, sem1.at[1]) for p in q1], s1, s0, cm)

    o1, o0 = split_w(woa_piece)
    o1_sem = [semt.at[j // 8] for j in range(len(o1))]

    def body(u, issue, comp, finish, first=False, last=False):
        kp = kv_pieces(k_hbm, kbuf, u)
        vp = kv_pieces(v_hbm, vbuf, u)
        waits = [(p, sem1.at[0]) for p in kp] + [(p, sem1.at[1]) for p in vp]
        s1, s0, cm = {}, {}, {}
        for t in range(16):
            at(s1, t, (vp[t], sem1.at[1]))
        if last:
            for t in range(16):
                at(s1, 16 + t, (o1[t], o1_sem[t]))
        else:
            kn = kv_pieces(k_hbm, kbuf, u + 1)
            for t in range(16):
                at(s1, 16 + t, (kn[t], sem1.at[0]))
        pcs, _ = b_chunk(*issue)
        for t in range(32):
            at(s0, t, (pcs[t], sem0.at[u & 1]))
        psem = sem0.at[(u + 1) & 1]
        if first:
            at(cm, bwait, wait_all(q0, psem))
            bc = [wqa_comp(j) for j in range(4)]
            btk = [bwait, bwait + 2, bwait + 5, bwait + 7]
        else:
            _, dst = b_chunk(*comp)
            at(cm, bwait, lambda: pltpu.make_async_copy(dst, dst, psem).wait())
            bc = b_comp[comp[0]](comp[1])
            if finish:
                bc = bc + [b_finish[comp[0]]]
            btk = [bwait, bwait + 3, bwait + 6, 25, 28, 30][:len(bc)]
        if do_compute:
            if not first:
                at(cm, 1, a_pv(u - 1))
            for t, f in zip(btk, bc):
                at(cm, t, f)
            for t, f in zip((16, 19, 22), a_qk(u)):
                at(cm, t, f)
        ticks(waits, s1, s0, cm)

    stages = [("wq", 4), ("wuk", 4), ("c", 16), ("wuv", 4), ("wo", 4)]
    u0 = 0
    prev = None
    for stage, n in stages:
        body(u0, (stage, 0), prev, prev is not None and prev[0] in b_finish, first=prev is None)
        hi = n - 1 if stage == "wo" else n

        def loop_body(i, carry, stage=stage, u0=u0):
            body(u0 + i, (stage, i), (stage, i - 1), False)
            return carry

        lax.fori_loop(1, hi, loop_body, 0)
        prev = (stage, n - 1)
        u0 += n
    body(NU - 1, ("wo", 3), ("wo", 2), False, last=True)

    s1, s0, cm = {}, {}, {}
    for t in range(len(o1) - D1):
        at(s1, t, (o1[D1 + t], o1_sem[D1 + t]))
    last0 = len(o1) - 8
    for j in range(len(o0)):
        at(s0, (j * last0) // len(o0), (o0[j], sem0.at[0]))
    _, dst = b_chunk("wo", 3)
    at(cm, bwait, lambda: pltpu.make_async_copy(dst, dst, sem0.at[1]).wait())
    at(cm, len(o1) - 3, wait_all(o0, sem0.at[0]))
    if do_compute:
        at(cm, 1, a_pv(NU - 1))
        for t, f in zip((bwait, bwait + 3), wob_comp(3)):
            at(cm, t, f)
        for g in range(6):
            r0, j = (0, g) if g < 4 else (4, g - 4)
            at(cm, max(8 * g + 7, 12 + g), woa_comp([4 * (r0 + r) + j for r in range(4)]))
        cm[len(o1) - 3].append(woa_comp([4 * r + j for r in range(4, 8) for j in (2, 3)]))
    ticks([(p, s) for p, s in zip(o1, o1_sem)], s1, s0, cm)
    if do_compute:
        o_ref[:, 0:DM] = out_s[0].astype(o_ref.dtype)
        o_ref[:, DM:2 * DM] = out_s[1].astype(o_ref.dtype)
    else:
        o_ref[...] = jnp.zeros(o_ref.shape, o_ref.dtype)


@jax.jit
def pallas_concat_heads__sliding_block_cached__compressed_kv_cla__decode_kernel(
    A_x: jax.Array,
    A_k_cache: jax.Array,
    A_v_cache: jax.Array,
    A_wq: jax.Array,
    A_wo: jax.Array,
    B_x: jax.Array,
    B_c_kv: jax.Array,
    B_w_q: jax.Array,
    B_w_uk: jax.Array,
    B_w_uv: jax.Array,
    B_w_o: jax.Array,
):
    assert A_x.shape == (NB, 1, DM) and B_x.shape == (NB, 1, DM)
    assert A_k_cache.shape == (NB, NH, SK, DH) and B_c_kv.shape == (NB, SK, DM)
    w3 = (8, 64, NH, DH)
    w2 = (8, 512, DM)
    wq = (8, 64, NH * DH)
    vm = pltpu.VMEM
    out = pl.pallas_call(
        _kernel,
        out_shape=jax.ShapeDtypeStruct((NB, 2 * DM), A_x.dtype),
        in_specs=[pl.BlockSpec(memory_space=pl.ANY)] * 11,
        out_specs=pl.BlockSpec(memory_space=pltpu.VMEM),
        scratch_shapes=[
            vm((NB, DM), BF16), vm((NB, DM), BF16),
            vm((2, 4, WIN, DH), BF16), vm((2, 4, WIN, DH), BF16),
            vm(wq, BF16), vm(w2, BF16),
            vm((2, NB, CK, DM), BF16),
            vm(w3, BF16), vm(w3, BF16), vm(w3, BF16), vm(w2, BF16),
            vm((4, NB, 128), F32),
            vm((NH * 8, DH), F32),
            vm((NH * 8, DH), F32),
            vm((4, WIN), F32),
            vm((4, 1), F32),
            vm((NB, NH * DH), F32),
            vm((4, NH * 8, 128), F32),
            vm((NB, NH, DM), BF16),
            vm((NB, NH, CK), F32),
            vm((NB, NH, CK), BF16),
            vm((NB, NH, 1), F32),
            vm((NB, NH, 1), F32), vm((NB, NH, 1), F32),
            vm((NB, NH, DM), F32),
            vm((4, NB * NH, 128), F32),
            vm((4, NB, 8 * DH), F32),
            vm((2, NB, DM), F32),
            pltpu.SemaphoreType.DMA((2,)), pltpu.SemaphoreType.DMA((2,)),
            pltpu.SemaphoreType.DMA((2,)), pltpu.SemaphoreType.DMA((6,)),
        ],
        compiler_params=pltpu.CompilerParams(
            vmem_limit_bytes=64 * 1024 * 1024,
            disable_bounds_checks=True,
            disable_semaphore_checks=True,
        ),
        name="concat_heads_decode",
    )(
        A_x.reshape(NB, DM), B_x.reshape(NB, DM), A_k_cache, A_v_cache,
        A_wq.reshape(wq), A_wo.reshape(w2), B_c_kv,
        B_w_q.reshape(w3), B_w_uk.reshape(w3), B_w_uv.reshape(w3), B_w_o.reshape(w2),
    )
    return out.reshape(NB, 1, 2 * DM)
```

```python
import jax
import jax.numpy as jnp
from jax import lax
import jax.experimental.pallas as pl
import jax.experimental.pallas.tpu as pltpu

F32 = jnp.float32
BF16 = jnp.bfloat16

NB = 4
NH = 32
DH = 128
DM = 512
SK = 4096
WIN = 1024
CK = 256
NU = 32
NT = ((1,), (1,)), ((), ())

CFG = dict(compute=True, pre0=5, bwait=6, adv=0, fine=True, w3sep=1)


def _mult(x, m):
    return x if isinstance(x, int) else pl.multiple_of(x, m)


def _kernel(xa_hbm, xb_hbm, k_hbm, v_hbm, wqa_hbm, woa_hbm, c_hbm, wqb_hbm, wuk_hbm,
            wuv_hbm, wob_hbm, o_ref,
            xa_buf, xb_buf, kbuf, vbuf, wqa_buf, woa_buf, cbuf, wqb_buf, wuk_buf,
            wuv_buf, wob_buf,
            xb_s, qa_t, oa_t, pa_s, la_s, qb_s, qabs_t, qabs_s, sb_s, pb_s, al_s,
            m_s, l_s, acc_s, cc_s, ctx_s, out_s, w2a_s, w2b_s,
            sem1, sem0, semx, semt):
    do_compute = CFG["compute"]
    w2_s = (w2a_s, w2b_s)
    scale = DH ** -0.5
    row4 = lax.broadcasted_iota(jnp.int32, (NB, DH), 0)

    def copy(piece, sem):
        return pltpu.make_async_copy(piece[0], piece[1], sem)

    def ticks(waits, starts1, starts0, comp):
        adv = CFG["adv"]
        if adv and do_compute:
            starts0 = {t: list(v) for t, v in starts0.items()}
            for t in sorted(comp):
                if any(getattr(f, "burst", True) for f in comp[t]):
                    for d in range(1, adv + 1):
                        if t + d in starts0:
                            starts0.setdefault(t, []).extend(starts0.pop(t + d))
        for t, (piece, sem) in enumerate(waits):
            copy(piece, sem).wait()
            for p, s in starts0.get(t, ()):
                copy(p, s).start(priority=0)
            for p, s in starts1.get(t, ()):
                copy(p, s).start(priority=1)
            for f in comp.get(t, ()):
                f()

    def unit_bh(u):
        return u & 3, (u >> 2) * 4

    def kv_pieces(hbm, buf, u):
        b, h0 = unit_bh(u)
        return [(hbm.at[b, pl.ds(h0, 4), pl.ds(SK - WIN + 64 * s, 64)],
                 buf.at[u & 1, :, pl.ds(64 * s, 64)]) for s in range(16)]

    def b_chunk(stage, i):
        if stage == "c":
            pcs = []
            for s in range(CK // 16):
                for b0 in (0, 2):
                    pcs.append((c_hbm.at[pl.ds(b0, 2), pl.ds(_mult(i * CK + 16 * s, 16), 16)],
                                cbuf.at[i & 1, pl.ds(b0, 2), pl.ds(16 * s, 16)]))
            return pcs, cbuf.at[i & 1]
        hbm, buf, rows = {"wq": (wqb_hbm, wqb_buf, 2), "wuk": (wuk_hbm, wuk_buf, 2),
                          "wuv": (wuv_hbm, wuv_buf, 2), "wo": (wob_hbm, wob_buf, 16)}[stage]
        pcs = []
        for s in range(32):
            idx = (pl.ds(2 * i, 2), pl.ds(rows * s, rows))
            pcs.append((hbm.at[idx], buf.at[idx]))
        return pcs, buf.at[pl.ds(2 * i, 2)]

    def wqa_piece(r0, nr, s):
        idx = (pl.ds(r0, nr), pl.ds(8 * (s // 4), 8), pl.ds(1024 * (s % 4), 1024))
        return wqa_hbm.at[idx], wqa_buf.at[idx]

    def woa_piece(r0, nr, s):
        idx = (pl.ds(r0, nr), pl.ds(16 * s, 16))
        return woa_hbm.at[idx], woa_buf.at[idx]

    def split_w(mk):
        p1 = [mk(0, 4, s) for s in range(32)] + [mk(4, 4, s) for s in range(16)]
        p0 = [mk(r, 2, s) for s0 in (16, 24) for r in (4, 6) for s in range(s0, s0 + 8)]
        return p1, p0

    def w3_block(buf, cb, hb):
        w = buf[pl.ds(2 * cb, 2), :, 8 * hb:8 * hb + 8, :]
        return w.reshape(128, 8, DH).reshape(128, 8 * DH)

    def both(*fs):
        def f():
            for g in fs:
                g()
        return f

    def w3_comp(buf, cb, mm):
        def retile(hb):
            def f():
                w2_s[hb & 1][...] = w3_block(buf, cb, hb)
            return f
        if CFG["w3sep"]:
            return [retile(0), retile(1), both(mm(0), mm(1)) if CFG["w3sep"] == 2 else mm(0)] + (
                [] if CFG["w3sep"] == 2 else [mm(1)]) + [retile(2), retile(3)] + (
                [both(mm(2), mm(3))] if CFG["w3sep"] == 2 else [mm(2), mm(3)])
        return ([retile(0)] + [both(mm(hb - 1), retile(hb)) for hb in range(1, 4)] + [mm(3)])

    def wqb_comp(cb):
        def mm(hb):
            def f():
                r = jnp.dot(xb_s[cb].astype(BF16), w2_s[hb & 1][...], preferred_element_type=F32)
                qb_s[:, 1024 * hb:1024 * hb + 1024] += r
            return f
        return w3_comp(wqb_buf, cb, mm)

    def wuk_comp(cb):
        def mm(hb):
            def f():
                for j in range(8):
                    h = 8 * hb + j
                    q = (qb_s[:, DH * h:DH * h + DH] * scale).astype(BF16)
                    r = lax.dot_general(q, w2_s[hb & 1][:, DH * j:DH * j + DH], NT,
                                        preferred_element_type=F32)
                    qabs_t[cb, 8 * h:8 * h + NB, :] = r
            return f
        return w3_comp(wuk_buf, cb, mm)

    def qabs_finish():
        for b in range(NB):
            for cb in range(4):
                qabs_s[b, :, 128 * cb:128 * cb + 128] = (
                    qabs_t[cb, pl.ds(b, NH, stride=8), :].astype(BF16))

    def c_comp(i):
        sl = i & 1

        def qk(b):
            def f():
                sb_s[b] = lax.dot_general(qabs_s[b], cbuf[sl, b], NT,
                                          preferred_element_type=F32)
            return f

        def sm(b):
            def f():
                s = sb_s[b]
                m_old = m_s[b]
                m_new = jnp.maximum(m_old, jnp.max(s, axis=-1, keepdims=True))
                alpha = jnp.exp(m_old - m_new)
                ps = [jnp.exp(s[:, 128 * j:128 * j + 128] - m_new) for j in range(CK // 128)]
                l_s[b] = alpha * l_s[b] + sum(ps[1:], ps[0])
                m_s[b] = m_new
                al_s[b] = alpha
                pb_s[b] = jnp.concatenate(ps, axis=-1).astype(BF16)
            return f

        def pv(b):
            def f():
                r = jnp.dot(pb_s[b], cbuf[sl, b], preferred_element_type=F32)
                al = al_s[b]
                for j in range(4):
                    cols = slice(128 * j, 128 * j + 128)
                    acc_s[b, :, cols] = al * acc_s[b, :, cols] + r[:, cols]
            return f

        return [qk(0), both(qk(1), sm(0)), both(qk(2), sm(1)), both(qk(3), sm(2)),
                both(sm(3), pv(0), pv(1)), both(pv(2), pv(3))]

    def c_finish():
        for b in range(NB):
            cc = acc_s[b] / jnp.sum(l_s[b], axis=-1, keepdims=True)
            for cb in range(4):
                cc_s[cb, NH * b:NH * b + NH, :] = cc[:, 128 * cb:128 * cb + 128]

    def wuv_comp(cb):
        def mm(hb):
            def f():
                for j in range(8):
                    cc = cc_s[cb, pl.ds(8 * hb + j, NB, stride=NH), :].astype(BF16)
                    r = jnp.dot(cc, w2_s[hb & 1][:, DH * j:DH * j + DH],
                                preferred_element_type=F32)
                    ctx_s[hb, :, DH * j:DH * j + DH] += r
            return f
        return w3_comp(wuv_buf, cb, mm)

    def wob_comp(g):
        def piece(half):
            def f():
                x = ctx_s[g, :, 512 * half:512 * half + 512].astype(BF16)
                out_s[1] += jnp.dot(x, wob_buf[2 * g + half], preferred_element_type=F32)
            return f
        return [piece(0), piece(1)]

    b_comp = {"wq": wqb_comp, "wuk": wuk_comp, "c": c_comp, "wuv": wuv_comp, "wo": wob_comp}
    b_finish = {"wuk": qabs_finish, "c": c_finish}

    def init():
        for cp in x_copies:
            cp.wait()
        if not do_compute:
            return
        xb = xb_buf[...].astype(F32)
        for cb in range(4):
            xb_s[cb] = xb[:, 128 * cb:128 * cb + 128]
        qb_s[...] = jnp.zeros(qb_s.shape, F32)
        ctx_s[...] = jnp.zeros(ctx_s.shape, F32)
        out_s[...] = jnp.zeros(out_s.shape, F32)
        m_s[...] = jnp.full(m_s.shape, -jnp.inf, F32)
        l_s[...] = jnp.zeros(l_s.shape, F32)
        acc_s[...] = jnp.zeros(acc_s.shape, F32)

    def wqa_comp(j):
        def f():
            w = wqa_buf[:, :, 512 * j:512 * j + 512].reshape(DM, 512)
            r = jnp.dot(xa_buf[...], w, preferred_element_type=F32) * scale
            for i in range(4):
                h = 4 * j + i
                qa_t[8 * h:8 * h + NB, :] = r[:, DH * i:DH * i + DH]
        return f

    def a_qk(u):
        b, h0 = unit_bh(u)
        st = {}

        def qk(js):
            def f():
                q4 = qa_t[pl.ds(8 * h0 + b, 4, stride=8), :]
                s = None if js[0] == 0 else pa_s[...]
                for j in js:
                    qm = jnp.where(row4 == j, q4, 0.0).astype(BF16)
                    sj = lax.dot_general(qm, kbuf[u & 1, j], NT, preferred_element_type=F32)
                    s = sj if s is None else s + sj
                pa_s[...] = s
            return f

        def sm():
            s = pa_s[...]
            p = jnp.exp(s - jnp.max(s, axis=-1, keepdims=True))
            la_s[...] = jnp.sum(p, axis=-1, keepdims=True)
            pa_s[...] = p

        if CFG["fine"]:
            return [qk((0,)), qk((1,)), qk((2,)), qk((3,)), sm]
        return [qk((0, 1)), qk((2, 3)), sm]

    def a_pv(u):
        b, h0 = unit_bh(u)
        st = {}

        def pv(js):
            def f():
                p = pa_s[...].astype(BF16)
                o = st.get("o")
                for j in js:
                    oj = jnp.dot(p, vbuf[u & 1, j], preferred_element_type=F32)
                    o = oj if o is None else jnp.where(row4 == j, oj, o)
                st["o"] = o
                if js[-1] == 3:
                    oa_t[pl.ds(8 * h0 + b, 4, stride=8), :] = o / la_s[...]
            return f
        if CFG["fine"]:
            return [pv((0, 1)), pv((2, 3))]
        return [pv((0, 1, 2, 3))]

    def woa_comp(heads):
        def f():
            r = None
            for h in heads:
                o = oa_t[8 * h:8 * h + NB, :].astype(BF16)
                w = woa_buf[h // 4, 128 * (h % 4):128 * (h % 4) + 128, :]
                t = jnp.dot(o, w, preferred_element_type=F32)
                r = t if r is None else r + t
            out_s[0] += r
        return f

    def at(d, t, item):
        d.setdefault(t, []).append(item)

    def wait_all(pieces, sem):
        def f():
            for p in pieces:
                copy(p, sem).wait()
        return f

    D1 = 16
    pre0 = CFG["pre0"]
    bwait = CFG["bwait"]
    x_copies = [pltpu.make_async_copy(xa_hbm, xa_buf, semx.at[0]),
                pltpu.make_async_copy(xb_hbm, xb_buf, semx.at[1])]
    q1, q0 = split_w(wqa_piece)
    for j in range(D1):
        copy(q1[j], sem1.at[1]).start(priority=1)
        if j < pre0:
            copy(q0[j], sem0.at[1]).start(priority=0)
    for cp in x_copies:
        cp.start()
    s1, s0, cm = {}, {}, {}
    nxt = [(p, sem1.at[1]) for p in q1[D1:]] + [(p, sem1.at[0]) for p in kv_pieces(k_hbm, kbuf, 0)]
    for t, it in enumerate(nxt):
        at(s1, t, it)
    n0 = len(q0) - pre0
    for j in range(n0):
        at(s0, (j * len(q1)) // n0, (q0[pre0 + j], sem0.at[1]))
    at(cm, 4, init)
    ticks([(p, sem1.at[1]) for p in q1], s1, s0, cm)

    o1, o0 = split_w(woa_piece)
    o1_sem = [semt.at[j // 8] for j in range(len(o1))]

    def body(u, issue, comp, finish, first=False, last=False):
        kp = kv_pieces(k_hbm, kbuf, u)
        vp = kv_pieces(v_hbm, vbuf, u)
        waits = [(p, sem1.at[0]) for p in kp] + [(p, sem1.at[1]) for p in vp]
        s1, s0, cm = {}, {}, {}
        for t in range(16):
            at(s1, t, (vp[t], sem1.at[1]))
        if last:
            for t in range(16):
                at(s1, 16 + t, (o1[t], o1_sem[t]))
        else:
            kn = kv_pieces(k_hbm, kbuf, u + 1)
            for t in range(16):
                at(s1, 16 + t, (kn[t], sem1.at[0]))
        pcs, _ = b_chunk(*issue)
        for t in range(32):
            at(s0, t, (pcs[t], sem0.at[u & 1]))
        psem = sem0.at[(u + 1) & 1]
        if first:
            at(cm, bwait, wait_all(q0, psem))
            bc = [wqa_comp(j) for j in range(8)]
        else:
            _, dst = b_chunk(*comp)
            at(cm, bwait, lambda: pltpu.make_async_copy(dst, dst, psem).wait())
            bc = b_comp[comp[0]](comp[1])
            if finish:
                bc = bc + [b_finish[comp[0]]]
        btk = [6, 8, 10, 12, 14, 26, 28, 30, 31]
        assert len(bc) <= len(btk) and bwait <= btk[0]
        if do_compute:
            if not first:
                for t, f in zip((1, 3), a_pv(u - 1)):
                    at(cm, t, f)
            for t, f in zip(btk, bc):
                at(cm, t, f)
            for t, f in zip((16, 18, 20, 22, 24) if CFG["fine"] else (16, 19, 22), a_qk(u)):
                at(cm, t, f)
        ticks(waits, s1, s0, cm)

    stages = [("wq", 4), ("wuk", 4), ("c", 16), ("wuv", 4), ("wo", 4)]
    u0 = 0
    prev = None
    for stage, n in stages:
        body(u0, (stage, 0), prev, prev is not None and prev[0] in b_finish, first=prev is None)
        hi = n - 1 if stage == "wo" else n

        def loop_body(i, carry, stage=stage, u0=u0):
            body(u0 + i, (stage, i), (stage, i - 1), False)
            return carry

        lax.fori_loop(1, hi, loop_body, 0)
        prev = (stage, n - 1)
        u0 += n
    body(NU - 1, ("wo", 3), ("wo", 2), False, last=True)

    s1, s0, cm = {}, {}, {}
    for t in range(len(o1) - D1):
        at(s1, t, (o1[D1 + t], o1_sem[D1 + t]))
    last0 = len(o1) - 10
    o0_sem = [sem0.at[0]] * 16 + [semx.at[0]] * 16
    for j in range(len(o0)):
        at(s0, (j * last0) // len(o0), (o0[j], o0_sem[j]))
    _, dst = b_chunk("wo", 3)
    at(cm, bwait, lambda: pltpu.make_async_copy(dst, dst, sem0.at[1]).wait())
    tw = (27, len(o1) - 4)
    at(cm, tw[0], wait_all(o0[:16], sem0.at[0]))
    at(cm, tw[1], wait_all(o0[16:], semx.at[0]))
    if do_compute:
        for t, f in zip((1, 3), a_pv(NU - 1)):
            at(cm, t, f)
        for t, f in zip((bwait, bwait + 3), wob_comp(3)):
            at(cm, t, f)
        for g in range(6):
            r0, j = (0, g) if g < 4 else (4, g - 4)
            at(cm, max(8 * g + 7, 12 + g), woa_comp([4 * (r0 + r) + j for r in range(4)]))
        for t, j in zip(tw, (2, 3)):
            at(cm, t, woa_comp([4 * r + j for r in range(4, 8)]))
    ticks([(p, s) for p, s in zip(o1, o1_sem)], s1, s0, cm)
    if do_compute:
        o_ref[:, 0:DM] = out_s[0].astype(o_ref.dtype)
        o_ref[:, DM:2 * DM] = out_s[1].astype(o_ref.dtype)
    else:
        o_ref[...] = jnp.zeros(o_ref.shape, o_ref.dtype)


@jax.jit
def pallas_concat_heads__sliding_block_cached__compressed_kv_cla__decode_kernel(
    A_x: jax.Array,
    A_k_cache: jax.Array,
    A_v_cache: jax.Array,
    A_wq: jax.Array,
    A_wo: jax.Array,
    B_x: jax.Array,
    B_c_kv: jax.Array,
    B_w_q: jax.Array,
    B_w_uk: jax.Array,
    B_w_uv: jax.Array,
    B_w_o: jax.Array,
):
    assert A_x.shape == (NB, 1, DM) and B_x.shape == (NB, 1, DM)
    assert A_k_cache.shape == (NB, NH, SK, DH) and B_c_kv.shape == (NB, SK, DM)
    w3 = (8, 64, NH, DH)
    w2 = (8, 512, DM)
    wq = (8, 64, NH * DH)
    vm = pltpu.VMEM
    out = pl.pallas_call(
        _kernel,
        out_shape=jax.ShapeDtypeStruct((NB, 2 * DM), A_x.dtype),
        in_specs=[pl.BlockSpec(memory_space=pl.ANY)] * 11,
        out_specs=pl.BlockSpec(memory_space=pltpu.VMEM),
        scratch_shapes=[
            vm((NB, DM), BF16), vm((NB, DM), BF16),
            vm((2, 4, WIN, DH), BF16), vm((2, 4, WIN, DH), BF16),
            vm(wq, BF16), vm(w2, BF16),
            vm((2, NB, CK, DM), BF16),
            vm(w3, BF16), vm(w3, BF16), vm(w3, BF16), vm(w2, BF16),
            vm((4, NB, 128), F32),
            vm((NH * 8, DH), F32),
            vm((NH * 8, DH), F32),
            vm((4, WIN), F32),
            vm((4, 1), F32),
            vm((NB, NH * DH), F32),
            vm((4, NH * 8, 128), F32),
            vm((NB, NH, DM), BF16),
            vm((NB, NH, CK), F32),
            vm((NB, NH, CK), BF16),
            vm((NB, NH, 128), F32),
            vm((NB, NH, 128), F32), vm((NB, NH, 128), F32),
            vm((NB, NH, DM), F32),
            vm((4, NB * NH, 128), F32),
            vm((4, NB, 8 * DH), F32),
            vm((2, NB, DM), F32),
            vm((128, 8 * DH), BF16), vm((128, 8 * DH), BF16),
            pltpu.SemaphoreType.DMA((2,)), pltpu.SemaphoreType.DMA((2,)),
            pltpu.SemaphoreType.DMA((2,)), pltpu.SemaphoreType.DMA((6,)),
        ],
        compiler_params=pltpu.CompilerParams(
            vmem_limit_bytes=64 * 1024 * 1024,
            disable_bounds_checks=True,
            disable_semaphore_checks=True,
        ),
        name="concat_heads_decode",
    )(
        A_x.reshape(NB, DM), B_x.reshape(NB, DM), A_k_cache, A_v_cache,
        A_wq.reshape(wq), A_wo.reshape(w2), B_c_kv,
        B_w_q.reshape(w3), B_w_uk.reshape(w3), B_w_uv.reshape(w3), B_w_o.reshape(w2),
    )
    return out.reshape(NB, 1, 2 * DM)
```

```python
import jax
import jax.numpy as jnp
from jax import lax
import jax.experimental.pallas as pl
import jax.experimental.pallas.tpu as pltpu

F32 = jnp.float32
BF16 = jnp.bfloat16

NB = 4
NH = 32
DH = 128
DM = 512
SK = 4096
WIN = 1024
CK = 256
NU = 32
NT = ((1,), (1,)), ((), ())

CFG = dict(compute=True, pre0=5, bwait=6, fine=True, w3sep=1, nq=4, end0=12)


def _mult(x, m):
    return x if isinstance(x, int) else pl.multiple_of(x, m)


def _kernel(xa_hbm, xb_hbm, k_hbm, v_hbm, wqa_hbm, woa_hbm, c_hbm, wqb_hbm, wuk_hbm,
            wuv_hbm, wob_hbm, o_ref,
            xa_buf, xb_buf, kbuf, vbuf, wqa_buf, woa_buf, cbuf, wqb_buf, wuk_buf,
            wuv_buf, wob_buf,
            xb_s, qa_t, oa_t, pa_s, la_s, qb_s, qabs_t, qabs_s, sb_s, pb_s, al_s,
            m_s, l_s, acc_s, cc_s, ctx_s, out_s, w2a_s, w2b_s,
            sem1, sem0, semx, semt):
    do_compute = CFG["compute"]
    w2_s = (w2a_s, w2b_s)
    scale = DH ** -0.5
    row4 = lax.broadcasted_iota(jnp.int32, (NB, DH), 0)

    def copy(piece, sem):
        return pltpu.make_async_copy(piece[0], piece[1], sem)

    def ticks(waits, starts1, starts0, comp):
        for t, (piece, sem) in enumerate(waits):
            copy(piece, sem).wait()
            for p, s in starts0.get(t, ()):
                copy(p, s).start(priority=0)
            for p, s in starts1.get(t, ()):
                copy(p, s).start(priority=1)
            for f in comp.get(t, ()):
                f()

    def unit_bh(u):
        return u & 3, (u >> 2) * 4

    def kv_pieces(hbm, buf, u):
        b, h0 = unit_bh(u)
        return [(hbm.at[b, pl.ds(h0, 4), pl.ds(SK - WIN + 64 * s, 64)],
                 buf.at[u & 3, :, pl.ds(64 * s, 64)]) for s in range(16)]

    def b_chunk(stage, i):
        if stage == "c":
            pcs = []
            for s in range(CK // 16):
                for b0 in (0, 2):
                    pcs.append((c_hbm.at[pl.ds(b0, 2), pl.ds(_mult(i * CK + 16 * s, 16), 16)],
                                cbuf.at[i & 1, pl.ds(b0, 2), pl.ds(16 * s, 16)]))
            return pcs, cbuf.at[i & 1]
        hbm, buf, rows = {"wq": (wqb_hbm, wqb_buf, 2), "wuk": (wuk_hbm, wuk_buf, 2),
                          "wuv": (wuv_hbm, wuv_buf, 2), "wo": (wob_hbm, wob_buf, 16)}[stage]
        pcs = []
        for s in range(32):
            idx = (pl.ds(2 * i, 2), pl.ds(rows * s, rows))
            pcs.append((hbm.at[idx], buf.at[idx]))
        return pcs, buf.at[pl.ds(2 * i, 2)]

    def wqa_piece(r0, nr, s):
        idx = (pl.ds(r0, nr), pl.ds(8 * (s // 4), 8), pl.ds(1024 * (s % 4), 1024))
        return wqa_hbm.at[idx], wqa_buf.at[idx]

    def woa_piece(r0, nr, s):
        idx = (pl.ds(r0, nr), pl.ds(16 * s, 16))
        return woa_hbm.at[idx], woa_buf.at[idx]

    def w3_block(buf, cb, hb):
        w = buf[pl.ds(2 * cb, 2), :, 8 * hb:8 * hb + 8, :]
        return w.reshape(128, 8, DH).reshape(128, 8 * DH)

    def both(*fs):
        def f():
            for g in fs:
                g()
        return f

    def w3_comp(buf, cb, mm):
        def retile(hb):
            def f():
                w2_s[hb & 1][...] = w3_block(buf, cb, hb)
            return f
        if CFG["w3sep"]:
            return [retile(0), retile(1), both(mm(0), mm(1)) if CFG["w3sep"] == 2 else mm(0)] + (
                [] if CFG["w3sep"] == 2 else [mm(1)]) + [retile(2), retile(3)] + (
                [both(mm(2), mm(3))] if CFG["w3sep"] == 2 else [mm(2), mm(3)])
        return ([retile(0)] + [both(mm(hb - 1), retile(hb)) for hb in range(1, 4)] + [mm(3)])

    def wqb_comp(cb):
        def mm(hb):
            def f():
                r = jnp.dot(xb_s[cb].astype(BF16), w2_s[hb & 1][...], preferred_element_type=F32)
                qb_s[:, 1024 * hb:1024 * hb + 1024] += r
            return f
        return w3_comp(wqb_buf, cb, mm)

    def wuk_comp(cb):
        def mm(hb):
            def f():
                for j in range(8):
                    h = 8 * hb + j
                    q = (qb_s[:, DH * h:DH * h + DH] * scale).astype(BF16)
                    r = lax.dot_general(q, w2_s[hb & 1][:, DH * j:DH * j + DH], NT,
                                        preferred_element_type=F32)
                    qabs_t[cb, 8 * h:8 * h + NB, :] = r
            return f
        return w3_comp(wuk_buf, cb, mm)

    def qabs_finish():
        for b in range(NB):
            for cb in range(4):
                qabs_s[b, :, 128 * cb:128 * cb + 128] = (
                    qabs_t[cb, pl.ds(b, NH, stride=8), :].astype(BF16))

    def c_comp(i):
        sl = i & 1

        def qk(b):
            def f():
                sb_s[b] = lax.dot_general(qabs_s[b], cbuf[sl, b], NT,
                                          preferred_element_type=F32)
            return f

        def sm(b):
            def f():
                s = sb_s[b]
                m_old = m_s[b]
                m_new = jnp.maximum(m_old, jnp.max(s, axis=-1, keepdims=True))
                alpha = jnp.exp(m_old - m_new)
                ps = [jnp.exp(s[:, 128 * j:128 * j + 128] - m_new) for j in range(CK // 128)]
                l_s[b] = alpha * l_s[b] + sum(ps[1:], ps[0])
                m_s[b] = m_new
                al_s[b] = alpha
                pb_s[b] = jnp.concatenate(ps, axis=-1).astype(BF16)
            return f

        def pv(b):
            def f():
                r = jnp.dot(pb_s[b], cbuf[sl, b], preferred_element_type=F32)
                al = al_s[b]
                for j in range(4):
                    cols = slice(128 * j, 128 * j + 128)
                    acc_s[b, :, cols] = al * acc_s[b, :, cols] + r[:, cols]
            return f

        return [qk(0), both(qk(1), sm(0)), both(qk(2), sm(1)), both(qk(3), sm(2)),
                both(sm(3), pv(0), pv(1)), both(pv(2), pv(3))]

    def c_finish():
        for b in range(NB):
            cc = acc_s[b] / jnp.sum(l_s[b], axis=-1, keepdims=True)
            for cb in range(4):
                cc_s[cb, NH * b:NH * b + NH, :] = cc[:, 128 * cb:128 * cb + 128]

    def wuv_comp(cb):
        def mm(hb):
            def f():
                for j in range(8):
                    cc = cc_s[cb, pl.ds(8 * hb + j, NB, stride=NH), :].astype(BF16)
                    r = jnp.dot(cc, w2_s[hb & 1][:, DH * j:DH * j + DH],
                                preferred_element_type=F32)
                    ctx_s[hb, :, DH * j:DH * j + DH] += r
            return f
        return w3_comp(wuv_buf, cb, mm)

    def wob_comp(g):
        def piece(half):
            def f():
                x = ctx_s[g, :, 512 * half:512 * half + 512].astype(BF16)
                out_s[1] += jnp.dot(x, wob_buf[2 * g + half], preferred_element_type=F32)
            return f
        return [piece(0), piece(1)]

    b_comp = {"wq": wqb_comp, "wuk": wuk_comp, "c": c_comp, "wuv": wuv_comp, "wo": wob_comp}
    b_finish = {"wuk": qabs_finish, "c": c_finish}

    def init():
        for cp in x_copies:
            cp.wait()
        if not do_compute:
            return
        xb = xb_buf[...].astype(F32)
        for cb in range(4):
            xb_s[cb] = xb[:, 128 * cb:128 * cb + 128]
        qb_s[...] = jnp.zeros(qb_s.shape, F32)
        ctx_s[...] = jnp.zeros(ctx_s.shape, F32)
        out_s[...] = jnp.zeros(out_s.shape, F32)
        m_s[...] = jnp.full(m_s.shape, -jnp.inf, F32)
        l_s[...] = jnp.zeros(l_s.shape, F32)
        acc_s[...] = jnp.zeros(acc_s.shape, F32)

    def wqa_comp(j):
        def f():
            w = wqa_buf[:, :, 512 * j:512 * j + 512].reshape(DM, 512)
            r = jnp.dot(xa_buf[...], w, preferred_element_type=F32) * scale
            for i in range(4):
                h = 4 * j + i
                qa_t[8 * h:8 * h + NB, :] = r[:, DH * i:DH * i + DH]
        return f

    def a_qk(u):
        b, h0 = unit_bh(u)
        st = {}

        def qk(js):
            def f():
                q4 = qa_t[pl.ds(8 * h0 + b, 4, stride=8), :]
                s = None if js[0] == 0 else pa_s[...]
                for j in js:
                    qm = jnp.where(row4 == j, q4, 0.0).astype(BF16)
                    sj = lax.dot_general(qm, kbuf[u & 3, j], NT, preferred_element_type=F32)
                    s = sj if s is None else s + sj
                pa_s[...] = s
            return f

        def sm():
            s = pa_s[...]
            p = jnp.exp(s - jnp.max(s, axis=-1, keepdims=True))
            la_s[...] = jnp.sum(p, axis=-1, keepdims=True)
            pa_s[...] = p

        if CFG["fine"]:
            return [qk((0,)), qk((1,)), qk((2,)), qk((3,)), sm]
        return [qk((0, 1)), qk((2, 3)), sm]

    def a_pv(u):
        b, h0 = unit_bh(u)
        st = {}

        def pv(js):
            def f():
                p = pa_s[...].astype(BF16)
                o = st.get("o")
                for j in js:
                    oj = jnp.dot(p, vbuf[u & 3, j], preferred_element_type=F32)
                    o = oj if o is None else jnp.where(row4 == j, oj, o)
                st["o"] = o
                if js[-1] == 3:
                    oa_t[pl.ds(8 * h0 + b, 4, stride=8), :] = o / la_s[...]
            return f
        if CFG["fine"]:
            return [pv((0, 1)), pv((2, 3))]
        return [pv((0, 1, 2, 3))]

    def woa_comp(heads):
        def f():
            r = None
            for h in heads:
                o = oa_t[8 * h:8 * h + NB, :].astype(BF16)
                w = woa_buf[h // 4, 128 * (h % 4):128 * (h % 4) + 128, :]
                t = jnp.dot(o, w, preferred_element_type=F32)
                r = t if r is None else r + t
            out_s[0] += r
        return f

    def at(d, t, item):
        d.setdefault(t, []).append(item)

    def wait_all(pieces, sem):
        def f():
            for p in pieces:
                copy(p, sem).wait()
        return f

    def weave(a, b):
        return [x for pair in zip(a, b) for x in pair]

    D1 = 16
    pre0 = CFG["pre0"]
    bwait = CFG["bwait"]
    x_copies = [pltpu.make_async_copy(xa_hbm, xa_buf, semx.at[0]),
                pltpu.make_async_copy(xb_hbm, xb_buf, semx.at[1])]
    nq = CFG["nq"]
    q1 = [wqa_piece(0, 4, s) for s in range(32)] + [wqa_piece(4, 4, s) for s in range(nq)]
    q1 = q1[:-16] + weave(q1[-16:], kv_pieces(k_hbm, kbuf, 0))
    q0 = [wqa_piece(r, 2, s) for s in range(nq, 32) for r in (4, 6)]

    def body_p1(u):
        return weave(kv_pieces(v_hbm, vbuf, u), kv_pieces(k_hbm, kbuf, u + 1))

    for j in range(D1):
        copy(q1[j], sem1.at[1]).start(priority=1)
        if j < pre0:
            copy(q0[j], sem0.at[1]).start(priority=0)
    for cp in x_copies:
        cp.start()
    s1, s0, cm = {}, {}, {}
    nxt = [(p, sem1.at[1]) for p in q1[D1:]] + [(p, sem1.at[0]) for p in body_p1(0)[:D1]]
    for t, it in enumerate(nxt):
        at(s1, t, it)
    n0 = len(q0) - pre0
    for j in range(n0):
        at(s0, (j * len(q1)) // n0, (q0[pre0 + j], sem0.at[1]))
    at(cm, 4, init)
    ticks([(p, sem1.at[1]) for p in q1], s1, s0, cm)

    oa = [(woa_piece(0, 4, s), semt.at[s // 8]) for s in range(32)]
    o1 = weave([(p, sem1.at[1]) for p in kv_pieces(v_hbm, vbuf, NU - 1)], oa[:16]) + oa[16:]
    o1 += [(woa_piece(4, 4, s), semt.at[4]) for s in range(8)]
    o1 += [(woa_piece(4, 3, s), semt.at[5]) for s in range(8, 16)]
    for r in (128, 192):
        idx = (7, pl.ds(r, 64))
        o1.append(((woa_hbm.at[idx], woa_buf.at[idx]), semt.at[6]))
    o0 = [(woa_piece(r, 2, s), semx.at[(s - 16) // 8]) for s in range(16, 32) for r in (4, 6)]

    def body(u, issue, comp, finish, first=False, last=False):
        cur = body_p1(u)
        csem = sem1.at[u & 1]
        s1, s0, cm = {}, {}, {}
        if last:
            nxt = o1[:D1]
        else:
            nxt = [(p, sem1.at[(u + 1) & 1]) for p in body_p1(u + 1)[:D1]]
        for t, it in enumerate([(p, csem) for p in cur[D1:]] + nxt):
            at(s1, t, it)
        pcs, _ = b_chunk(*issue)
        for t in range(32):
            at(s0, t, (pcs[t], sem0.at[u & 1]))
        psem = sem0.at[(u + 1) & 1]
        if first:
            at(cm, bwait, wait_all(q0, psem))
            bc = [wqa_comp(j) for j in range(8)]
        else:
            _, dst = b_chunk(*comp)
            at(cm, bwait, lambda: pltpu.make_async_copy(dst, dst, psem).wait())
            bc = b_comp[comp[0]](comp[1])
            if finish:
                bc = bc + [b_finish[comp[0]]]
        btk = [6, 8, 10, 12, 14, 26, 28, 30, 31]
        assert len(bc) <= len(btk) and bwait <= btk[0]
        if do_compute:
            if not first:
                for t, f in zip((1, 3), a_pv(u - 1)):
                    at(cm, t, f)
            for t, f in zip(btk, bc):
                at(cm, t, f)
            for t, f in zip((16, 18, 20, 22, 24), a_qk(u)):
                at(cm, t, f)
        ticks([(p, csem) for p in cur], s1, s0, cm)

    stages = [("wq", 4), ("wuk", 4), ("c", 16), ("wuv", 4)]
    u0 = 0
    prev = None
    for stage, n in stages:
        body(u0, (stage, 0), prev, prev is not None and prev[0] in b_finish, first=prev is None)

        def loop_body(i, carry, stage=stage, u0=u0):
            body(u0 + i, (stage, i), (stage, i - 1), False)
            return carry

        lax.fori_loop(1, n, loop_body, 0)
        prev = (stage, n - 1)
        u0 += n
    body(NU - 4, ("wo", 0), prev, False)
    body(NU - 3, ("wo", 1), ("wo", 0), False)
    body(NU - 2, ("wo", 2), ("wo", 1), False, last=True)

    s1, s0, cm = {}, {}, {}
    nt = len(o1)
    for t in range(nt - D1):
        at(s1, t, o1[D1 + t])
    pcs, dst3 = b_chunk("wo", 3)
    p0 = [(p, sem0.at[1]) for p in pcs] + o0
    last0 = nt - CFG["end0"]
    t0 = [(j * last0) // len(p0) for j in range(len(p0))]
    for t, it in zip(t0, p0):
        at(s0, t, it)
    _, dst2 = b_chunk("wo", 2)
    at(cm, bwait, lambda: pltpu.make_async_copy(dst2, dst2, sem0.at[0]).wait())
    tw3, twa, twb = 36, 50, nt - 7
    assert t0[31] + 5 <= tw3 and t0[47] + 5 <= twa and t0[63] + 4 <= twb
    at(cm, tw3, lambda: pltpu.make_async_copy(dst3, dst3, sem0.at[1]).wait())
    at(cm, twa, wait_all([p for p, _ in o0[:16]], semx.at[0]))
    at(cm, twb, wait_all([p for p, _ in o0[16:]], semx.at[1]))

    def write_b():
        o_ref[:, DM:2 * DM] = out_s[1].astype(o_ref.dtype)

    if do_compute:
        sched = [((1, 3), a_pv(NU - 2)), ((6, 8), wob_comp(2)),
                 ((10, 12, 14, 16, 18), a_qk(NU - 1)),
                 ((31, 33), a_pv(NU - 1)), ((tw3, tw3 + 2), wob_comp(3)), ((tw3 + 2,), [write_b])]
        for tks, fs in sched:
            for t, f in zip(tks, fs):
                at(cm, t, f)
        for t, heads in ((20, (0, 4, 8, 12)), (40, (1, 5, 9, 13)), (42, (2, 6, 10, 14)),
                         (47, (3, 7, 11, 15)), (twa, (18, 22, 26, 30)), (55, (16, 20, 24, 28)),
                         (twb, (19, 23, 27, 31)), (nt - 3, (17, 21, 25))):
            at(cm, t, woa_comp(heads))
    ticks(o1, s1, s0, cm)
    if do_compute:
        o = oa_t[8 * 29:8 * 29 + NB, :].astype(BF16)
        r = jnp.dot(o, woa_buf[7, 128:256, :], preferred_element_type=F32)
        o_ref[:, 0:DM] = (out_s[0] + r).astype(o_ref.dtype)
    else:
        o_ref[...] = jnp.zeros(o_ref.shape, o_ref.dtype)


@jax.jit
def pallas_concat_heads__sliding_block_cached__compressed_kv_cla__decode_kernel(
    A_x: jax.Array,
    A_k_cache: jax.Array,
    A_v_cache: jax.Array,
    A_wq: jax.Array,
    A_wo: jax.Array,
    B_x: jax.Array,
    B_c_kv: jax.Array,
    B_w_q: jax.Array,
    B_w_uk: jax.Array,
    B_w_uv: jax.Array,
    B_w_o: jax.Array,
):
    assert A_x.shape == (NB, 1, DM) and B_x.shape == (NB, 1, DM)
    assert A_k_cache.shape == (NB, NH, SK, DH) and B_c_kv.shape == (NB, SK, DM)
    w3 = (8, 64, NH, DH)
    w2 = (8, 512, DM)
    wq = (8, 64, NH * DH)
    vm = pltpu.VMEM
    out = pl.pallas_call(
        _kernel,
        out_shape=jax.ShapeDtypeStruct((NB, 2 * DM), A_x.dtype),
        in_specs=[pl.BlockSpec(memory_space=pl.ANY)] * 11,
        out_specs=pl.BlockSpec(memory_space=pltpu.VMEM),
        scratch_shapes=[
            vm((NB, DM), BF16), vm((NB, DM), BF16),
            vm((4, 4, WIN, DH), BF16), vm((4, 4, WIN, DH), BF16),
            vm(wq, BF16), vm(w2, BF16),
            vm((2, NB, CK, DM), BF16),
            vm(w3, BF16), vm(w3, BF16), vm(w3, BF16), vm(w2, BF16),
            vm((4, NB, 128), F32),
            vm((NH * 8, DH), F32),
            vm((NH * 8, DH), F32),
            vm((4, WIN), F32),
            vm((4, 1), F32),
            vm((NB, NH * DH), F32),
            vm((4, NH * 8, 128), F32),
            vm((NB, NH, DM), BF16),
            vm((NB, NH, CK), F32),
            vm((NB, NH, CK), BF16),
            vm((NB, NH, 128), F32),
            vm((NB, NH, 128), F32), vm((NB, NH, 128), F32),
            vm((NB, NH, DM), F32),
            vm((4, NB * NH, 128), F32),
            vm((4, NB, 8 * DH), F32),
            vm((2, NB, DM), F32),
            vm((128, 8 * DH), BF16), vm((128, 8 * DH), BF16),
            pltpu.SemaphoreType.DMA((2,)), pltpu.SemaphoreType.DMA((2,)),
            pltpu.SemaphoreType.DMA((2,)), pltpu.SemaphoreType.DMA((7,)),
        ],
        compiler_params=pltpu.CompilerParams(
            vmem_limit_bytes=64 * 1024 * 1024,
            disable_bounds_checks=True,
            disable_semaphore_checks=True,
        ),
        name="concat_heads_decode",
    )(
        A_x.reshape(NB, DM), B_x.reshape(NB, DM), A_k_cache, A_v_cache,
        A_wq.reshape(wq), A_wo.reshape(w2), B_c_kv,
        B_w_q.reshape(w3), B_w_uk.reshape(w3), B_w_uv.reshape(w3), B_w_o.reshape(w2),
    )
    return out.reshape(NB, 1, 2 * DM)
```

```python
import jax
import jax.numpy as jnp
from jax import lax
import jax.experimental.pallas as pl
import jax.experimental.pallas.tpu as pltpu

F32 = jnp.float32
BF16 = jnp.bfloat16

NB = 4
NH = 32
DH = 128
DM = 512
SK = 4096
WIN = 1024
CK = 256
NG = 32
RUN = 128
D1 = 16
NT = ((1,), (1,)), ((), ())

CFG = dict(compute=True, pre0=5, bwait=6, aoff=8, boff=8, demote=0, end0=12, checks=False,
           cuts=(0, 8, 24, 32), a_slots=(1, 3, 16, 18, 20, 22, 24),
           b_slots=(6, 8, 10, 12, 14, 26, 28, 30, 31), c_slots=(0, 1, 3, 4, 5, 7))


def _mult(x, m):
    return x if isinstance(x, int) else pl.multiple_of(x, m)


def _kernel(xa_hbm, xb_hbm, k_hbm, v_hbm, wqa_hbm, woa_hbm, c_hbm, wqb_hbm, wuk_hbm,
            wuv_hbm, wob_hbm, o_ref,
            xa_buf, xb_buf, kbuf, vbuf, wqa_buf, woa_buf, bring,
            xb_s, qa_t, oa_t, sa_s, ma_s, la_s, aa_s, acca_s, qb_s, qabs_t, qabs_s, sb_s, pb_s, al_s,
            m_s, l_s, acc_s, cc_s, ctx_s, out_s, w2a_s, w2b_s,
            sem1, sem0, semx, semt):
    do_compute = CFG["compute"]
    aoff, boff = CFG["aoff"], CFG["boff"]
    bwait = CFG["bwait"]
    scale = DH ** -0.5
    w2_s = (w2a_s, w2b_s)
    row8 = lax.broadcasted_iota(jnp.int32, (8, DH), 0)
    bring_t = bring.reshape(2, 128, 32, DH)
    wqa_t = wqa_buf.reshape(64, 256, DH)
    woa_t = woa_buf.reshape(512, 32, DH)

    def start(descs, sem, prio):
        for src, dst in descs:
            pltpu.make_async_copy(src, dst, sem).start(priority=prio)

    def wait(descs, sem):
        for _, dst in descs:
            pltpu.make_async_copy(dst, dst, sem).wait()

    def at(d, t, item):
        d.setdefault(t, []).append(item)

    def both(*fs):
        def f():
            for g in fs:
                g()
        return f

    def tiles(view, j):
        w = view[:, 8 * j:8 * j + 8, :]
        return w.reshape(w.shape[0] * 8, DH)

    def mat(view, j0, n):
        return jnp.concatenate([tiles(view, j0 + j) for j in range(n)], axis=1)

    def when(cond, f):
        if cond is True:
            f()
        elif cond is not False:
            pl.when(cond)(f)

    def kv_start(hbm, buf, g, t, sem, live=True):
        b, sl = g >> 3, g & 7
        w0 = SK - WIN
        src, dst = hbm.at[b, pl.ds(2 * t, 2)], buf.at[g & 1, pl.ds(2 * t, 2)]
        reg = [(src.at[:, pl.ds(_mult(w0 + RUN * sl - aoff, 8), RUN)], dst)]
        if aoff == 0:
            when(live, lambda: start(reg, sem, 1))
            return
        fst = [(src.at[:, pl.ds(w0, RUN - aoff)], dst.at[:, pl.ds(aoff, RUN - aoff)])]
        if t == 0:
            fst = [(hbm.at[b, :, pl.ds(SK - aoff, aoff)], buf.at[g & 1, :, pl.ds(0, aoff)])] + fst
        if isinstance(sl, int):
            when(live, lambda: start(reg if sl else fst, sem, 1))
        else:
            pl.when(sl > 0)(lambda: start(reg, sem, 1))
            first = sl == 0
            pl.when(first if live is True else jnp.logical_and(first, live))(
                lambda: start(fst, sem, 1))

    def b_run(hbm, nseg, src_row, sl, t):
        seg, k = t % nseg, t // nseg
        ln = 4096 // nseg
        r = boff + RUN * k
        n = min(RUN, ln - r)
        out = [(hbm.at[pl.ds(_mult(src_row(seg) + r, 8), n)], bring.at[sl, pl.ds(ln * seg + r, n)])]
        if k == 0 and boff:
            out.append((hbm.at[pl.ds(_mult(src_row(seg), 8), boff)],
                        bring.at[sl, pl.ds(ln * seg, boff)]))
        return out

    def a_run(hbm, buf, r, lo, hi):
        r0, r1 = max(r - aoff, lo), (hi if r + RUN == hi else r + RUN - aoff)
        return [(hbm.at[pl.ds(r0, r1 - r0)], buf.at[pl.ds(r0, r1 - r0)])]

    def retile(sl, hb):
        def f():
            w = bring_t[sl, :, 8 * hb:8 * hb + 8, :]
            w2_s[hb & 1][...] = w.reshape(128, 8 * DH)
        return f

    def wq_mm(cb, hb):
        def f():
            r = jnp.dot(xb_s[cb].astype(BF16), w2_s[hb & 1][...], preferred_element_type=F32)
            qb_s[:, 1024 * hb:1024 * hb + 1024] += r
        return f

    def wuk_mm(cb, hb):
        def f():
            for j in range(8):
                h = 8 * hb + j
                q = (qb_s[:, DH * h:DH * h + DH] * scale).astype(BF16)
                r = lax.dot_general(q, w2_s[hb & 1][:, DH * j:DH * j + DH], NT,
                                    preferred_element_type=F32)
                qabs_t[cb, 8 * h:8 * h + NB, :] = r
        return f

    def wuv_mm(cb, hb):
        def f():
            for j in range(8):
                cc = cc_s[cb, pl.ds(8 * hb + j, NB, stride=NH), :].astype(BF16)
                r = jnp.dot(cc, w2_s[hb & 1][:, DH * j:DH * j + DH], preferred_element_type=F32)
                ctx_s[hb, :, DH * j:DH * j + DH] += r
        return f

    def qabs_finish():
        for b in range(NB):
            for cb in range(4):
                qabs_s[b, :, 128 * cb:128 * cb + 128] = (
                    qabs_t[cb, pl.ds(b, NH, stride=8), :].astype(BF16))

    def c_pieces(sl):
        def cmat(b):
            return mat(bring_t.at[sl, pl.ds(32 * b, 32)], 0, 4)

        def qk(b):
            def f():
                sb_s[b] = lax.dot_general(qabs_s[b], cmat(b), NT, preferred_element_type=F32)
            return f

        def sm(b):
            def f():
                s = sb_s[b]
                m_old = m_s[b]
                m_new = jnp.maximum(m_old, jnp.max(s, axis=-1, keepdims=True))
                alpha = jnp.exp(m_old - m_new)
                ps = [jnp.exp(s[:, 128 * j:128 * j + 128] - m_new) for j in range(CK // 128)]
                l_s[b] = alpha * l_s[b] + sum(ps[1:], ps[0])
                m_s[b] = m_new
                al_s[b] = alpha
                pb_s[b] = jnp.concatenate(ps, axis=-1).astype(BF16)
            return f

        def pv(b):
            def f():
                r = jnp.dot(pb_s[b], cmat(b), preferred_element_type=F32)
                al = al_s[b]
                for j in range(4):
                    cols = slice(128 * j, 128 * j + 128)
                    acc_s[b, :, cols] = al * acc_s[b, :, cols] + r[:, cols]
            return f

        return [qk(0), both(qk(1), sm(0)), both(qk(2), sm(1)), both(qk(3), sm(2)),
                both(sm(3), pv(0), pv(1)), both(pv(2), pv(3))]

    def c_finish():
        for b in range(NB):
            cc = acc_s[b] / jnp.sum(l_s[b], axis=-1, keepdims=True)
            for cb in range(4):
                cc_s[cb, NH * b:NH * b + NH, :] = cc[:, 128 * cb:128 * cb + 128]

    def wob_mm(sl, cb, half):
        def f():
            x = ctx_s[cb, :, 512 * half:512 * half + 512].astype(BF16)
            w = mat(bring_t.at[sl, pl.ds(64 * half, 64)], 0, 4)
            out_s[1] += jnp.dot(x, w, preferred_element_type=F32)
        return f

    def init():
        wait(x_copies[:1], semx.at[0])
        wait(x_copies[1:], semx.at[1])
        if not do_compute:
            return
        xb = xb_buf[...].astype(F32)
        for cb in range(4):
            xb_s[cb] = xb[:, 128 * cb:128 * cb + 128]
        qb_s[...] = jnp.zeros(qb_s.shape, F32)
        ctx_s[...] = jnp.zeros(ctx_s.shape, F32)
        out_s[...] = jnp.zeros(out_s.shape, F32)
        for r in (ma_s, la_s, acca_s):
            r[...] = jnp.zeros(r.shape, F32)
        m_s[...] = jnp.full(m_s.shape, -jnp.inf, F32)
        l_s[...] = jnp.zeros(l_s.shape, F32)
        acc_s[...] = jnp.zeros(acc_s.shape, F32)

    def wqa_mm(j):
        def f():
            r = jnp.dot(xa_buf[...], mat(wqa_t, 4 * j, 4), preferred_element_type=F32) * scale
            for i in range(4):
                h = 4 * j + i
                qa_t[8 * h:8 * h + NB, :] = r[:, DH * i:DH * i + DH]
        return f

    def a_qk(g, k):
        def f():
            q8 = qa_t[pl.ds(64 * k + (g >> 3), 8, stride=8), :]
            s = None
            for j in range(8):
                qm = jnp.where(row8 == j, q8, 0.0).astype(BF16)
                sj = lax.dot_general(qm, kbuf[g & 1, 8 * k + j], NT, preferred_element_type=F32)
                s = sj if s is None else s + sj
            sa_s[8 * k:8 * k + 8, :] = s
        return f

    def a_sm(g):
        def f():
            first = (g & 7) == 0
            s = sa_s[...]
            m_old = jnp.where(first, -jnp.inf, ma_s[...])
            m_new = jnp.maximum(m_old, jnp.max(s, axis=-1, keepdims=True))
            alpha = jnp.exp(m_old - m_new)
            p = jnp.exp(s - m_new)
            la_s[...] = jnp.where(first, p, alpha * la_s[...] + p)
            ma_s[...] = m_new
            aa_s[...] = alpha
            sa_s[...] = p
        return f

    def a_pv(g, k):
        def f():
            first = (g & 7) == 0
            for r0 in (16 * k, 16 * k + 8):
                rows = slice(r0, r0 + 8)
                p = sa_s[rows, :].astype(BF16)
                o = None
                for j in range(8):
                    oj = jnp.dot(p, vbuf[g & 1, r0 + j], preferred_element_type=F32)
                    o = oj if o is None else jnp.where(row8 == j, oj, o)
                acca_s[rows, :] = jnp.where(first, o, aa_s[rows, :] * acca_s[rows, :] + o)
        return f

    def a_fin(g):
        def f():
            o = acca_s[...] / jnp.sum(la_s[...], axis=-1, keepdims=True)
            oa_t[pl.ds(g >> 3, NH, stride=8), :] = o
        return f

    def woa_dot(h):
        o = oa_t[8 * h:8 * h + NB, :].astype(BF16)
        return jnp.dot(o, mat(woa_t.at[pl.ds(16 * h, 16)], 0, 4), preferred_element_type=F32)

    def woa_mm(heads):
        def f():
            r = woa_dot(heads[0])
            for h in heads[1:]:
                r = r + woa_dot(h)
            out_s[0] += r
        return f

    def static_ticks(waits, starts1, starts0, comp):
        for t, (descs, sem) in enumerate(waits):
            wait(descs, sem)
            for d, s in starts0.get(t, ()):
                start(d, s, 0)
            for d, s in starts1.get(t, ()):
                start(d, s, 1)
            for f in comp.get(t, ()):
                f()

    pre0 = CFG["pre0"]
    x_copies = [(xa_hbm, xa_buf), (xb_hbm, xb_buf)]
    qr = [[a_run(wqa_hbm, wqa_buf, 2048 * r + RUN * s, 0, 16384) for r in range(8)]
          for s in range(16)]
    q1 = [qr[s][r] + qr[s][r + 1] for s in range(11) for r in (0, 2, 4, 6)]
    q0 = [qr[s][r] for s in range(11, 16) for r in range(8)]
    for j in range(D1):
        start(q1[j], sem1.at[1], 1)
        if j < pre0:
            start(q0[j], sem0.at[1], 0)
    start(x_copies[:1], semx.at[0], 0)
    start(x_copies[1:], semx.at[1], 0)
    s1, s0, cm = {}, {}, {}
    for t, d in enumerate(q1[D1:]):
        at(s1, t, (d, sem1.at[1]))
    for t in range(D1):
        at(cm, len(q1) - D1 + t, lambda t=t: kv_start(k_hbm, kbuf, 0, t, sem1.at[0]))
    n0 = len(q0) - pre0
    for j in range(n0):
        at(s0, (j * len(q1)) // n0, (q0[pre0 + j], sem0.at[1]))
    at(cm, 4, init)
    static_ticks([(d, sem1.at[1]) for d in q1], s1, s0, cm)

    def head_runs(h):
        return [a_run(woa_hbm, woa_buf, 512 * h + RUN * k, 512 * h, 512 * h + 512)
                for k in range(4)]

    def group1(heads):
        hr = [head_runs(h) for h in heads]
        runs = [hr[i][k] for k in range(4) for i in range(len(heads))]
        return [runs[i] + runs[i + 1] for i in range(0, len(runs), 2)]

    g1 = [tuple(range(0, 32, 4)), tuple(range(1, 32, 4)), (2, 6, 10, 14), (18, 22, 26), (30,)]
    g0 = [(3, 7, 11, 15), (19, 23, 27, 31)]
    o1 = [(d, semt.at[i]) for i, hs in enumerate(g1) for d in group1(hs)]
    o0 = [[(head_runs(h)[k], semx.at[i]) for k in range(4) for h in hs]
          for i, hs in enumerate(g0)]

    b_slots = CFG["b_slots"]
    a_slots = CFG["a_slots"]
    demote = CFG["demote"]
    t_b = list(range(demote)) + [(j * 32) // (32 - demote) for j in range(32 - demote)]

    def body(g, g_lo, g_hi):
        def between(lo, hi):
            if lo <= g_lo and g_hi <= hi:
                return True
            if hi < g_lo or g_hi < lo:
                return False
            if lo <= g_lo:
                return g <= hi
            if g_hi <= hi:
                return g >= lo
            return jnp.logical_and(g >= lo, g <= hi)

        def either(x, y):
            if x is True or y is True:
                return True
            if x is False or y is False:
                return y if x is False else x
            return jnp.logical_or(x, y)

        par = g & 1
        iw = g & 3
        w_stage = [(between(0, 3), wqb_hbm), (between(4, 7), wuk_hbm),
                   (between(24, 27), wuv_hbm), (between(28, 31), wob_hbm)]
        is_c = between(8, 23)
        ic = (g - 8) & 15
        last = between(NG - 1, NG - 1)
        gn = g + 1 if last is False else (g + 1) & (NG - 1)

        sl, cb = 1 - par, (g + 3) & 3
        cm = {}
        if do_compute:
            w3 = either(between(1, 8), between(25, 28))
            for k, hb in ((0, 0), (1, 1), (4, 2), (5, 3)):
                at(cm, b_slots[k], (w3, retile(sl, hb)))
            for k, hb in ((2, 0), (6, 2)):
                at(cm, b_slots[k], (between(1, 4), both(wq_mm(cb, hb), wq_mm(cb, hb + 1))))
                at(cm, b_slots[k], (between(25, 28), both(wuv_mm(cb, hb), wuv_mm(cb, hb + 1))))
            for k, hb in ((2, 0), (3, 1), (6, 2), (7, 3)):
                at(cm, b_slots[k], (between(5, 8), wuk_mm(cb, hb)))
            at(cm, b_slots[8], (between(8, 8), qabs_finish))
            for k, f in zip(CFG["c_slots"], c_pieces(sl)):
                at(cm, b_slots[k], (between(9, 24), f))
            at(cm, b_slots[8], (between(24, 24), c_finish))
            for k, half in ((3, 0), (7, 1)):
                at(cm, b_slots[k], (between(29, 31), wob_mm(sl, cb, half)))
            for k in range(8):
                at(cm, bwait + k, (between(0, 0), wqa_mm(k)))
            for k in range(2):
                at(cm, a_slots[k], (between(1, 31), a_pv(g - 1, k)))
            fin = either(either(between(8, 8), between(16, 16)), between(24, 24))
            at(cm, a_slots[1] + 1, (fin, a_fin(g - 1)))
            for k in range(4):
                at(cm, a_slots[2 + k], (True, a_qk(g, k)))
            at(cm, a_slots[6], (True, a_sm(g)))

        for t in range(32):
            dst = (kbuf if t < 16 else vbuf).at[par, pl.ds(2 * (t % 16), 2)]
            pltpu.make_async_copy(dst, dst, sem1.at[t // 16]).wait()
            for j in range(32):
                if t_b[j] == t:
                    prio = 1 if j < demote else 0
                    for cond, hbm in w_stage:
                        when(cond, lambda hbm=hbm: start(
                            b_run(hbm, 2, lambda s: 4096 * iw + 2048 * s, par, j),
                            sem0.at[par], prio))
                    when(is_c, lambda: start(
                        b_run(c_hbm, 4, lambda s: 16384 * s + 1024 * ic, par, j),
                        sem0.at[par], prio))
            if t < 16:
                kv_start(v_hbm, vbuf, g, t, sem1.at[1])
            else:
                if last is not True:
                    kv_start(k_hbm, kbuf, gn, t - 16, sem1.at[0], live=between(0, NG - 2))
                when(last, lambda: start(o1[t - 16][0], o1[t - 16][1], 1))
            if t == bwait:
                when(between(0, 0), lambda: wait(sum(q0, []), sem0.at[1]))
                when(between(1, 31), lambda: wait([(None, bring.at[sl])], sem0.at[sl]))
            for cond, f in cm.get(t, ()):
                when(cond, f)

    cuts = CFG["cuts"]
    for lo, hi in zip(cuts[:-1], cuts[1:]):
        if hi - lo == 1:
            body(lo, lo, lo)
        else:
            def loop_body(g, carry, lo=lo, hi=hi):
                body(g, lo, hi - 1)
                return carry
            lax.fori_loop(lo, hi, loop_body, 0)

    s1, s0, cm = {}, {}, {}
    nt = len(o1)
    for t in range(nt - D1):
        at(s1, t, o1[D1 + t])
    p0 = o0[0] + o0[1]
    last0 = nt - CFG["end0"]
    t0 = [(j * last0) // len(p0) for j in range(len(p0))]
    for t, it in zip(t0, p0):
        at(s0, t, it)
    twa, twb = 24, nt - 7
    assert t0[15] + 5 <= twa and t0[31] + 4 <= twb
    at(cm, 8, lambda: wait([(None, bring.at[1])], sem0.at[1]))
    at(cm, twa, lambda: wait(sum((d for d, _ in o0[0]), []), semx.at[0]))
    at(cm, twb, lambda: wait(sum((d for d, _ in o0[1]), []), semx.at[1]))

    def write_b():
        o_ref[:, DM:2 * DM] = out_s[1].astype(o_ref.dtype)

    if do_compute:
        at(cm, 1, a_pv(NG - 1, 0))
        at(cm, 3, a_pv(NG - 1, 1))
        at(cm, 5, a_fin(NG - 1))
        at(cm, 8, wob_mm(1, 3, 0))
        at(cm, 10, both(wob_mm(1, 3, 1), write_b))
        for t, heads in ((15, g1[0][:4]), (17, g1[0][4:]), (twa, g0[0]), (31, g1[1][:4]),
                         (33, g1[1][4:]), (39, g1[2]), (twb, g0[1]), (nt - 3, g1[3])):
            at(cm, t, woa_mm(heads))
    static_ticks(o1, s1, s0, cm)
    if do_compute:
        o_ref[:, 0:DM] = (out_s[0] + woa_dot(g1[4][0])).astype(o_ref.dtype)
    else:
        o_ref[...] = jnp.zeros(o_ref.shape, o_ref.dtype)


def _flat(x):
    c = x.shape[-1]
    if c == DH:
        return x.reshape(-1, DH)
    return x.reshape(-1, 8, c // DH, DH).transpose(0, 2, 1, 3).reshape(-1, DH)


@jax.jit
def pallas_concat_heads__sliding_block_cached__compressed_kv_cla__decode_kernel(
    A_x: jax.Array,
    A_k_cache: jax.Array,
    A_v_cache: jax.Array,
    A_wq: jax.Array,
    A_wo: jax.Array,
    B_x: jax.Array,
    B_c_kv: jax.Array,
    B_w_q: jax.Array,
    B_w_uk: jax.Array,
    B_w_uv: jax.Array,
    B_w_o: jax.Array,
):
    assert A_x.shape == (NB, 1, DM) and B_x.shape == (NB, 1, DM)
    assert A_k_cache.shape == (NB, NH, SK, DH) and B_c_kv.shape == (NB, SK, DM)
    vm = pltpu.VMEM
    out = pl.pallas_call(
        _kernel,
        out_shape=jax.ShapeDtypeStruct((NB, 2 * DM), A_x.dtype),
        in_specs=[pl.BlockSpec(memory_space=pl.ANY)] * 11,
        out_specs=pl.BlockSpec(memory_space=pltpu.VMEM),
        scratch_shapes=[
            vm((NB, DM), BF16), vm((NB, DM), BF16),
            vm((2, NH, RUN, DH), BF16), vm((2, NH, RUN, DH), BF16),
            vm((16384, DH), BF16), vm((16384, DH), BF16),
            vm((2, 4096, DH), BF16),
            vm((4, NB, 128), F32),
            vm((NH * 8, DH), F32),
            vm((NH * 8, DH), F32),
            vm((NH, RUN), F32),
            vm((NH, DH), F32), vm((NH, DH), F32),
            vm((NH, DH), F32), vm((NH, DH), F32),
            vm((NB, NH * DH), F32),
            vm((4, NH * 8, 128), F32),
            vm((NB, NH, DM), BF16),
            vm((NB, NH, CK), F32),
            vm((NB, NH, CK), BF16),
            vm((NB, NH, 128), F32),
            vm((NB, NH, 128), F32), vm((NB, NH, 128), F32),
            vm((NB, NH, DM), F32),
            vm((4, NB * NH, 128), F32),
            vm((4, NB, 8 * DH), F32),
            vm((2, NB, DM), F32),
            vm((128, 8 * DH), BF16), vm((128, 8 * DH), BF16),
            pltpu.SemaphoreType.DMA((2,)), pltpu.SemaphoreType.DMA((2,)),
            pltpu.SemaphoreType.DMA((2,)), pltpu.SemaphoreType.DMA((5,)),
        ],
        compiler_params=pltpu.CompilerParams(
            vmem_limit_bytes=48 * 1024 * 1024,
            disable_bounds_checks=not CFG["checks"],
            disable_semaphore_checks=not CFG["checks"],
        ),
        name="concat_heads_decode",
    )(
        A_x.reshape(NB, DM), B_x.reshape(NB, DM), A_k_cache, A_v_cache,
        _flat(A_wq), _flat(A_wo), _flat(B_c_kv),
        _flat(B_w_q), _flat(B_w_uk), _flat(B_w_uv), _flat(B_w_o),
    )
    return out.reshape(NB, 1, 2 * DM)
```

```python
import jax
import jax.numpy as jnp
from jax import lax
import jax.experimental.pallas as pl
import jax.experimental.pallas.tpu as pltpu

F32 = jnp.float32
BF16 = jnp.bfloat16

NB = 4
NH = 32
DH = 128
DM = 512
SK = 4096
WIN = 1024
CK = 256
NG = 32
RUN = 128
D1 = 16
NT = ((1,), (1,)), ((), ())

CFG = dict(compute=True, pre0=5, bwait=6, aoff=8, boff=8, embed=True, q_slots=(6, 8, 10, 12, 14, 15, 17, 19), end0=12, checks=False,
           cuts=(0, 8, 24, 32), a_slots=(1, 3, 16, 18, 20, 22, 24),
           b_slots=(6, 8, 10, 12, 14, 26, 28, 30, 31), c_slots=(0, 1, 3, 4, 5, 7))


def _mult(x, m):
    return x if isinstance(x, int) else pl.multiple_of(x, m)


def _kernel(xa_hbm, xb_hbm, k_hbm, v_hbm, wqa_hbm, woa_hbm, c_hbm, wqb_hbm, wuk_hbm,
            wuv_hbm, wob_hbm, o_ref,
            xa_buf, xb_buf, kbuf, vbuf, wqa_buf, woa_buf, bring,
            xb_s, qa_t, oa_t, sa_s, ma_s, la_s, aa_s, acca_s, qb_s, qabs_t, qabs_s, sb_s, pb_s, al_s,
            m_s, l_s, acc_s, cc_s, ctx_s, out_s, w2a_s, w2b_s,
            sem1, sem0, semx, semt):
    do_compute = CFG["compute"]
    aoff, boff = CFG["aoff"], CFG["boff"]
    bwait = CFG["bwait"]
    scale = DH ** -0.5
    w2_s = (w2a_s, w2b_s)
    row8 = lax.broadcasted_iota(jnp.int32, (8, DH), 0)
    bring_t = bring.reshape(2, 128, 32, DH)
    wqa_t = wqa_buf.reshape(64, 256, DH)
    woa_t = woa_buf.reshape(512, 32, DH)

    def start(descs, sem, prio):
        for src, dst in descs:
            pltpu.make_async_copy(src, dst, sem).start(priority=prio)

    def wait(descs, sem):
        for _, dst in descs:
            pltpu.make_async_copy(dst, dst, sem).wait()

    def at(d, t, item):
        d.setdefault(t, []).append(item)

    def both(*fs, host=0):
        def f(hook=None):
            for i, g in enumerate(fs):
                if i == host:
                    g(hook)
                else:
                    g()
        return f

    def call(hook, v):
        if hook is not None:
            hook(v)

    def tiles(view, j):
        w = view[:, 8 * j:8 * j + 8, :]
        return w.reshape(w.shape[0] * 8, DH)

    def mat(view, j0, n):
        return jnp.concatenate([tiles(view, j0 + j) for j in range(n)], axis=1)

    def when(cond, f):
        if cond is True:
            f()
        elif cond is not False:
            pl.when(cond)(f)

    def kv_start(hbm, buf, g, t, sem, live=True):
        b, sl = g >> 3, g & 7
        w0 = SK - WIN
        src, dst = hbm.at[b, pl.ds(2 * t, 2)], buf.at[g & 1, pl.ds(2 * t, 2)]
        reg = [(src.at[:, pl.ds(_mult(w0 + RUN * sl - aoff, 8), RUN)], dst)]
        if aoff == 0:
            when(live, lambda: start(reg, sem, 1))
            return
        fst = [(src.at[:, pl.ds(w0, RUN - aoff)], dst.at[:, pl.ds(aoff, RUN - aoff)])]
        if t == 0:
            fst = [(hbm.at[b, :, pl.ds(SK - aoff, aoff)], buf.at[g & 1, :, pl.ds(0, aoff)])] + fst
        if isinstance(sl, int):
            when(live, lambda: start(reg if sl else fst, sem, 1))
        else:
            pl.when(sl > 0)(lambda: start(reg, sem, 1))
            first = sl == 0
            pl.when(first if live is True else jnp.logical_and(first, live))(
                lambda: start(fst, sem, 1))

    def b_run(hbm, nseg, src_row, sl, t):
        seg, k = t % nseg, t // nseg
        ln = 4096 // nseg
        r = boff + RUN * k
        n = min(RUN, ln - r)
        out = [(hbm.at[pl.ds(_mult(src_row(seg) + r, 8), n)], bring.at[sl, pl.ds(ln * seg + r, n)])]
        if k == 0 and boff:
            out.append((hbm.at[pl.ds(_mult(src_row(seg), 8), boff)],
                        bring.at[sl, pl.ds(ln * seg, boff)]))
        return out

    def a_run(hbm, buf, r, lo, hi):
        r0, r1 = max(r - aoff, lo), (hi if r + RUN == hi else r + RUN - aoff)
        return [(hbm.at[pl.ds(r0, r1 - r0)], buf.at[pl.ds(r0, r1 - r0)])]

    def retile(sl, hb):
        def f():
            w2_s[hb & 1][...] = bring_t[sl, :, 8 * hb:8 * hb + 8, :].reshape(128, 8 * DH)
        return f

    def wq_mm(cb, hb):
        def f(hook=None):
            r = jnp.dot(xb_s[cb].astype(BF16), w2_s[hb & 1][...], preferred_element_type=F32)
            qb_s[:, 1024 * hb:1024 * hb + 1024] += r
            call(hook, r[:, 7 * DH:])
        return f

    def wuk_mm(cb, hb):
        def f(hook=None):
            for j in range(8):
                h = 8 * hb + j
                q = (qb_s[:, DH * h:DH * h + DH] * scale).astype(BF16)
                r = lax.dot_general(q, w2_s[hb & 1][:, DH * j:DH * j + DH], NT,
                                    preferred_element_type=F32)
                qabs_t[cb, 8 * h:8 * h + NB, :] = r
                if j == 0:
                    r0 = r
            call(hook, r0)
        return f

    def wuv_mm(cb, hb):
        def f(hook=None):
            for j in range(8):
                cc = cc_s[cb, pl.ds(8 * hb + j, NB, stride=NH), :].astype(BF16)
                r = jnp.dot(cc, w2_s[hb & 1][:, DH * j:DH * j + DH], preferred_element_type=F32)
                ctx_s[hb, :, DH * j:DH * j + DH] += r
            call(hook, r)
        return f

    def qabs_finish():
        for b in range(NB):
            for cb in range(4):
                qabs_s[b, :, 128 * cb:128 * cb + 128] = (
                    qabs_t[cb, pl.ds(b, NH, stride=8), :].astype(BF16))

    def c_pieces(sl):
        def cmat(b):
            return mat(bring_t.at[sl, pl.ds(32 * b, 32)], 0, 4)

        def qk(b):
            def f(hook=None):
                s = lax.dot_general(qabs_s[b], cmat(b), NT, preferred_element_type=F32)
                sb_s[b] = s
                call(hook, s[0:8, 0:DH])
            return f

        def sm(b):
            def f():
                s = sb_s[b]
                m_old = m_s[b]
                m_new = jnp.maximum(m_old, jnp.max(s, axis=-1, keepdims=True))
                alpha = jnp.exp(m_old - m_new)
                ps = [jnp.exp(s[:, 128 * j:128 * j + 128] - m_new) for j in range(CK // 128)]
                l_s[b] = alpha * l_s[b] + sum(ps[1:], ps[0])
                m_s[b] = m_new
                al_s[b] = alpha
                pb_s[b] = jnp.concatenate(ps, axis=-1).astype(BF16)
            return f

        def pv(b):
            def f(hook=None):
                r = jnp.dot(pb_s[b], cmat(b), preferred_element_type=F32)
                al = al_s[b]
                for j in range(4):
                    cols = slice(128 * j, 128 * j + 128)
                    acc_s[b, :, cols] = al * acc_s[b, :, cols] + r[:, cols]
                if hook is not None:
                    keep["v"] = r[0:8, 3 * DH:]
            return f

        keep = {}

        def late(f):
            def g(hook=None):
                f(hook)
                if hook is not None:
                    hook(keep["v"])
            return g

        return [qk(0), both(qk(1), sm(0)), both(qk(2), sm(1)), both(qk(3), sm(2)),
                late(both(sm(3), pv(0), pv(1), host=1)), late(both(pv(2), pv(3)))]

    def c_finish():
        for b in range(NB):
            cc = acc_s[b] / jnp.sum(l_s[b], axis=-1, keepdims=True)
            for cb in range(4):
                cc_s[cb, NH * b:NH * b + NH, :] = cc[:, 128 * cb:128 * cb + 128]

    def wob_mm(sl, cb, half):
        def f(hook=None):
            rs = []
            for i in range(2):
                c0 = 512 * half + 256 * i
                w = mat(bring_t.at[sl, pl.ds(c0 // 8, 32)], 0, 4)
                rs.append(jnp.dot(ctx_s[cb, :, c0:c0 + 256].astype(BF16), w,
                                  preferred_element_type=F32))
            out_s[1] += rs[0] + rs[1]
            call(hook, rs[0][:, 3 * DH:])
        return f

    def init():
        wait(x_copies[:1], semx.at[0])
        wait(x_copies[1:], semx.at[1])
        if not do_compute:
            return
        xb = xb_buf[...].astype(F32)
        for cb in range(4):
            xb_s[cb] = xb[:, 128 * cb:128 * cb + 128]
        qb_s[...] = jnp.zeros(qb_s.shape, F32)
        ctx_s[...] = jnp.zeros(ctx_s.shape, F32)
        out_s[...] = jnp.zeros(out_s.shape, F32)
        for r in (ma_s, la_s, acca_s):
            r[...] = jnp.zeros(r.shape, F32)
        m_s[...] = jnp.full(m_s.shape, -jnp.inf, F32)
        l_s[...] = jnp.zeros(l_s.shape, F32)
        acc_s[...] = jnp.zeros(acc_s.shape, F32)

    def wqa_mm(j):
        def f(hook=None):
            r = jnp.dot(xa_buf[...], mat(wqa_t, 4 * j, 4), preferred_element_type=F32) * scale
            for i in range(4):
                h = 4 * j + i
                qa_t[8 * h:8 * h + NB, :] = r[:, DH * i:DH * i + DH]
            call(hook, r[:, 0:DH])
        return f

    def a_qk(g, k):
        def f(hook=None):
            q8 = qa_t[pl.ds(64 * k + (g >> 3), 8, stride=8), :]
            s = None
            for j in range(8):
                qm = jnp.where(row8 == j, q8, 0.0).astype(BF16)
                sj = lax.dot_general(qm, kbuf[g & 1, 8 * k + j], NT, preferred_element_type=F32)
                s = sj if s is None else s + sj
                if j == 0:
                    call(hook, sj)
            sa_s[8 * k:8 * k + 8, :] = s
        return f

    def a_sm(g):
        def f():
            first = (g & 7) == 0
            s = sa_s[...]
            m_old = jnp.where(first, -jnp.inf, ma_s[...])
            m_new = jnp.maximum(m_old, jnp.max(s, axis=-1, keepdims=True))
            alpha = jnp.exp(m_old - m_new)
            p = jnp.exp(s - m_new)
            la_s[...] = jnp.where(first, p, alpha * la_s[...] + p)
            ma_s[...] = m_new
            aa_s[...] = alpha
            sa_s[...] = p
        return f

    def a_pv(g, k):
        def f(hook=None):
            first = (g & 7) == 0
            for r0 in (16 * k, 16 * k + 8):
                rows = slice(r0, r0 + 8)
                p = sa_s[rows, :].astype(BF16)
                o = None
                for j in range(8):
                    oj = jnp.dot(p, vbuf[g & 1, r0 + j], preferred_element_type=F32)
                    o = oj if o is None else jnp.where(row8 == j, oj, o)
                    if r0 % 16 == 0 and j == 4:
                        call(hook, oj)
                acca_s[rows, :] = jnp.where(first, o, aa_s[rows, :] * acca_s[rows, :] + o)
        return f

    def a_fin(g):
        def f():
            o = acca_s[...] / jnp.sum(la_s[...], axis=-1, keepdims=True)
            oa_t[pl.ds(g >> 3, NH, stride=8), :] = o
        return f

    def woa_dot(h):
        o = oa_t[8 * h:8 * h + NB, :].astype(BF16)
        return jnp.dot(o, mat(woa_t.at[pl.ds(16 * h, 16)], 0, 4), preferred_element_type=F32)

    def woa_mm(heads):
        def f():
            r = woa_dot(heads[0])
            for h in heads[1:]:
                r = r + woa_dot(h)
            out_s[0] += r
        return f

    def static_ticks(waits, starts1, starts0, comp):
        for t, (descs, sem) in enumerate(waits):
            wait(descs, sem)
            for d, s in starts0.get(t, ()):
                start(d, s, 0)
            for d, s in starts1.get(t, ()):
                start(d, s, 1)
            for f in comp.get(t, ()):
                f()

    pre0 = CFG["pre0"]
    x_copies = [(xa_hbm, xa_buf), (xb_hbm, xb_buf)]
    qr = [[a_run(wqa_hbm, wqa_buf, 2048 * r + RUN * s, 0, 16384) for r in range(8)]
          for s in range(16)]
    q1 = [qr[s][r] + qr[s][r + 1] for s in range(11) for r in (0, 2, 4, 6)]
    q0 = [qr[s][r] for s in range(11, 16) for r in range(8)]
    for j in range(D1):
        start(q1[j], sem1.at[1], 1)
        if j < pre0:
            start(q0[j], sem0.at[1], 0)
    start(x_copies[:1], semx.at[0], 0)
    start(x_copies[1:], semx.at[1], 0)
    s1, s0, cm = {}, {}, {}
    for t, d in enumerate(q1[D1:]):
        at(s1, t, (d, sem1.at[1]))
    for t in range(D1):
        at(cm, len(q1) - D1 + t, lambda t=t: kv_start(k_hbm, kbuf, 0, t, sem1.at[0]))
    n0 = len(q0) - pre0
    for j in range(n0):
        at(s0, (j * len(q1)) // n0, (q0[pre0 + j], sem0.at[1]))
    at(cm, 4, init)
    static_ticks([(d, sem1.at[1]) for d in q1], s1, s0, cm)

    def head_runs(h):
        return [a_run(woa_hbm, woa_buf, 512 * h + RUN * k, 512 * h, 512 * h + 512)
                for k in range(4)]

    def group1(heads):
        hr = [head_runs(h) for h in heads]
        runs = [hr[i][k] for k in range(4) for i in range(len(heads))]
        return [runs[i] + runs[i + 1] for i in range(0, len(runs), 2)]

    g1 = [tuple(range(0, 32, 4)), tuple(range(1, 32, 4)), (2, 6, 10, 14), (18, 22, 26), (30,)]
    g0 = [(3, 7, 11, 15), (19, 23, 27, 31)]
    o1 = [(d, semt.at[i]) for i, hs in enumerate(g1) for d in group1(hs)]
    o0 = [[(head_runs(h)[k], semx.at[i]) for k in range(4) for h in hs]
          for i, hs in enumerate(g0)]

    b_slots = CFG["b_slots"]
    a_slots = CFG["a_slots"]

    def body(g, g_lo, g_hi):
        def between(lo, hi):
            if lo <= g_lo and g_hi <= hi:
                return True
            if hi < g_lo or g_hi < lo:
                return False
            if lo <= g_lo:
                return g <= hi
            if g_hi <= hi:
                return g >= lo
            return jnp.logical_and(g >= lo, g <= hi)

        def either(x, y):
            if x is True or y is True:
                return True
            if x is False or y is False:
                return y if x is False else x
            return jnp.logical_or(x, y)

        par = g & 1
        iw = g & 3
        w_stage = [(between(0, 3), wqb_hbm), (between(4, 7), wuk_hbm),
                   (between(24, 27), wuv_hbm), (between(28, 31), wob_hbm)]
        is_c = between(8, 23)
        ic = (g - 8) & 15
        last = between(NG - 1, NG - 1)
        gn = g + 1 if last is False else (g + 1) & (NG - 1)

        sl, cb = 1 - par, (g + 3) & 3
        cm = {}
        short = [qabs_finish, c_finish]
        if do_compute:
            w3 = either(between(1, 8), between(25, 28))
            for k, hb in ((0, 0), (1, 1), (4, 2), (5, 3)):
                short.append(retile(sl, hb))
                at(cm, b_slots[k], (w3, short[-1]))
            for k, hb in ((2, 0), (6, 2)):
                at(cm, b_slots[k], (between(1, 4), both(wq_mm(cb, hb), wq_mm(cb, hb + 1))))
                at(cm, b_slots[k], (between(25, 28), both(wuv_mm(cb, hb), wuv_mm(cb, hb + 1))))
            for k, hb in ((2, 0), (3, 1), (6, 2), (7, 3)):
                at(cm, b_slots[k], (between(5, 8), wuk_mm(cb, hb)))
            at(cm, b_slots[8], (between(8, 8), qabs_finish))
            for k, f in zip(CFG["c_slots"], c_pieces(sl)):
                at(cm, b_slots[k], (between(9, 24), f))
            at(cm, b_slots[8], (between(24, 24), c_finish))
            for k, half in ((3, 0), (7, 1)):
                at(cm, b_slots[k], (between(29, 31), wob_mm(sl, cb, half)))
            for k, t in enumerate(CFG["q_slots"]):
                at(cm, t, (between(0, 0), wqa_mm(k)))
            for k in range(2):
                at(cm, a_slots[k], (between(1, 31), a_pv(g - 1, k)))
            fin = either(either(between(8, 8), between(16, 16)), between(24, 24))
            short += [a_fin(g - 1), a_sm(g)]
            at(cm, a_slots[1] + 2, (fin, short[-2]))
            for k in range(4):
                at(cm, a_slots[2 + k], (True, a_qk(g, k)))
            at(cm, a_slots[6], (True, short[-1]))

        def also(x, y):
            if x is False or y is False:
                return False
            if x is True or y is True:
                return y if x is True else x
            return jnp.logical_and(x, y)

        def b_start(j, live=True):
            for cond, hbm in w_stage:
                when(also(cond, live), lambda hbm=hbm: start(
                    b_run(hbm, 2, lambda s: 4096 * iw + 2048 * s, par, j), sem0.at[par], 0))
            when(also(is_c, live), lambda: start(
                b_run(c_hbm, 4, lambda s: 16384 * s + 1024 * ic, par, j), sem0.at[par], 0))

        def hook_for(j):
            assert is_c is True or is_c is False
            nseg = 4 if is_c else 2
            r = (4096 // nseg) * (j % nseg) + RUN * (j // nseg) + 16

            def hook(v):
                bring[par, pl.ds(r, v.shape[0]), :] = v.astype(BF16)
                b_start(j)
            return hook

        embed = CFG["embed"] and not isinstance(g, int)
        hosted = False
        for t in range(32):
            dst = (kbuf if t < 16 else vbuf).at[par, pl.ds(2 * (t % 16), 2)]
            pltpu.make_async_copy(dst, dst, sem1.at[t // 16]).wait()
            if hosted is not True:
                b_start(t, True if hosted is False else jnp.logical_not(hosted))
            if t < 16:
                kv_start(v_hbm, vbuf, g, t, sem1.at[1])
            else:
                if last is not True:
                    kv_start(k_hbm, kbuf, gn, t - 16, sem1.at[0], live=between(0, NG - 2))
                when(last, lambda: start(o1[t - 16][0], o1[t - 16][1], 1))
            if t == bwait:
                when(between(0, 0), lambda: wait(sum(q0, []), sem0.at[1]))
                when(between(1, 31), lambda: wait([(None, bring.at[sl])], sem0.at[sl]))
            hosted = False
            for cond, f in cm.get(t, ()):
                if embed and t < 31 and cond is not False and f not in short:
                    hosted = either(hosted, cond)
                    pl.when(g >= 0 if cond is True else cond)(
                        lambda f=f: f(hook_for(t + 1)))
                else:
                    when(cond, f)

    cuts = CFG["cuts"]
    for lo, hi in zip(cuts[:-1], cuts[1:]):
        if hi - lo == 1:
            body(lo, lo, lo)
        else:
            def loop_body(g, carry, lo=lo, hi=hi):
                body(g, lo, hi - 1)
                return carry
            lax.fori_loop(lo, hi, loop_body, 0)

    s1, s0, cm = {}, {}, {}
    nt = len(o1)
    for t in range(nt - D1):
        at(s1, t, o1[D1 + t])
    p0 = o0[0] + o0[1]
    last0 = nt - CFG["end0"]
    t0 = [(j * last0) // len(p0) for j in range(len(p0))]
    for t, it in zip(t0, p0):
        at(s0, t, it)
    twa, twb = 24, nt - 7
    assert t0[15] + 5 <= twa and t0[31] + 4 <= twb
    at(cm, 8, lambda: wait([(None, bring.at[1])], sem0.at[1]))
    at(cm, twa, lambda: wait(sum((d for d, _ in o0[0]), []), semx.at[0]))
    at(cm, twb, lambda: wait(sum((d for d, _ in o0[1]), []), semx.at[1]))

    def write_b():
        o_ref[:, DM:2 * DM] = out_s[1].astype(o_ref.dtype)

    if do_compute:
        at(cm, 1, a_pv(NG - 1, 0))
        at(cm, 3, a_pv(NG - 1, 1))
        at(cm, 5, a_fin(NG - 1))
        at(cm, 8, wob_mm(1, 3, 0))
        at(cm, 10, both(wob_mm(1, 3, 1), write_b))
        for t, heads in ((15, g1[0][:4]), (17, g1[0][4:]), (twa, g0[0]), (31, g1[1][:4]),
                         (33, g1[1][4:]), (39, g1[2]), (twb, g0[1]), (nt - 3, g1[3])):
            at(cm, t, woa_mm(heads))
    static_ticks(o1, s1, s0, cm)
    if do_compute:
        o_ref[:, 0:DM] = (out_s[0] + woa_dot(g1[4][0])).astype(o_ref.dtype)
    else:
        o_ref[...] = jnp.zeros(o_ref.shape, o_ref.dtype)


def _flat(x):
    c = x.shape[-1]
    if c == DH:
        return x.reshape(-1, DH)
    return x.reshape(-1, 8, c // DH, DH).transpose(0, 2, 1, 3).reshape(-1, DH)


@jax.jit
def pallas_concat_heads__sliding_block_cached__compressed_kv_cla__decode_kernel(
    A_x: jax.Array,
    A_k_cache: jax.Array,
    A_v_cache: jax.Array,
    A_wq: jax.Array,
    A_wo: jax.Array,
    B_x: jax.Array,
    B_c_kv: jax.Array,
    B_w_q: jax.Array,
    B_w_uk: jax.Array,
    B_w_uv: jax.Array,
    B_w_o: jax.Array,
):
    assert A_x.shape == (NB, 1, DM) and B_x.shape == (NB, 1, DM)
    assert A_k_cache.shape == (NB, NH, SK, DH) and B_c_kv.shape == (NB, SK, DM)
    vm = pltpu.VMEM
    out = pl.pallas_call(
        _kernel,
        out_shape=jax.ShapeDtypeStruct((NB, 2 * DM), A_x.dtype),
        in_specs=[pl.BlockSpec(memory_space=pl.ANY)] * 11,
        out_specs=pl.BlockSpec(memory_space=pltpu.VMEM),
        scratch_shapes=[
            vm((NB, DM), BF16), vm((NB, DM), BF16),
            vm((2, NH, RUN, DH), BF16), vm((2, NH, RUN, DH), BF16),
            vm((16384, DH), BF16), vm((16384, DH), BF16),
            vm((2, 4096, DH), BF16),
            vm((4, NB, 128), F32),
            vm((NH * 8, DH), F32),
            vm((NH * 8, DH), F32),
            vm((NH, RUN), F32),
            vm((NH, DH), F32), vm((NH, DH), F32),
            vm((NH, DH), F32), vm((NH, DH), F32),
            vm((NB, NH * DH), F32),
            vm((4, NH * 8, 128), F32),
            vm((NB, NH, DM), BF16),
            vm((NB, NH, CK), F32),
            vm((NB, NH, CK), BF16),
            vm((NB, NH, 128), F32),
            vm((NB, NH, 128), F32), vm((NB, NH, 128), F32),
            vm((NB, NH, DM), F32),
            vm((4, NB * NH, 128), F32),
            vm((4, NB, 8 * DH), F32),
            vm((2, NB, DM), F32),
            vm((128, 8 * DH), BF16), vm((128, 8 * DH), BF16),
            pltpu.SemaphoreType.DMA((2,)), pltpu.SemaphoreType.DMA((2,)),
            pltpu.SemaphoreType.DMA((2,)), pltpu.SemaphoreType.DMA((5,)),
        ],
        compiler_params=pltpu.CompilerParams(
            vmem_limit_bytes=48 * 1024 * 1024,
            disable_bounds_checks=not CFG["checks"],
            disable_semaphore_checks=not CFG["checks"],
        ),
        name="concat_heads_decode",
    )(
        A_x.reshape(NB, DM), B_x.reshape(NB, DM), A_k_cache, A_v_cache,
        _flat(A_wq), _flat(A_wo), _flat(B_c_kv),
        _flat(B_w_q), _flat(B_w_uk), _flat(B_w_uv), _flat(B_w_o),
    )
    return out.reshape(NB, 1, 2 * DM)
```

```python
import jax
import jax.numpy as jnp
from jax import lax
import jax.experimental.pallas as pl
import jax.experimental.pallas.tpu as pltpu

F32 = jnp.float32
BF16 = jnp.bfloat16

NB = 4
NH = 32
DH = 128
DM = 512
SK = 4096
WIN = 1024
CK = 256
NG = 32
RUN = 128
D1 = 16
NT = ((1,), (1,)), ((), ())

CFG = dict(compute=True, pre0=3, bwait=6, aoff=8, boff=8, embed=True, lat0=6,
           g1=(tuple(range(0, 32, 4)), tuple(range(1, 32, 4)), (2, 6, 10, 14), (18, 22, 26), (30,)),
           g0=((3, 7, 11, 15), (19, 23, 27, 31)), q_slots=(6, 8, 10, 12, 14, 15, 17, 19), end0=11, checks=False,
           cuts=(0, 8, 24, 32), a_slots=(1, 3, 16, 18, 20, 22, 24),
           b_slots=(6, 8, 10, 12, 14, 26, 28, 30, 31), c_slots=(0, 1, 2, 3, 5, 6))


def _mult(x, m):
    return x if isinstance(x, int) else pl.multiple_of(x, m)


def _kernel(xa_hbm, xb_hbm, k_hbm, v_hbm, wqa_hbm, woa_hbm, c_hbm, wqb_hbm, wuk_hbm,
            wuv_hbm, wob_hbm, o_ref,
            xa_buf, xb_buf, kbuf, vbuf, wqa_buf, woa_buf, bring,
            xb_s, qa_t, oa_t, sa_s, ma_s, la_s, aa_s, acca_s, qb_s, qabs_t, qabs_s, sb_s, pb_s, al_s,
            m_s, l_s, acc_s, cc_s, ctx_s, out_s, w2a_s, w2b_s,
            sem1, sem0, semx, semt):
    do_compute = CFG["compute"]
    aoff, boff = CFG["aoff"], CFG["boff"]
    bwait = CFG["bwait"]
    scale = DH ** -0.5
    w2_s = (w2a_s, w2b_s)
    row8 = lax.broadcasted_iota(jnp.int32, (8, DH), 0)
    bring_t = bring.reshape(2, 128, 32, DH)
    wqa_t = wqa_buf.reshape(64, 256, DH)
    woa_t = woa_buf.reshape(512, 32, DH)

    def start(descs, sem, prio):
        for src, dst in descs:
            pltpu.make_async_copy(src, dst, sem).start(priority=prio)

    def wait(descs, sem):
        for _, dst in descs:
            pltpu.make_async_copy(dst, dst, sem).wait()

    def at(d, t, item):
        d.setdefault(t, []).append(item)

    def both(*fs, host=0):
        def f(hook=None):
            for i, g in enumerate(fs):
                if i == host:
                    g(hook)
                else:
                    g()
        return f

    def call(hook, v):
        if hook is not None:
            hook(v)

    def tiles(view, j):
        w = view[:, 8 * j:8 * j + 8, :]
        return w.reshape(w.shape[0] * 8, DH)

    def mat(view, j0, n):
        return jnp.concatenate([tiles(view, j0 + j) for j in range(n)], axis=1)

    def when(cond, f):
        if cond is True:
            f()
        elif cond is not False:
            pl.when(cond)(f)

    def kv_start(hbm, buf, g, t, sem, live=True):
        b, sl = g >> 3, g & 7
        w0 = SK - WIN
        src, dst = hbm.at[b, pl.ds(2 * t, 2)], buf.at[g & 1, pl.ds(2 * t, 2)]
        reg = [(src.at[:, pl.ds(_mult(w0 + RUN * sl - aoff, 8), RUN)], dst)]
        if aoff == 0:
            when(live, lambda: start(reg, sem, 1))
            return
        fst = [(src.at[:, pl.ds(w0, RUN - aoff)], dst.at[:, pl.ds(aoff, RUN - aoff)])]
        if t == 0:
            fst = [(hbm.at[b, :, pl.ds(SK - aoff, aoff)], buf.at[g & 1, :, pl.ds(0, aoff)])] + fst
        if isinstance(sl, int):
            when(live, lambda: start(reg if sl else fst, sem, 1))
        else:
            pl.when(sl > 0)(lambda: start(reg, sem, 1))
            first = sl == 0
            pl.when(first if live is True else jnp.logical_and(first, live))(
                lambda: start(fst, sem, 1))

    def b_run(hbm, nseg, src_row, sl, t):
        seg, k = t % nseg, t // nseg
        ln = 4096 // nseg
        r = boff + RUN * k
        n = min(RUN, ln - r)
        out = [(hbm.at[pl.ds(_mult(src_row(seg) + r, 8), n)], bring.at[sl, pl.ds(ln * seg + r, n)])]
        if k == 0 and boff:
            out.append((hbm.at[pl.ds(_mult(src_row(seg), 8), boff)],
                        bring.at[sl, pl.ds(ln * seg, boff)]))
        return out

    def a_run(hbm, buf, r, lo, hi):
        r0, r1 = max(r - aoff, lo), (hi if r + RUN == hi else r + RUN - aoff)
        return [(hbm.at[pl.ds(r0, r1 - r0)], buf.at[pl.ds(r0, r1 - r0)])]

    def retile(sl, hb):
        def f():
            w2_s[hb & 1][...] = bring_t[sl, :, 8 * hb:8 * hb + 8, :].reshape(128, 8 * DH)
        return f

    def wq_mm(cb, hb):
        def f(hook=None):
            r = jnp.dot(xb_s[cb].astype(BF16), w2_s[hb & 1][...], preferred_element_type=F32)
            qb_s[:, 1024 * hb:1024 * hb + 1024] += r
            call(hook, r[:, 7 * DH:])
        return f

    def wuk_mm(cb, hb):
        def f(hook=None):
            for j in range(8):
                h = 8 * hb + j
                q = (qb_s[:, DH * h:DH * h + DH] * scale).astype(BF16)
                r = lax.dot_general(q, w2_s[hb & 1][:, DH * j:DH * j + DH], NT,
                                    preferred_element_type=F32)
                qabs_t[cb, 8 * h:8 * h + NB, :] = r
                if j == 0:
                    r0 = r
            call(hook, r0)
        return f

    def wuv_mm(cb, hb):
        def f(hook=None):
            for j in range(8):
                cc = cc_s[cb, pl.ds(8 * hb + j, NB, stride=NH), :].astype(BF16)
                r = jnp.dot(cc, w2_s[hb & 1][:, DH * j:DH * j + DH], preferred_element_type=F32)
                ctx_s[hb, :, DH * j:DH * j + DH] += r
            call(hook, r)
        return f

    def qabs_finish():
        for b in range(NB):
            for cb in range(4):
                qabs_s[b, :, 128 * cb:128 * cb + 128] = (
                    qabs_t[cb, pl.ds(b, NH, stride=8), :].astype(BF16))

    def c_pieces(sl):
        def cmat(b):
            return mat(bring_t.at[sl, pl.ds(32 * b, 32)], 0, 4)

        def qk(b):
            def f(hook=None):
                s = lax.dot_general(qabs_s[b], cmat(b), NT, preferred_element_type=F32)
                sb_s[b] = s
                call(hook, s[0:8, 0:DH])
            return f

        def sm(b):
            def f():
                s = sb_s[b]
                m_old = m_s[b]
                m_new = jnp.maximum(m_old, jnp.max(s, axis=-1, keepdims=True))
                alpha = jnp.exp(m_old - m_new)
                ps = [jnp.exp(s[:, 128 * j:128 * j + 128] - m_new) for j in range(CK // 128)]
                l_s[b] = alpha * l_s[b] + sum(ps[1:], ps[0])
                m_s[b] = m_new
                al_s[b] = alpha
                pb_s[b] = jnp.concatenate(ps, axis=-1).astype(BF16)
            return f

        def pv(b):
            def f(hook=None):
                r = jnp.dot(pb_s[b], cmat(b), preferred_element_type=F32)
                al = al_s[b]
                for j in range(4):
                    cols = slice(128 * j, 128 * j + 128)
                    acc_s[b, :, cols] = al * acc_s[b, :, cols] + r[:, cols]
                if hook is not None:
                    keep["v"] = r[0:8, 3 * DH:]
            return f

        keep = {}

        def late(f):
            def g(hook=None):
                f(hook)
                if hook is not None:
                    hook(keep["v"])
            return g

        return [qk(0), both(qk(1), sm(0)), both(qk(2), sm(1)), both(qk(3), sm(2)),
                late(both(sm(3), pv(0), pv(1), host=1)), late(both(pv(2), pv(3)))]

    def c_finish():
        for b in range(NB):
            cc = acc_s[b] / jnp.sum(l_s[b], axis=-1, keepdims=True)
            for cb in range(4):
                cc_s[cb, NH * b:NH * b + NH, :] = cc[:, 128 * cb:128 * cb + 128]

    def wob_mm(sl, cb, half):
        def f(hook=None):
            rs = []
            for i in range(2):
                c0 = 512 * half + 256 * i
                w = mat(bring_t.at[sl, pl.ds(c0 // 8, 32)], 0, 4)
                rs.append(jnp.dot(ctx_s[cb, :, c0:c0 + 256].astype(BF16), w,
                                  preferred_element_type=F32))
            out_s[1, 0:NB, :] += rs[0] + rs[1]
            call(hook, rs[0][:, 3 * DH:])
        return f

    def init():
        wait(x_copies[:1], semx.at[0])
        wait(x_copies[1:], semx.at[1])
        if not do_compute:
            return
        xb = xb_buf[...].astype(F32)
        for cb in range(4):
            xb_s[cb] = xb[:, 128 * cb:128 * cb + 128]
        qb_s[...] = jnp.zeros(qb_s.shape, F32)
        ctx_s[...] = jnp.zeros(ctx_s.shape, F32)
        out_s[...] = jnp.zeros(out_s.shape, F32)
        for r in (ma_s, la_s, acca_s):
            r[...] = jnp.zeros(r.shape, F32)
        m_s[...] = jnp.full(m_s.shape, -jnp.inf, F32)
        l_s[...] = jnp.zeros(l_s.shape, F32)
        acc_s[...] = jnp.zeros(acc_s.shape, F32)

    def wqa_mm(j):
        def f(hook=None):
            r = jnp.dot(xa_buf[...], mat(wqa_t, 4 * j, 4), preferred_element_type=F32) * scale
            for i in range(4):
                h = 4 * j + i
                qa_t[8 * h:8 * h + NB, :] = r[:, DH * i:DH * i + DH]
            call(hook, r[:, 0:DH])
        return f

    def a_qk(g, k):
        def f(hook=None):
            q8 = qa_t[pl.ds(64 * k + (g >> 3), 8, stride=8), :]
            s = None
            for j in range(8):
                qm = jnp.where(row8 == j, q8, 0.0).astype(BF16)
                sj = lax.dot_general(qm, kbuf[g & 1, 8 * k + j], NT, preferred_element_type=F32)
                s = sj if s is None else s + sj
                if j == 0:
                    call(hook, sj)
            sa_s[8 * k:8 * k + 8, :] = s
        return f

    def a_sm(g):
        def f():
            first = (g & 7) == 0
            s = sa_s[...]
            m_old = jnp.where(first, -jnp.inf, ma_s[...])
            m_new = jnp.maximum(m_old, jnp.max(s, axis=-1, keepdims=True))
            alpha = jnp.exp(m_old - m_new)
            p = jnp.exp(s - m_new)
            la_s[...] = jnp.where(first, p, alpha * la_s[...] + p)
            ma_s[...] = m_new
            aa_s[...] = alpha
            sa_s[...] = p
        return f

    def a_pv(g, k):
        def f(hook=None):
            first = (g & 7) == 0
            for r0 in (16 * k, 16 * k + 8):
                rows = slice(r0, r0 + 8)
                p = sa_s[rows, :].astype(BF16)
                o = None
                for j in range(8):
                    oj = jnp.dot(p, vbuf[g & 1, r0 + j], preferred_element_type=F32)
                    o = oj if o is None else jnp.where(row8 == j, oj, o)
                    if r0 % 16 == 0 and j == 4:
                        call(hook, oj)
                acca_s[rows, :] = jnp.where(first, o, aa_s[rows, :] * acca_s[rows, :] + o)
        return f

    def a_fin(g):
        def f():
            o = acca_s[...] / jnp.sum(la_s[...], axis=-1, keepdims=True)
            oa_t[pl.ds(g >> 3, NH, stride=8), :] = o
        return f

    def woa_dot(h):
        o = oa_t[8 * h:8 * h + NB, :].astype(BF16)
        return jnp.dot(o, mat(woa_t.at[pl.ds(16 * h, 16)], 0, 4), preferred_element_type=F32)

    def woa_mm(heads):
        def f():
            r = woa_dot(heads[0])
            for h in heads[1:]:
                r = r + woa_dot(h)
            out_s[0, 0:NB, :] += r
        return f

    def static_ticks(waits, starts1, starts0, comp):
        for t, (descs, sem) in enumerate(waits):
            wait(descs, sem)
            for d, s in starts0.get(t, ()):
                start(d, s, 0)
            for d, s in starts1.get(t, ()):
                start(d, s, 1)
            for f in comp.get(t, ()):
                f()

    pre0 = CFG["pre0"]
    x_copies = [(xa_hbm, xa_buf), (xb_hbm, xb_buf)]
    qr = [[a_run(wqa_hbm, wqa_buf, 2048 * r + RUN * s, 0, 16384) for r in range(8)]
          for s in range(16)]
    q1 = [qr[s][r] + qr[s][r + 1] for s in range(11) for r in (0, 2, 4, 6)]
    q0 = [qr[s][r] for s in range(11, 16) for r in range(8)]
    for j in range(D1):
        start(q1[j], sem1.at[1], 1)
        if j < pre0:
            start(q0[j], sem0.at[1], 0)
    start(x_copies[:1], semx.at[0], 0)
    start(x_copies[1:], semx.at[1], 0)
    s1, s0, cm = {}, {}, {}
    for t, d in enumerate(q1[D1:]):
        at(s1, t, (d, sem1.at[1]))
    for t in range(D1):
        at(cm, len(q1) - D1 + t, lambda t=t: kv_start(k_hbm, kbuf, 0, t, sem1.at[0]))
    n0 = len(q0) - pre0
    for j in range(n0):
        at(s0, (j * len(q1)) // n0, (q0[pre0 + j], sem0.at[1]))
    at(cm, 4, init)
    static_ticks([(d, sem1.at[1]) for d in q1], s1, s0, cm)

    def head_runs(h):
        return [a_run(woa_hbm, woa_buf, 512 * h + RUN * k, 512 * h, 512 * h + 512)
                for k in range(4)]

    def group1(heads):
        hr = [head_runs(h) for h in heads]
        runs = [hr[i][k] for k in range(4) for i in range(len(heads))]
        return [runs[i] + runs[i + 1] for i in range(0, len(runs), 2)]

    g1, g0 = CFG["g1"], CFG["g0"]
    assert sorted(sum(g1 + g0, ())) == list(range(NH))
    o1 = [(d, semt.at[i]) for i, hs in enumerate(g1) for d in group1(hs)]
    o0 = [[(head_runs(h)[k], semx.at[i]) for k in range(4) for h in hs]
          for i, hs in enumerate(g0)]

    b_slots = CFG["b_slots"]
    a_slots = CFG["a_slots"]

    def body(g, g_lo, g_hi):
        def between(lo, hi):
            if lo <= g_lo and g_hi <= hi:
                return True
            if hi < g_lo or g_hi < lo:
                return False
            if lo <= g_lo:
                return g <= hi
            if g_hi <= hi:
                return g >= lo
            return jnp.logical_and(g >= lo, g <= hi)

        def either(x, y):
            if x is True or y is True:
                return True
            if x is False or y is False:
                return y if x is False else x
            return jnp.logical_or(x, y)

        par = g & 1
        iw = g & 3
        w_stage = [(between(0, 3), wqb_hbm), (between(4, 7), wuk_hbm),
                   (between(24, 27), wuv_hbm), (between(28, 31), wob_hbm)]
        is_c = between(8, 23)
        ic = (g - 8) & 15
        last = between(NG - 1, NG - 1)
        gn = g + 1 if last is False else (g + 1) & (NG - 1)

        sl, cb = 1 - par, (g + 3) & 3
        cm = {}
        short = [qabs_finish, c_finish]
        if do_compute:
            w3 = either(between(1, 8), between(25, 28))
            for k, hb in ((0, 0), (1, 1), (4, 2), (5, 3)):
                short.append(retile(sl, hb))
                at(cm, b_slots[k], (w3, short[-1]))
            for k, hb in ((2, 0), (6, 2)):
                at(cm, b_slots[k], (between(1, 4), both(wq_mm(cb, hb), wq_mm(cb, hb + 1))))
                at(cm, b_slots[k], (between(25, 28), both(wuv_mm(cb, hb), wuv_mm(cb, hb + 1))))
            for k, hb in ((2, 0), (3, 1), (6, 2), (7, 3)):
                at(cm, b_slots[k], (between(5, 8), wuk_mm(cb, hb)))
            at(cm, b_slots[8], (between(8, 8), qabs_finish))
            for k, f in zip(CFG["c_slots"], c_pieces(sl)):
                at(cm, b_slots[k], (between(9, 24), f))
            at(cm, b_slots[8], (between(24, 24), c_finish))
            for k, half in ((3, 0), (7, 1)):
                at(cm, b_slots[k], (between(29, 31), wob_mm(sl, cb, half)))
            for k, t in enumerate(CFG["q_slots"]):
                at(cm, t, (between(0, 0), wqa_mm(k)))
            for k in range(2):
                at(cm, a_slots[k], (between(1, 31), a_pv(g - 1, k)))
            fin = either(either(between(8, 8), between(16, 16)), between(24, 24))
            short += [a_fin(g - 1), a_sm(g)]
            at(cm, a_slots[1] + 2, (fin, short[-2]))
            for k in range(4):
                at(cm, a_slots[2 + k], (True, a_qk(g, k)))
            at(cm, a_slots[6], (True, short[-1]))

        def also(x, y):
            if x is False or y is False:
                return False
            if x is True or y is True:
                return y if x is True else x
            return jnp.logical_and(x, y)

        def b_start(j, live=True):
            for cond, hbm in w_stage:
                when(also(cond, live), lambda hbm=hbm: start(
                    b_run(hbm, 2, lambda s: 4096 * iw + 2048 * s, par, j), sem0.at[par], 0))
            when(also(is_c, live), lambda: start(
                b_run(c_hbm, 4, lambda s: 16384 * s + 1024 * ic, par, j), sem0.at[par], 0))

        def hook_for(j):
            assert is_c is True or is_c is False
            nseg = 4 if is_c else 2
            r = (4096 // nseg) * (j % nseg) + RUN * (j // nseg) + 16

            def hook(v):
                bring[par, pl.ds(r, v.shape[0]), :] = v.astype(BF16)
                b_start(j)
            return hook

        embed = CFG["embed"] and not isinstance(g, int)
        hosted = False
        for t in range(32):
            dst = (kbuf if t < 16 else vbuf).at[par, pl.ds(2 * (t % 16), 2)]
            pltpu.make_async_copy(dst, dst, sem1.at[t // 16]).wait()
            if hosted is not True:
                b_start(t, True if hosted is False else jnp.logical_not(hosted))
            if t < 16:
                kv_start(v_hbm, vbuf, g, t, sem1.at[1])
            else:
                if last is not True:
                    kv_start(k_hbm, kbuf, gn, t - 16, sem1.at[0], live=between(0, NG - 2))
                when(last, lambda: start(o1[t - 16][0], o1[t - 16][1], 1))
            if t == bwait:
                when(between(0, 0), lambda: wait(sum(q0, []), sem0.at[1]))
                when(between(1, 31), lambda: wait([(None, bring.at[sl])], sem0.at[sl]))
            hosted = False
            for cond, f in cm.get(t, ()):
                if embed and t < 31 and cond is not False and f not in short:
                    hosted = either(hosted, cond)
                    pl.when(g >= 0 if cond is True else cond)(
                        lambda f=f: f(hook_for(t + 1)))
                else:
                    when(cond, f)

    cuts = CFG["cuts"]
    for lo, hi in zip(cuts[:-1], cuts[1:]):
        if hi - lo == 1:
            body(lo, lo, lo)
        else:
            def loop_body(g, carry, lo=lo, hi=hi):
                body(g, lo, hi - 1)
                return carry
            lax.fori_loop(lo, hi, loop_body, 0)

    s1, s0, cm = {}, {}, {}
    nt = len(o1)
    for t in range(nt - D1):
        at(s1, t, o1[D1 + t])
    p0 = o0[0] + o0[1]
    last0 = nt - CFG["end0"]
    t0 = [(j * last0) // len(p0) for j in range(len(p0))]
    for t, it in zip(t0, p0):
        at(s0, t, it)
    n00 = len(o0[0])
    twa, twb = t0[n00 - 1] + 6, t0[-1] + CFG["lat0"]
    at(cm, 8, lambda: wait([(None, bring.at[1])], sem0.at[1]))
    at(cm, twa, lambda: wait(sum((d for d, _ in o0[0]), []), semx.at[0]))
    at(cm, twb, lambda: wait(sum((d for d, _ in o0[1]), []), semx.at[1]))

    def write_b():
        o_ref[:, DM:2 * DM] = out_s[1, 0:NB, :].astype(o_ref.dtype)

    if do_compute:
        at(cm, 1, a_pv(NG - 1, 0))
        at(cm, 3, a_pv(NG - 1, 1))
        at(cm, 5, a_fin(NG - 1))
        at(cm, 8, wob_mm(1, 3, 0))
        at(cm, 10, both(wob_mm(1, 3, 1), write_b))
        at(cm, twa, woa_mm(g0[0]))
        at(cm, twb, woa_mm(g0[1]))
        t = -1
        for heads in g1[:-1]:
            t += 2 * len(heads)
            for i in range(0, len(heads), 4):
                at(cm, t + i // 2, woa_mm(heads[i:i + 4]))
    static_ticks(o1, s1, s0, cm)
    if do_compute:
        o_ref[:, 0:DM] = (out_s[0, 0:NB, :] + sum(woa_dot(h) for h in g1[-1])).astype(o_ref.dtype)
    else:
        o_ref[...] = jnp.zeros(o_ref.shape, o_ref.dtype)


def _flat(x):
    c = x.shape[-1]
    if c == DH:
        return x.reshape(-1, DH)
    return x.reshape(-1, 8, c // DH, DH).transpose(0, 2, 1, 3).reshape(-1, DH)


@jax.jit
def pallas_concat_heads__sliding_block_cached__compressed_kv_cla__decode_kernel(
    A_x: jax.Array,
    A_k_cache: jax.Array,
    A_v_cache: jax.Array,
    A_wq: jax.Array,
    A_wo: jax.Array,
    B_x: jax.Array,
    B_c_kv: jax.Array,
    B_w_q: jax.Array,
    B_w_uk: jax.Array,
    B_w_uv: jax.Array,
    B_w_o: jax.Array,
):
    assert A_x.shape == (NB, 1, DM) and B_x.shape == (NB, 1, DM)
    assert A_k_cache.shape == (NB, NH, SK, DH) and B_c_kv.shape == (NB, SK, DM)
    vm = pltpu.VMEM
    out = pl.pallas_call(
        _kernel,
        out_shape=jax.ShapeDtypeStruct((NB, 2 * DM), A_x.dtype),
        in_specs=[pl.BlockSpec(memory_space=pl.ANY)] * 11,
        out_specs=pl.BlockSpec(memory_space=pltpu.VMEM),
        scratch_shapes=[
            vm((NB, DM), BF16), vm((NB, DM), BF16),
            vm((2, NH, RUN, DH), BF16), vm((2, NH, RUN, DH), BF16),
            vm((16384, DH), BF16), vm((16384, DH), BF16),
            vm((2, 4096, DH), BF16),
            vm((4, NB, 128), F32),
            vm((NH * 8, DH), F32),
            vm((NH * 8, DH), F32),
            vm((NH, RUN), F32),
            vm((NH, DH), F32), vm((NH, DH), F32),
            vm((NH, DH), F32), vm((NH, DH), F32),
            vm((NB, NH * DH), F32),
            vm((4, NH * 8, 128), F32),
            vm((NB, NH, DM), BF16),
            vm((NB, NH, CK), F32),
            vm((NB, NH, CK), BF16),
            vm((NB, NH, 128), F32),
            vm((NB, NH, 128), F32), vm((NB, NH, 128), F32),
            vm((NB, NH, DM), F32),
            vm((4, NB * NH, 128), F32),
            vm((4, NB, 8 * DH), F32),
            vm((2, 8, DM), F32),
            vm((128, 8 * DH), BF16), vm((128, 8 * DH), BF16),
            pltpu.SemaphoreType.DMA((2,)), pltpu.SemaphoreType.DMA((2,)),
            pltpu.SemaphoreType.DMA((2,)), pltpu.SemaphoreType.DMA((len(CFG["g1"]),)),
        ],
        compiler_params=pltpu.CompilerParams(
            vmem_limit_bytes=48 * 1024 * 1024,
            disable_bounds_checks=not CFG["checks"],
            disable_semaphore_checks=not CFG["checks"],
        ),
        name="concat_heads_decode",
    )(
        A_x.reshape(NB, DM), B_x.reshape(NB, DM), A_k_cache, A_v_cache,
        _flat(A_wq), _flat(A_wo), _flat(B_c_kv),
        _flat(B_w_q), _flat(B_w_uk), _flat(B_w_uv), _flat(B_w_o),
    )
    return out.reshape(NB, 1, 2 * DM)
```

```python
import jax
import jax.numpy as jnp
from jax import lax
import jax.experimental.pallas as pl
import jax.experimental.pallas.tpu as pltpu

F32 = jnp.float32
BF16 = jnp.bfloat16

NB = 4
NH = 32
DH = 128
DM = 512
SK = 4096
WIN = 1024
CK = 256
NG = 32
RUN = 128
RT = 16
D1 = 16
NT = ((1,), (1,)), ((), ())

CFG = dict(compute=True, pre0=3, bwait=6, aoff=1, boff=1, embed=True, lat0=6,
           g1=(tuple(range(0, 32, 4)), tuple(range(1, 32, 4)), (2, 6, 10, 14), (18, 22, 26), (30,)),
           g0=((3, 7, 11, 15), (19, 23, 27, 31)), q_slots=(6, 8, 10, 12, 14, 15, 17, 19), end0=11, checks=False,
           cuts=(0, 8, 24, 32), a_slots=(1, 3, 16, 18, 20, 22, 24),
           b_slots=(6, 8, 10, 12, 14, 26, 28, 30, 31), c_slots=(0, 1, 2, 3, 5, 6))


def _mult(x, m):
    return x if isinstance(x, int) else pl.multiple_of(x, m)


def _kernel(xa_hbm, xb_hbm, k_hbm, v_hbm, wqa_hbm, woa_hbm, c_hbm, wqb_hbm, wuk_hbm,
            wuv_hbm, wob_hbm, o_ref,
            xa_buf, xb_buf, kbuf, vbuf, wqa_buf, woa_buf, bring,
            xb_s, qa_t, oa_t, sa_s, ma_s, la_s, aa_s, acca_s, qb_s, qabs_t, qabs_s, sb_s, pb_s, al_s,
            m_s, l_s, acc_s, cc_s, ctx_s, out_s, w2a_s, w2b_s,
            sem1, sem0, semx, semt):
    do_compute = CFG["compute"]
    aoff, boff = CFG["aoff"], CFG["boff"]
    bwait = CFG["bwait"]
    scale = DH ** -0.5
    w2_s = (w2a_s, w2b_s)
    row8 = lax.broadcasted_iota(jnp.int32, (8, DH), 0)

    def start(descs, sem, prio):
        for src, dst in descs:
            pltpu.make_async_copy(src, dst, sem).start(priority=prio)

    def wait(descs, sem):
        for _, dst in descs:
            pltpu.make_async_copy(dst, dst, sem).wait()

    def at(d, t, item):
        d.setdefault(t, []).append(item)

    def both(*fs, host=0):
        def f(hook=None):
            for i, g in enumerate(fs):
                if i == host:
                    g(hook)
                else:
                    g()
        return f

    def call(hook, v):
        if hook is not None:
            hook(v)

    def mat(w, ncol, j0, n):
        w = w.reshape(w.shape[0] // ncol, ncol, 8, DH)
        cols = [w[:, j0 + j].reshape(w.shape[0] * 8, DH) for j in range(n)]
        return jnp.concatenate(cols, axis=1)

    def when(cond, f):
        if cond is True:
            f()
        elif cond is not False:
            pl.when(cond)(f)

    def kv_start(hbm, buf, g, t, sem, live=True):
        b, sl = g >> 3, g & 7
        ko = 8 * aoff
        w0 = SK - WIN
        src, dst = hbm.at[b, pl.ds(2 * t, 2)], buf.at[g & 1, pl.ds(2 * t, 2)]
        reg = [(src.at[:, pl.ds(_mult(w0 + RUN * sl - ko, 8), RUN)], dst)]
        if ko == 0:
            when(live, lambda: start(reg, sem, 1))
            return
        fst = [(src.at[:, pl.ds(w0, RUN - ko)], dst.at[:, pl.ds(ko, RUN - ko)])]
        if t == 0:
            fst = [(hbm.at[b, :, pl.ds(SK - ko, ko)], buf.at[g & 1, :, pl.ds(0, ko)])] + fst
        if isinstance(sl, int):
            when(live, lambda: start(reg if sl else fst, sem, 1))
        else:
            pl.when(sl > 0)(lambda: start(reg, sem, 1))
            first = sl == 0
            pl.when(first if live is True else jnp.logical_and(first, live))(
                lambda: start(fst, sem, 1))

    def b_run(hbm, nseg, src, sl, t):
        seg, k = t % nseg, t // nseg
        ln = 512 // nseg
        r = boff + RT * k
        n = min(RT, ln - r)
        out = [(hbm.at[pl.ds(src(seg) + r, n)], bring.at[sl, pl.ds(ln * seg + r, n)])]
        if k == 0 and boff:
            out.append((hbm.at[pl.ds(src(seg), boff)], bring.at[sl, pl.ds(ln * seg, boff)]))
        return out

    def a_run(hbm, buf, r, lo, hi):
        r0, r1 = max(r - aoff, lo), (hi if r + RT == hi else r + RT - aoff)
        return [(hbm.at[pl.ds(r0, r1 - r0)], buf.at[pl.ds(r0, r1 - r0)])]

    def retile(sl, hb):
        def f():
            w = bring[sl].reshape(128, 4, 8, DH)[:, hb]
            w2_s[hb & 1][...] = w.reshape(128, 8 * DH)
        return f

    def wq_mm(cb, hb):
        def f(hook=None):
            r = jnp.dot(xb_s[cb].astype(BF16), w2_s[hb & 1][...], preferred_element_type=F32)
            qb_s[:, 1024 * hb:1024 * hb + 1024] += r
            call(hook, r[:, 7 * DH:])
        return f

    def wuk_mm(cb, hb):
        def f(hook=None):
            for j in range(8):
                h = 8 * hb + j
                q = (qb_s[:, DH * h:DH * h + DH] * scale).astype(BF16)
                r = lax.dot_general(q, w2_s[hb & 1][:, DH * j:DH * j + DH], NT,
                                    preferred_element_type=F32)
                qabs_t[cb, 8 * h:8 * h + NB, :] = r
                if j == 0:
                    r0 = r
            call(hook, r0)
        return f

    def wuv_mm(cb, hb):
        def f(hook=None):
            for j in range(8):
                cc = cc_s[cb, pl.ds(8 * hb + j, NB, stride=NH), :].astype(BF16)
                r = jnp.dot(cc, w2_s[hb & 1][:, DH * j:DH * j + DH], preferred_element_type=F32)
                ctx_s[hb, :, DH * j:DH * j + DH] += r
            call(hook, r)
        return f

    def qabs_finish():
        for b in range(NB):
            for cb in range(4):
                qabs_s[b, :, 128 * cb:128 * cb + 128] = (
                    qabs_t[cb, pl.ds(b, NH, stride=8), :].astype(BF16))

    def c_pieces(sl):
        def cmat(b):
            return mat(bring[sl, 128 * b:128 * b + 128], 4, 0, 4)

        def qk(b):
            def f(hook=None):
                s = lax.dot_general(qabs_s[b], cmat(b), NT, preferred_element_type=F32)
                sb_s[b] = s
                call(hook, s[0:8, 0:DH])
            return f

        def sm(b):
            def f():
                s = sb_s[b]
                m_old = m_s[b]
                m_new = jnp.maximum(m_old, jnp.max(s, axis=-1, keepdims=True))
                alpha = jnp.exp(m_old - m_new)
                ps = [jnp.exp(s[:, 128 * j:128 * j + 128] - m_new) for j in range(CK // 128)]
                l_s[b] = alpha * l_s[b] + sum(ps[1:], ps[0])
                m_s[b] = m_new
                al_s[b] = alpha
                pb_s[b] = jnp.concatenate(ps, axis=-1).astype(BF16)
            return f

        def pv(b):
            def f(hook=None):
                r = jnp.dot(pb_s[b], cmat(b), preferred_element_type=F32)
                al = al_s[b]
                for j in range(4):
                    cols = slice(128 * j, 128 * j + 128)
                    acc_s[b, :, cols] = al * acc_s[b, :, cols] + r[:, cols]
                if hook is not None:
                    keep["v"] = r[0:8, 3 * DH:]
            return f

        keep = {}

        def late(f):
            def g(hook=None):
                f(hook)
                if hook is not None:
                    hook(keep["v"])
            return g

        return [qk(0), both(qk(1), sm(0)), both(qk(2), sm(1)), both(qk(3), sm(2)),
                late(both(sm(3), pv(0), pv(1), host=1)), late(both(pv(2), pv(3)))]

    def c_finish():
        for b in range(NB):
            cc = acc_s[b] / jnp.sum(l_s[b], axis=-1, keepdims=True)
            for cb in range(4):
                cc_s[cb, NH * b:NH * b + NH, :] = cc[:, 128 * cb:128 * cb + 128]

    def wob_mm(sl, cb, half):
        def f(hook=None):
            rs = []
            for i in range(2):
                c0 = 512 * half + 256 * i
                w = mat(bring[sl, c0 // 2:c0 // 2 + 128], 4, 0, 4)
                rs.append(jnp.dot(ctx_s[cb, :, c0:c0 + 256].astype(BF16), w,
                                  preferred_element_type=F32))
            out_s[1, 0:NB, :] += rs[0] + rs[1]
            call(hook, rs[0][:, 3 * DH:])
        return f

    def init():
        wait(x_copies[:1], semx.at[0])
        wait(x_copies[1:], semx.at[1])
        if not do_compute:
            return
        xb = xb_buf[...].astype(F32)
        for cb in range(4):
            xb_s[cb] = xb[:, 128 * cb:128 * cb + 128]
        qb_s[...] = jnp.zeros(qb_s.shape, F32)
        ctx_s[...] = jnp.zeros(ctx_s.shape, F32)
        out_s[...] = jnp.zeros(out_s.shape, F32)
        for r in (ma_s, la_s, acca_s):
            r[...] = jnp.zeros(r.shape, F32)
        m_s[...] = jnp.full(m_s.shape, -jnp.inf, F32)
        l_s[...] = jnp.zeros(l_s.shape, F32)
        acc_s[...] = jnp.zeros(acc_s.shape, F32)

    def wqa_mm(j):
        def f(hook=None):
            r = jnp.dot(xa_buf[...], mat(wqa_buf[...], 32, 4 * j, 4), preferred_element_type=F32) * scale
            for i in range(4):
                h = 4 * j + i
                qa_t[8 * h:8 * h + NB, :] = r[:, DH * i:DH * i + DH]
            call(hook, r[:, 0:DH])
        return f

    def a_qk(g, k):
        def f(hook=None):
            q8 = qa_t[pl.ds(64 * k + (g >> 3), 8, stride=8), :]
            s = None
            for j in range(8):
                qm = jnp.where(row8 == j, q8, 0.0).astype(BF16)
                sj = lax.dot_general(qm, kbuf[g & 1, 8 * k + j], NT, preferred_element_type=F32)
                s = sj if s is None else s + sj
                if j == 0:
                    call(hook, sj)
            sa_s[8 * k:8 * k + 8, :] = s
        return f

    def a_sm(g):
        def f():
            first = (g & 7) == 0
            s = sa_s[...]
            m_old = jnp.where(first, -jnp.inf, ma_s[...])
            m_new = jnp.maximum(m_old, jnp.max(s, axis=-1, keepdims=True))
            alpha = jnp.exp(m_old - m_new)
            p = jnp.exp(s - m_new)
            la_s[...] = jnp.where(first, p, alpha * la_s[...] + p)
            ma_s[...] = m_new
            aa_s[...] = alpha
            sa_s[...] = p
        return f

    def a_pv(g, k):
        def f(hook=None):
            first = (g & 7) == 0
            for r0 in (16 * k, 16 * k + 8):
                rows = slice(r0, r0 + 8)
                p = sa_s[rows, :].astype(BF16)
                o = None
                for j in range(8):
                    oj = jnp.dot(p, vbuf[g & 1, r0 + j], preferred_element_type=F32)
                    o = oj if o is None else jnp.where(row8 == j, oj, o)
                    if r0 % 16 == 0 and j == 4:
                        call(hook, oj)
                acca_s[rows, :] = jnp.where(first, o, aa_s[rows, :] * acca_s[rows, :] + o)
        return f

    def a_fin(g):
        def f():
            o = acca_s[...] / jnp.sum(la_s[...], axis=-1, keepdims=True)
            oa_t[pl.ds(g >> 3, NH, stride=8), :] = o
        return f

    def woa_dot(h):
        o = oa_t[8 * h:8 * h + NB, :].astype(BF16)
        return jnp.dot(o, mat(woa_buf[64 * h:64 * h + 64], 4, 0, 4), preferred_element_type=F32)

    def woa_mm(heads):
        def f():
            r = woa_dot(heads[0])
            for h in heads[1:]:
                r = r + woa_dot(h)
            out_s[0, 0:NB, :] += r
        return f

    def static_ticks(waits, starts1, starts0, comp):
        for t, (descs, sem) in enumerate(waits):
            wait(descs, sem)
            for d, s in starts0.get(t, ()):
                start(d, s, 0)
            for d, s in starts1.get(t, ()):
                start(d, s, 1)
            for f in comp.get(t, ()):
                f()

    pre0 = CFG["pre0"]
    x_copies = [(xa_hbm, xa_buf), (xb_hbm, xb_buf)]
    qr = [[a_run(wqa_hbm, wqa_buf, 256 * r + RT * s, 0, 2048) for r in range(8)]
          for s in range(16)]
    q1 = [qr[s][r] + qr[s][r + 1] for s in range(11) for r in (0, 2, 4, 6)]
    q0 = [qr[s][r] for s in range(11, 16) for r in range(8)]
    for j in range(D1):
        start(q1[j], sem1.at[1], 1)
        if j < pre0:
            start(q0[j], sem0.at[1], 0)
    start(x_copies[:1], semx.at[0], 0)
    start(x_copies[1:], semx.at[1], 0)
    s1, s0, cm = {}, {}, {}
    for t, d in enumerate(q1[D1:]):
        at(s1, t, (d, sem1.at[1]))
    for t in range(D1):
        at(cm, len(q1) - D1 + t, lambda t=t: kv_start(k_hbm, kbuf, 0, t, sem1.at[0]))
    n0 = len(q0) - pre0
    for j in range(n0):
        at(s0, (j * len(q1)) // n0, (q0[pre0 + j], sem0.at[1]))
    at(cm, 4, init)
    static_ticks([(d, sem1.at[1]) for d in q1], s1, s0, cm)

    def head_runs(h):
        return [a_run(woa_hbm, woa_buf, 64 * h + RT * k, 64 * h, 64 * h + 64)
                for k in range(4)]

    def group1(heads):
        hr = [head_runs(h) for h in heads]
        runs = [hr[i][k] for k in range(4) for i in range(len(heads))]
        return [runs[i] + runs[i + 1] for i in range(0, len(runs), 2)]

    g1, g0 = CFG["g1"], CFG["g0"]
    assert sorted(sum(g1 + g0, ())) == list(range(NH))
    o1 = [(d, semt.at[i]) for i, hs in enumerate(g1) for d in group1(hs)]
    o0 = [[(head_runs(h)[k], semx.at[i]) for k in range(4) for h in hs]
          for i, hs in enumerate(g0)]

    b_slots = CFG["b_slots"]
    a_slots = CFG["a_slots"]

    def body(g, g_lo, g_hi):
        def between(lo, hi):
            if lo <= g_lo and g_hi <= hi:
                return True
            if hi < g_lo or g_hi < lo:
                return False
            if lo <= g_lo:
                return g <= hi
            if g_hi <= hi:
                return g >= lo
            return jnp.logical_and(g >= lo, g <= hi)

        def either(x, y):
            if x is True or y is True:
                return True
            if x is False or y is False:
                return y if x is False else x
            return jnp.logical_or(x, y)

        par = g & 1
        iw = g & 3
        w_stage = [(between(0, 3), wqb_hbm), (between(4, 7), wuk_hbm),
                   (between(24, 27), wuv_hbm), (between(28, 31), wob_hbm)]
        is_c = between(8, 23)
        ic = (g - 8) & 15
        last = between(NG - 1, NG - 1)
        gn = g + 1 if last is False else (g + 1) & (NG - 1)

        sl, cb = 1 - par, (g + 3) & 3
        cm = {}
        short = [qabs_finish, c_finish]
        if do_compute:
            w3 = either(between(1, 8), between(25, 28))
            for k, hb in ((0, 0), (1, 1), (4, 2), (5, 3)):
                short.append(retile(sl, hb))
                at(cm, b_slots[k], (w3, short[-1]))
            for k, hb in ((2, 0), (6, 2)):
                at(cm, b_slots[k], (between(1, 4), both(wq_mm(cb, hb), wq_mm(cb, hb + 1))))
                at(cm, b_slots[k], (between(25, 28), both(wuv_mm(cb, hb), wuv_mm(cb, hb + 1))))
            for k, hb in ((2, 0), (3, 1), (6, 2), (7, 3)):
                at(cm, b_slots[k], (between(5, 8), wuk_mm(cb, hb)))
            at(cm, b_slots[8], (between(8, 8), qabs_finish))
            for k, f in zip(CFG["c_slots"], c_pieces(sl)):
                at(cm, b_slots[k], (between(9, 24), f))
            at(cm, b_slots[8], (between(24, 24), c_finish))
            for k, half in ((3, 0), (7, 1)):
                at(cm, b_slots[k], (between(29, 31), wob_mm(sl, cb, half)))
            for k, t in enumerate(CFG["q_slots"]):
                at(cm, t, (between(0, 0), wqa_mm(k)))
            for k in range(2):
                at(cm, a_slots[k], (between(1, 31), a_pv(g - 1, k)))
            fin = either(either(between(8, 8), between(16, 16)), between(24, 24))
            short += [a_fin(g - 1), a_sm(g)]
            at(cm, a_slots[1] + 2, (fin, short[-2]))
            for k in range(4):
                at(cm, a_slots[2 + k], (True, a_qk(g, k)))
            at(cm, a_slots[6], (True, short[-1]))

        def also(x, y):
            if x is False or y is False:
                return False
            if x is True or y is True:
                return y if x is True else x
            return jnp.logical_and(x, y)

        def b_start(j, live=True):
            for cond, hbm in w_stage:
                when(also(cond, live), lambda hbm=hbm: start(
                    b_run(hbm, 2, lambda s: 512 * iw + 256 * s, par, j), sem0.at[par], 0))
            when(also(is_c, live), lambda: start(
                b_run(c_hbm, 4, lambda s: 2048 * s + 128 * ic, par, j), sem0.at[par], 0))

        def hook_for(j):
            assert is_c is True or is_c is False
            nseg = 4 if is_c else 2
            r = (512 // nseg) * (j % nseg) + RT * (j // nseg) + boff

            def hook(v):
                bring[par, r, 0:v.shape[0], :] = v.astype(BF16)
                b_start(j)
            return hook

        embed = CFG["embed"] and not isinstance(g, int)
        hosted = False
        for t in range(32):
            dst = (kbuf if t < 16 else vbuf).at[par, pl.ds(2 * (t % 16), 2)]
            pltpu.make_async_copy(dst, dst, sem1.at[t // 16]).wait()
            if hosted is not True:
                b_start(t, True if hosted is False else jnp.logical_not(hosted))
            if t < 16:
                kv_start(v_hbm, vbuf, g, t, sem1.at[1])
            else:
                if last is not True:
                    kv_start(k_hbm, kbuf, gn, t - 16, sem1.at[0], live=between(0, NG - 2))
                when(last, lambda: start(o1[t - 16][0], o1[t - 16][1], 1))
            if t == bwait:
                when(between(0, 0), lambda: wait(sum(q0, []), sem0.at[1]))
                when(between(1, 31), lambda: wait([(None, bring.at[sl])], sem0.at[sl]))
            hosted = False
            for cond, f in cm.get(t, ()):
                if embed and t < 31 and cond is not False and f not in short:
                    hosted = either(hosted, cond)
                    pl.when(g >= 0 if cond is True else cond)(
                        lambda f=f: f(hook_for(t + 1)))
                else:
                    when(cond, f)

    cuts = CFG["cuts"]
    for lo, hi in zip(cuts[:-1], cuts[1:]):
        if hi - lo == 1:
            body(lo, lo, lo)
        else:
            def loop_body(g, carry, lo=lo, hi=hi):
                body(g, lo, hi - 1)
                return carry
            lax.fori_loop(lo, hi, loop_body, 0)

    s1, s0, cm = {}, {}, {}
    nt = len(o1)
    for t in range(nt - D1):
        at(s1, t, o1[D1 + t])
    p0 = o0[0] + o0[1]
    last0 = nt - CFG["end0"]
    t0 = [(j * last0) // len(p0) for j in range(len(p0))]
    for t, it in zip(t0, p0):
        at(s0, t, it)
    n00 = len(o0[0])
    twa, twb = t0[n00 - 1] + 6, t0[-1] + CFG["lat0"]
    at(cm, 8, lambda: wait([(None, bring.at[1])], sem0.at[1]))
    at(cm, twa, lambda: wait(sum((d for d, _ in o0[0]), []), semx.at[0]))
    at(cm, twb, lambda: wait(sum((d for d, _ in o0[1]), []), semx.at[1]))

    def write_b():
        o_ref[:, DM:2 * DM] = out_s[1, 0:NB, :].astype(o_ref.dtype)

    if do_compute:
        at(cm, 1, a_pv(NG - 1, 0))
        at(cm, 3, a_pv(NG - 1, 1))
        at(cm, 5, a_fin(NG - 1))
        at(cm, 8, wob_mm(1, 3, 0))
        at(cm, 10, both(wob_mm(1, 3, 1), write_b))
        at(cm, twa, woa_mm(g0[0]))
        at(cm, twb, woa_mm(g0[1]))
        t = -1
        for heads in g1[:-1]:
            t += 2 * len(heads)
            for i in range(0, len(heads), 4):
                at(cm, t + i // 2, woa_mm(heads[i:i + 4]))
    static_ticks(o1, s1, s0, cm)
    if do_compute:
        o_ref[:, 0:DM] = (out_s[0, 0:NB, :] + sum(woa_dot(h) for h in g1[-1])).astype(o_ref.dtype)
    else:
        o_ref[...] = jnp.zeros(o_ref.shape, o_ref.dtype)


def _tiles(x):
    c = x.shape[-1]
    return x.reshape(-1, 8, c // DH, DH).transpose(0, 2, 1, 3).reshape(-1, 8, DH)


@jax.jit
def pallas_concat_heads__sliding_block_cached__compressed_kv_cla__decode_kernel(
    A_x: jax.Array,
    A_k_cache: jax.Array,
    A_v_cache: jax.Array,
    A_wq: jax.Array,
    A_wo: jax.Array,
    B_x: jax.Array,
    B_c_kv: jax.Array,
    B_w_q: jax.Array,
    B_w_uk: jax.Array,
    B_w_uv: jax.Array,
    B_w_o: jax.Array,
):
    assert A_x.shape == (NB, 1, DM) and B_x.shape == (NB, 1, DM)
    assert A_k_cache.shape == (NB, NH, SK, DH) and B_c_kv.shape == (NB, SK, DM)
    vm = pltpu.VMEM
    out = pl.pallas_call(
        _kernel,
        out_shape=jax.ShapeDtypeStruct((NB, 2 * DM), A_x.dtype),
        in_specs=[pl.BlockSpec(memory_space=pl.ANY)] * 11,
        out_specs=pl.BlockSpec(memory_space=pltpu.VMEM),
        scratch_shapes=[
            vm((NB, DM), BF16), vm((NB, DM), BF16),
            vm((2, NH, RUN, DH), BF16), vm((2, NH, RUN, DH), BF16),
            vm((2048, 8, DH), BF16), vm((2048, 8, DH), BF16),
            vm((2, 512, 8, DH), BF16),
            vm((4, NB, 128), F32),
            vm((NH * 8, DH), F32),
            vm((NH * 8, DH), F32),
            vm((NH, RUN), F32),
            vm((NH, DH), F32), vm((NH, DH), F32),
            vm((NH, DH), F32), vm((NH, DH), F32),
            vm((NB, NH * DH), F32),
            vm((4, NH * 8, 128), F32),
            vm((NB, NH, DM), BF16),
            vm((NB, NH, CK), F32),
            vm((NB, NH, CK), BF16),
            vm((NB, NH, 128), F32),
            vm((NB, NH, 128), F32), vm((NB, NH, 128), F32),
            vm((NB, NH, DM), F32),
            vm((4, NB * NH, 128), F32),
            vm((4, NB, 8 * DH), F32),
            vm((2, 8, DM), F32),
            vm((128, 8 * DH), BF16), vm((128, 8 * DH), BF16),
            pltpu.SemaphoreType.DMA((2,)), pltpu.SemaphoreType.DMA((2,)),
            pltpu.SemaphoreType.DMA((2,)), pltpu.SemaphoreType.DMA((len(CFG["g1"]),)),
        ],
        compiler_params=pltpu.CompilerParams(
            vmem_limit_bytes=48 * 1024 * 1024,
            disable_bounds_checks=not CFG["checks"],
            disable_semaphore_checks=not CFG["checks"],
        ),
        name="concat_heads_decode",
    )(
        A_x.reshape(NB, DM), B_x.reshape(NB, DM), A_k_cache, A_v_cache,
        _tiles(A_wq), _tiles(A_wo), _tiles(B_c_kv),
        _tiles(B_w_q), _tiles(B_w_uk), _tiles(B_w_uv), _tiles(B_w_o),
    )
    return out.reshape(NB, 1, 2 * DM)
```

```python
import jax
import jax.numpy as jnp
from jax import lax
import jax.experimental.pallas as pl
import jax.experimental.pallas.tpu as pltpu

F32 = jnp.float32
BF16 = jnp.bfloat16

NB = 4
NH = 32
DH = 128
DM = 512
SK = 4096
WIN = 1024
CK = 256
NG = 32
RUN = 128
RT = 16
D1 = 16
NT = ((1,), (1,)), ((), ())

CFG = dict(compute=True, pre0=3, bwait=6, aoff=1, boff=1, embed=True, olead=(6, 6),
           opat=("110" * 10 + "11", "011" * 10 + "11", "011" * 10 + "11", "011" * 5 + "0",
                 "11011011", "1111", "1111"),
           q_slots=(6, 8, 10, 12, 14, 15, 17, 19), checks=False,
           cuts=(0, 8, 24, 32), a_slots=(1, 3, 16, 18, 20, 22, 24),
           b_slots=(6, 8, 10, 12, 14, 26, 28, 30, 31), c_slots=(0, 1, 2, 3, 5, 6))


def _mult(x, m):
    return x if isinstance(x, int) else pl.multiple_of(x, m)


def _kernel(xa_hbm, xb_hbm, k_hbm, v_hbm, wqa_hbm, woa_hbm, c_hbm, wqb_hbm, wuk_hbm,
            wuv_hbm, wob_hbm, o_ref,
            xa_buf, xb_buf, kbuf, vbuf, wqa_buf, woa_buf, bring,
            xb_s, qa_t, oa_t, sa_s, ma_s, la_s, aa_s, acca_s, qb_s, qabs_t, qabs_s, sb_s, pb_s, al_s,
            m_s, l_s, acc_s, cc_s, ctx_s, out_s, oq_s, w2a_s, w2b_s,
            sem1, sem0, semx, semt):
    do_compute = CFG["compute"]
    aoff, boff = CFG["aoff"], CFG["boff"]
    bwait = CFG["bwait"]
    scale = DH ** -0.5
    w2_s = (w2a_s, w2b_s)
    row8 = lax.broadcasted_iota(jnp.int32, (8, DH), 0)

    def start(descs, sem, prio):
        for src, dst in descs:
            pltpu.make_async_copy(src, dst, sem).start(priority=prio)

    def wait(descs, sem):
        for _, dst in descs:
            pltpu.make_async_copy(dst, dst, sem).wait()

    def at(d, t, item):
        d.setdefault(t, []).append(item)

    def both(*fs, host=0):
        def f(hook=None):
            for i, g in enumerate(fs):
                if i == host:
                    g(hook)
                else:
                    g()
        return f

    def call(hook, v):
        if hook is not None:
            hook(v)

    def mat(w, ncol, j0, n):
        w = w.reshape(w.shape[0] // ncol, ncol, 8, DH)
        cols = [w[:, j0 + j].reshape(w.shape[0] * 8, DH) for j in range(n)]
        return jnp.concatenate(cols, axis=1)

    def when(cond, f):
        if cond is True:
            f()
        elif cond is not False:
            pl.when(cond)(f)

    def kv_start(hbm, buf, g, t, sem, live=True):
        b, sl = g >> 3, g & 7
        ko = 8 * aoff
        w0 = SK - WIN
        src, dst = hbm.at[b, pl.ds(2 * t, 2)], buf.at[g & 1, pl.ds(2 * t, 2)]
        reg = [(src.at[:, pl.ds(_mult(w0 + RUN * sl - ko, 8), RUN)], dst)]
        if ko == 0:
            when(live, lambda: start(reg, sem, 1))
            return
        fst = [(src.at[:, pl.ds(w0, RUN - ko)], dst.at[:, pl.ds(ko, RUN - ko)])]
        if t == 0:
            fst = [(hbm.at[b, :, pl.ds(SK - ko, ko)], buf.at[g & 1, :, pl.ds(0, ko)])] + fst
        if isinstance(sl, int):
            when(live, lambda: start(reg if sl else fst, sem, 1))
        else:
            pl.when(sl > 0)(lambda: start(reg, sem, 1))
            first = sl == 0
            pl.when(first if live is True else jnp.logical_and(first, live))(
                lambda: start(fst, sem, 1))

    def b_run(hbm, nseg, src, sl, t):
        seg, k = t % nseg, t // nseg
        ln = 512 // nseg
        r = boff + RT * k
        n = min(RT, ln - r)
        out = [(hbm.at[pl.ds(src(seg) + r, n)], bring.at[sl, pl.ds(ln * seg + r, n)])]
        if k == 0 and boff:
            out.append((hbm.at[pl.ds(src(seg), boff)], bring.at[sl, pl.ds(ln * seg, boff)]))
        return out

    def a_run(hbm, buf, r, lo, hi):
        r0, r1 = max(r - aoff, lo), (hi if r + RT == hi else r + RT - aoff)
        return [(hbm.at[pl.ds(r0, r1 - r0)], buf.at[pl.ds(r0, r1 - r0)])]

    def retile(sl, hb):
        def f():
            w = bring[sl].reshape(128, 4, 8, DH)[:, hb]
            w2_s[hb & 1][...] = w.reshape(128, 8 * DH)
        return f

    def wq_mm(cb, hb):
        def f(hook=None):
            r = jnp.dot(xb_s[cb].astype(BF16), w2_s[hb & 1][...], preferred_element_type=F32)
            qb_s[:, 1024 * hb:1024 * hb + 1024] += r
            call(hook, r[:, 7 * DH:])
        return f

    def wuk_mm(cb, hb):
        def f(hook=None):
            for j in range(8):
                h = 8 * hb + j
                q = (qb_s[:, DH * h:DH * h + DH] * scale).astype(BF16)
                r = lax.dot_general(q, w2_s[hb & 1][:, DH * j:DH * j + DH], NT,
                                    preferred_element_type=F32)
                qabs_t[cb, 8 * h:8 * h + NB, :] = r
                if j == 0:
                    r0 = r
            call(hook, r0)
        return f

    def wuv_mm(cb, hb):
        def f(hook=None):
            for j in range(8):
                cc = cc_s[cb, pl.ds(8 * hb + j, NB, stride=NH), :].astype(BF16)
                r = jnp.dot(cc, w2_s[hb & 1][:, DH * j:DH * j + DH], preferred_element_type=F32)
                ctx_s[hb, :, DH * j:DH * j + DH] += r
            call(hook, r)
        return f

    def qabs_finish():
        for b in range(NB):
            for cb in range(4):
                qabs_s[b, :, 128 * cb:128 * cb + 128] = (
                    qabs_t[cb, pl.ds(b, NH, stride=8), :].astype(BF16))

    def c_pieces(sl):
        def cmat(b):
            return mat(bring[sl, 128 * b:128 * b + 128], 4, 0, 4)

        def qk(b):
            def f(hook=None):
                s = lax.dot_general(qabs_s[b], cmat(b), NT, preferred_element_type=F32)
                sb_s[b] = s
                call(hook, s[0:8, 0:DH])
            return f

        def sm(b):
            def f():
                s = sb_s[b]
                m_old = m_s[b]
                m_new = jnp.maximum(m_old, jnp.max(s, axis=-1, keepdims=True))
                alpha = jnp.exp(m_old - m_new)
                ps = [jnp.exp(s[:, 128 * j:128 * j + 128] - m_new) for j in range(CK // 128)]
                l_s[b] = alpha * l_s[b] + sum(ps[1:], ps[0])
                m_s[b] = m_new
                al_s[b] = alpha
                pb_s[b] = jnp.concatenate(ps, axis=-1).astype(BF16)
            return f

        def pv(b):
            def f(hook=None):
                r = jnp.dot(pb_s[b], cmat(b), preferred_element_type=F32)
                al = al_s[b]
                for j in range(4):
                    cols = slice(128 * j, 128 * j + 128)
                    acc_s[b, :, cols] = al * acc_s[b, :, cols] + r[:, cols]
                if hook is not None:
                    keep["v"] = r[0:8, 3 * DH:]
            return f

        keep = {}

        def late(f):
            def g(hook=None):
                f(hook)
                if hook is not None:
                    hook(keep["v"])
            return g

        return [qk(0), both(qk(1), sm(0)), both(qk(2), sm(1)), both(qk(3), sm(2)),
                late(both(sm(3), pv(0), pv(1), host=1)), late(both(pv(2), pv(3)))]

    def c_finish():
        for b in range(NB):
            cc = acc_s[b] / jnp.sum(l_s[b], axis=-1, keepdims=True)
            for cb in range(4):
                cc_s[cb, NH * b:NH * b + NH, :] = cc[:, 128 * cb:128 * cb + 128]

    def wob_mm(sl, cb, half):
        def f(hook=None):
            rs = []
            for i in range(2):
                c0 = 512 * half + 256 * i
                w = mat(bring[sl, c0 // 2:c0 // 2 + 128], 4, 0, 4)
                rs.append(jnp.dot(ctx_s[cb, :, c0:c0 + 256].astype(BF16), w,
                                  preferred_element_type=F32))
            out_s[1, 0:NB, :] += rs[0] + rs[1]
            call(hook, rs[0][:, 3 * DH:])
        return f

    def init():
        wait(x_copies[:1], semx.at[0])
        wait(x_copies[1:], semx.at[1])
        if not do_compute:
            return
        xb = xb_buf[...].astype(F32)
        for cb in range(4):
            xb_s[cb] = xb[:, 128 * cb:128 * cb + 128]
        qb_s[...] = jnp.zeros(qb_s.shape, F32)
        ctx_s[...] = jnp.zeros(ctx_s.shape, F32)
        out_s[...] = jnp.zeros(out_s.shape, F32)
        for r in (ma_s, la_s, acca_s):
            r[...] = jnp.zeros(r.shape, F32)
        m_s[...] = jnp.full(m_s.shape, -jnp.inf, F32)
        l_s[...] = jnp.zeros(l_s.shape, F32)
        acc_s[...] = jnp.zeros(acc_s.shape, F32)

    def wqa_mm(j):
        def f(hook=None):
            r = jnp.dot(xa_buf[...], mat(wqa_buf[...], 32, 4 * j, 4), preferred_element_type=F32) * scale
            for i in range(4):
                h = 4 * j + i
                qa_t[8 * h:8 * h + NB, :] = r[:, DH * i:DH * i + DH]
            call(hook, r[:, 0:DH])
        return f

    def a_qk(g, k):
        def f(hook=None):
            q8 = qa_t[pl.ds(64 * k + (g >> 3), 8, stride=8), :]
            s = None
            for j in range(8):
                qm = jnp.where(row8 == j, q8, 0.0).astype(BF16)
                sj = lax.dot_general(qm, kbuf[g & 1, 8 * k + j], NT, preferred_element_type=F32)
                s = sj if s is None else s + sj
                if j == 0:
                    call(hook, sj)
            sa_s[8 * k:8 * k + 8, :] = s
        return f

    def a_sm(g):
        def f():
            first = (g & 7) == 0
            s = sa_s[...]
            m_old = jnp.where(first, -jnp.inf, ma_s[...])
            m_new = jnp.maximum(m_old, jnp.max(s, axis=-1, keepdims=True))
            alpha = jnp.exp(m_old - m_new)
            p = jnp.exp(s - m_new)
            la_s[...] = jnp.where(first, p, alpha * la_s[...] + p)
            ma_s[...] = m_new
            aa_s[...] = alpha
            sa_s[...] = p
        return f

    def a_pv(g, k):
        def f(hook=None):
            first = (g & 7) == 0
            for r0 in (16 * k, 16 * k + 8):
                rows = slice(r0, r0 + 8)
                p = sa_s[rows, :].astype(BF16)
                o = None
                for j in range(8):
                    oj = jnp.dot(p, vbuf[g & 1, r0 + j], preferred_element_type=F32)
                    o = oj if o is None else jnp.where(row8 == j, oj, o)
                    if r0 % 16 == 0 and j == 4:
                        call(hook, oj)
                acca_s[rows, :] = jnp.where(first, o, aa_s[rows, :] * acca_s[rows, :] + o)
        return f

    def a_fin(g):
        def f():
            o = acca_s[...] / jnp.sum(la_s[...], axis=-1, keepdims=True)
            oa_t[pl.ds(g >> 3, NH, stride=8), :] = o
        return f

    def woa_dot(h):
        o = oa_t[8 * h:8 * h + NB, :].astype(BF16)
        return jnp.dot(o, mat(woa_buf[64 * h:64 * h + 64], 4, 0, 4), preferred_element_type=F32)

    quads = [(hs, k) for k in (3, 2, 1, 0) for hs in ((0, 4, 8, 12), (16, 20, 24, 28))]

    def quad_lhs():
        for n, (hs, k) in enumerate(quads):
            oq_s[n, 0:NB, :] = jnp.concatenate(
                [oa_t[8 * h:8 * h + NB, 32 * k:32 * k + 32] for h in hs], axis=1)

    def quad_dot(n):
        hs, k = quads[n]
        w = jnp.concatenate([woa_buf[64 * h + RT * k:64 * h + RT * k + RT] for h in hs], axis=0)
        return jnp.dot(oq_s[n, 0:NB, :].astype(BF16), mat(w, 4, 0, 4), preferred_element_type=F32)

    def woa_mm(dot, items):
        def f():
            r = dot(items[0])
            for i in items[1:]:
                r = r + dot(i)
            out_s[0, 0:NB, :] += r
        return f

    def static_ticks(waits, starts1, starts0, comp):
        for t, (descs, sem) in enumerate(waits):
            wait(descs, sem)
            for d, s in starts0.get(t, ()):
                start(d, s, 0)
            for d, s in starts1.get(t, ()):
                start(d, s, 1)
            for f in comp.get(t, ()):
                f()

    pre0 = CFG["pre0"]
    x_copies = [(xa_hbm, xa_buf), (xb_hbm, xb_buf)]
    qr = [[a_run(wqa_hbm, wqa_buf, 256 * r + RT * s, 0, 2048) for r in range(8)]
          for s in range(16)]
    q1 = [qr[s][r] + qr[s][r + 1] for s in range(11) for r in (0, 2, 4, 6)]
    q0 = [qr[s][r] for s in range(11, 16) for r in range(8)]
    for j in range(D1):
        start(q1[j], sem1.at[1], 1)
        if j < pre0:
            start(q0[j], sem0.at[1], 0)
    start(x_copies[:1], semx.at[0], 0)
    start(x_copies[1:], semx.at[1], 0)
    s1, s0, cm = {}, {}, {}
    for t, d in enumerate(q1[D1:]):
        at(s1, t, (d, sem1.at[1]))
    for t in range(D1):
        at(cm, len(q1) - D1 + t, lambda t=t: kv_start(k_hbm, kbuf, 0, t, sem1.at[0]))
    n0 = len(q0) - pre0
    for j in range(n0):
        at(s0, (j * len(q1)) // n0, (q0[pre0 + j], sem0.at[1]))
    at(cm, 4, init)
    static_ticks([(d, sem1.at[1]) for d in q1], s1, s0, cm)

    oruns = [a_run(woa_hbm, woa_buf, 256 * r + RT * k, 256 * r, 256 * r + 256)
             for k in range(15, -1, -1) for r in range(8)]
    o1, o0, o_end = [], [], []
    for i, pat in enumerate(CFG["opat"]):
        lo = [oruns.pop(0) for _ in pat]
        ones = [r for r, c in zip(lo, pat) if c == "1"]
        o0.append([(len(o1) + pat[:n].count("1") // 2, r)
                   for n, (r, c) in enumerate(zip(lo, pat)) if c == "0"])
        o1 += [(ones[n] + ones[n + 1], semt.at[0, i]) for n in range(0, len(ones), 2)]
        o_end.append(len(o1) - 1)
    assert not oruns

    b_slots = CFG["b_slots"]
    a_slots = CFG["a_slots"]

    def body(g, g_lo, g_hi):
        def between(lo, hi):
            if lo <= g_lo and g_hi <= hi:
                return True
            if hi < g_lo or g_hi < lo:
                return False
            if lo <= g_lo:
                return g <= hi
            if g_hi <= hi:
                return g >= lo
            return jnp.logical_and(g >= lo, g <= hi)

        def either(x, y):
            if x is True or y is True:
                return True
            if x is False or y is False:
                return y if x is False else x
            return jnp.logical_or(x, y)

        par = g & 1
        iw = g & 3
        w_stage = [(between(0, 3), wqb_hbm), (between(4, 7), wuk_hbm),
                   (between(24, 27), wuv_hbm), (between(28, 31), wob_hbm)]
        is_c = between(8, 23)
        ic = (g - 8) & 15
        last = between(NG - 1, NG - 1)
        gn = g + 1 if last is False else (g + 1) & (NG - 1)

        sl, cb = 1 - par, (g + 3) & 3
        cm = {}
        short = [qabs_finish, c_finish]
        if do_compute:
            w3 = either(between(1, 8), between(25, 28))
            for k, hb in ((0, 0), (1, 1), (4, 2), (5, 3)):
                short.append(retile(sl, hb))
                at(cm, b_slots[k], (w3, short[-1]))
            for k, hb in ((2, 0), (6, 2)):
                at(cm, b_slots[k], (between(1, 4), both(wq_mm(cb, hb), wq_mm(cb, hb + 1))))
                at(cm, b_slots[k], (between(25, 28), both(wuv_mm(cb, hb), wuv_mm(cb, hb + 1))))
            for k, hb in ((2, 0), (3, 1), (6, 2), (7, 3)):
                at(cm, b_slots[k], (between(5, 8), wuk_mm(cb, hb)))
            at(cm, b_slots[8], (between(8, 8), qabs_finish))
            for k, f in zip(CFG["c_slots"], c_pieces(sl)):
                at(cm, b_slots[k], (between(9, 24), f))
            at(cm, b_slots[8], (between(24, 24), c_finish))
            for k, half in ((3, 0), (7, 1)):
                at(cm, b_slots[k], (between(29, 31), wob_mm(sl, cb, half)))
            for k, t in enumerate(CFG["q_slots"]):
                at(cm, t, (between(0, 0), wqa_mm(k)))
            for k in range(2):
                at(cm, a_slots[k], (between(1, 31), a_pv(g - 1, k)))
            fin = either(either(between(8, 8), between(16, 16)), between(24, 24))
            short += [a_fin(g - 1), a_sm(g)]
            at(cm, a_slots[1] + 2, (fin, short[-2]))
            for k in range(4):
                at(cm, a_slots[2 + k], (True, a_qk(g, k)))
            at(cm, a_slots[6], (True, short[-1]))

        def also(x, y):
            if x is False or y is False:
                return False
            if x is True or y is True:
                return y if x is True else x
            return jnp.logical_and(x, y)

        def b_start(j, live=True):
            for cond, hbm in w_stage:
                when(also(cond, live), lambda hbm=hbm: start(
                    b_run(hbm, 2, lambda s: 512 * iw + 256 * s, par, j), sem0.at[par], 0))
            when(also(is_c, live), lambda: start(
                b_run(c_hbm, 4, lambda s: 2048 * s + 128 * ic, par, j), sem0.at[par], 0))

        def hook_for(j):
            assert is_c is True or is_c is False
            nseg = 4 if is_c else 2
            r = (512 // nseg) * (j % nseg) + RT * (j // nseg) + boff

            def hook(v):
                bring[par, r, 0:v.shape[0], :] = v.astype(BF16)
                b_start(j)
            return hook

        embed = CFG["embed"] and not isinstance(g, int)
        hosted = False
        for t in range(32):
            dst = (kbuf if t < 16 else vbuf).at[par, pl.ds(2 * (t % 16), 2)]
            pltpu.make_async_copy(dst, dst, sem1.at[t // 16]).wait()
            if hosted is not True:
                b_start(t, True if hosted is False else jnp.logical_not(hosted))
            if t < 16:
                kv_start(v_hbm, vbuf, g, t, sem1.at[1])
            else:
                if last is not True:
                    kv_start(k_hbm, kbuf, gn, t - 16, sem1.at[0], live=between(0, NG - 2))
                when(last, lambda: start(o1[t - 16][0], o1[t - 16][1], 1))
            if t == bwait:
                when(between(0, 0), lambda: wait(sum(q0, []), sem0.at[1]))
                when(between(1, 31), lambda: wait([(None, bring.at[sl])], sem0.at[sl]))
            hosted = False
            for cond, f in cm.get(t, ()):
                if embed and t < 31 and cond is not False and f not in short:
                    hosted = either(hosted, cond)
                    pl.when(g >= 0 if cond is True else cond)(
                        lambda f=f: f(hook_for(t + 1)))
                else:
                    when(cond, f)

    cuts = CFG["cuts"]
    for lo, hi in zip(cuts[:-1], cuts[1:]):
        if hi - lo == 1:
            body(lo, lo, lo)
        else:
            def loop_body(g, carry, lo=lo, hi=hi):
                body(g, lo, hi - 1)
                return carry
            lax.fori_loop(lo, hi, loop_body, 0)

    s1, s0, cm = {}, {}, {}
    nt = len(o1)
    for t in range(nt - D1):
        at(s1, t, o1[D1 + t])
    la, lb = CFG["olead"]
    for i, grp in enumerate(o0):
        for p, r in grp:
            at(s0, max(0, p - (la + ((lb - la) * p) // nt)), (r, semt.at[1, i]))
        at(cm, o_end[i], lambda i=i, grp=grp: wait(sum((r for _, r in grp), []), semt.at[1, i]))
    at(cm, 7, lambda: wait([(None, bring.at[1])], sem0.at[1]))

    def write_b():
        o_ref[:, DM:2 * DM] = out_s[1, 0:NB, :].astype(o_ref.dtype)

    if do_compute:
        at(cm, 1, a_pv(NG - 1, 0))
        at(cm, 3, a_pv(NG - 1, 1))
        at(cm, 5, a_fin(NG - 1))
        at(cm, 7, wob_mm(1, 3, 0))
        at(cm, 15, both(wob_mm(1, 3, 1), write_b))
        at(cm, 17, quad_lhs)
        for i in range(3):
            at(cm, o_end[i], woa_mm(woa_dot, tuple(range(3 - i, 16, 4))))
            at(cm, o_end[i] + 2, woa_mm(woa_dot, tuple(range(19 - i, 32, 4))))
        n = 0
        for i, pat in list(enumerate(CFG["opat"]))[3:-1]:
            at(cm, o_end[i], woa_mm(quad_dot, tuple(range(n, n + len(pat) // 4))))
            n += len(pat) // 4
    static_ticks(o1, s1, s0, cm)
    if do_compute:
        r = out_s[0, 0:NB, :]
        for i in range(n, 8):
            r = r + quad_dot(i)
        o_ref[:, 0:DM] = r.astype(o_ref.dtype)
    else:
        o_ref[...] = jnp.zeros(o_ref.shape, o_ref.dtype)


def _tiles(x):
    c = x.shape[-1]
    return x.reshape(-1, 8, c // DH, DH).transpose(0, 2, 1, 3).reshape(-1, 8, DH)


@jax.jit
def pallas_concat_heads__sliding_block_cached__compressed_kv_cla__decode_kernel(
    A_x: jax.Array,
    A_k_cache: jax.Array,
    A_v_cache: jax.Array,
    A_wq: jax.Array,
    A_wo: jax.Array,
    B_x: jax.Array,
    B_c_kv: jax.Array,
    B_w_q: jax.Array,
    B_w_uk: jax.Array,
    B_w_uv: jax.Array,
    B_w_o: jax.Array,
):
    assert A_x.shape == (NB, 1, DM) and B_x.shape == (NB, 1, DM)
    assert A_k_cache.shape == (NB, NH, SK, DH) and B_c_kv.shape == (NB, SK, DM)
    vm = pltpu.VMEM
    out = pl.pallas_call(
        _kernel,
        out_shape=jax.ShapeDtypeStruct((NB, 2 * DM), A_x.dtype),
        in_specs=[pl.BlockSpec(memory_space=pl.ANY)] * 11,
        out_specs=pl.BlockSpec(memory_space=pltpu.VMEM),
        scratch_shapes=[
            vm((NB, DM), BF16), vm((NB, DM), BF16),
            vm((2, NH, RUN, DH), BF16), vm((2, NH, RUN, DH), BF16),
            vm((2048, 8, DH), BF16), vm((2048, 8, DH), BF16),
            vm((2, 512, 8, DH), BF16),
            vm((4, NB, 128), F32),
            vm((NH * 8, DH), F32),
            vm((NH * 8, DH), F32),
            vm((NH, RUN), F32),
            vm((NH, DH), F32), vm((NH, DH), F32),
            vm((NH, DH), F32), vm((NH, DH), F32),
            vm((NB, NH * DH), F32),
            vm((4, NH * 8, 128), F32),
            vm((NB, NH, DM), BF16),
            vm((NB, NH, CK), F32),
            vm((NB, NH, CK), BF16),
            vm((NB, NH, 128), F32),
            vm((NB, NH, 128), F32), vm((NB, NH, 128), F32),
            vm((NB, NH, DM), F32),
            vm((4, NB * NH, 128), F32),
            vm((4, NB, 8 * DH), F32),
            vm((2, 8, DM), F32),
            vm((8, 8, DH), F32),
            vm((128, 8 * DH), BF16), vm((128, 8 * DH), BF16),
            pltpu.SemaphoreType.DMA((2,)), pltpu.SemaphoreType.DMA((2,)),
            pltpu.SemaphoreType.DMA((2,)), pltpu.SemaphoreType.DMA((2, len(CFG["opat"]))),
        ],
        compiler_params=pltpu.CompilerParams(
            vmem_limit_bytes=48 * 1024 * 1024,
            disable_bounds_checks=not CFG["checks"],
            disable_semaphore_checks=not CFG["checks"],
        ),
        name="concat_heads_decode",
    )(
        A_x.reshape(NB, DM), B_x.reshape(NB, DM), A_k_cache, A_v_cache,
        _tiles(A_wq), _tiles(A_wo), _tiles(B_c_kv),
        _tiles(B_w_q), _tiles(B_w_uk), _tiles(B_w_uv), _tiles(B_w_o),
    )
    return out.reshape(NB, 1, 2 * DM)
```

```python
import jax
import jax.numpy as jnp
from jax import lax
import jax.experimental.pallas as pl
import jax.experimental.pallas.tpu as pltpu

F32 = jnp.float32
BF16 = jnp.bfloat16

NB = 4
NH = 32
DH = 128
DM = 512
SK = 4096
WIN = 1024
CK = 256
NG = 32
RUN = 128
RT = 16
D1 = 16
NT = ((1,), (1,)), ((), ())

CFG = dict(compute=True, pre0=6, bwait=6, aoff=1, boff=1, embed=True,
           worder=(1, 2, 4, 3, 7, 8, 6, 5, 13, 14, 0, 15, 11, 12, 10, 9), corder=(0, 1, 2, 4, 3, 7, 5, 6),
           qorder=(1, 2, 4, 3, 7, 8, 6, 5, 13, 14, 0, 15, 11, 12, 10, 9), qord=True, olead=(6, 6),
           opat=("110" * 10 + "11", "011" * 10 + "11", "011" * 10 + "11", "011" * 5 + "0",
                 "11011011", "1111", "1111"),
           q_slots=(6, 8, 10, 12, 14, 15, 17, 19), checks=False,
           cuts=(0, 8, 24, 32), a_slots=(1, 3, 16, 18, 20, 22, 24),
           b_slots=(6, 8, 10, 12, 14, 26, 28, 30, 31), c_slots=(0, 1, 2, 3, 5, 6))


def _mult(x, m):
    return x if isinstance(x, int) else pl.multiple_of(x, m)


def _kernel(xa_hbm, xb_hbm, k_hbm, v_hbm, wqa_hbm, woa_hbm, c_hbm, wqb_hbm, wuk_hbm,
            wuv_hbm, wob_hbm, o_ref,
            xa_buf, xb_buf, kbuf, vbuf, wqa_buf, woa_buf, bring,
            xb_s, qa_t, oa_t, sa_s, ma_s, la_s, aa_s, acca_s, qb_s, qabs_t, qabs_s, sb_s, pb_s, al_s,
            m_s, l_s, acc_s, cc_s, ctx_s, out_s, oq_s, w2a_s, w2b_s,
            sem1, sem0, semx, semt):
    do_compute = CFG["compute"]
    aoff, boff = CFG["aoff"], CFG["boff"]
    bwait = CFG["bwait"]
    scale = DH ** -0.5
    w2_s = (w2a_s, w2b_s)
    row8 = lax.broadcasted_iota(jnp.int32, (8, DH), 0)

    def start(descs, sem, prio):
        for src, dst in descs:
            pltpu.make_async_copy(src, dst, sem).start(priority=prio)

    def wait(descs, sem):
        for _, dst in descs:
            pltpu.make_async_copy(dst, dst, sem).wait()

    def at(d, t, item):
        d.setdefault(t, []).append(item)

    def both(*fs, host=0):
        def f(hook=None):
            for i, g in enumerate(fs):
                if i == host:
                    g(hook)
                else:
                    g()
        return f

    def call(hook, v):
        if hook is not None:
            hook(v)

    def mat(w, ncol, j0, n):
        w = w.reshape(w.shape[0] // ncol, ncol, 8, DH)
        cols = [w[:, j0 + j].reshape(w.shape[0] * 8, DH) for j in range(n)]
        return jnp.concatenate(cols, axis=1)

    def when(cond, f):
        if cond is True:
            f()
        elif cond is not False:
            pl.when(cond)(f)

    def kv_start(hbm, buf, g, t, sem, live=True):
        b, sl = g >> 3, g & 7
        ko = 8 * aoff
        w0 = SK - WIN
        src, dst = hbm.at[b, pl.ds(2 * t, 2)], buf.at[g & 1, pl.ds(2 * t, 2)]
        reg = [(src.at[:, pl.ds(_mult(w0 + RUN * sl - ko, 8), RUN)], dst)]
        if ko == 0:
            when(live, lambda: start(reg, sem, 1))
            return
        fst = [(src.at[:, pl.ds(w0, RUN - ko)], dst.at[:, pl.ds(ko, RUN - ko)])]
        if t == 0:
            fst = [(hbm.at[b, :, pl.ds(SK - ko, ko)], buf.at[g & 1, :, pl.ds(0, ko)])] + fst
        if isinstance(sl, int):
            when(live, lambda: start(reg if sl else fst, sem, 1))
        else:
            pl.when(sl > 0)(lambda: start(reg, sem, 1))
            first = sl == 0
            pl.when(first if live is True else jnp.logical_and(first, live))(
                lambda: start(fst, sem, 1))

    def b_order(nseg):
        return CFG["worder"] if nseg == 2 else CFG["corder"]

    def b_run(hbm, nseg, src, sl, t):
        seg, k = t % nseg, b_order(nseg)[t // nseg]
        ln = 512 // nseg
        r = boff + RT * k
        n = min(RT, ln - r)
        out = [(hbm.at[pl.ds(src(seg) + r, n)], bring.at[sl, pl.ds(ln * seg + r, n)])]
        if k == 0 and boff:
            out.append((hbm.at[pl.ds(src(seg), boff)], bring.at[sl, pl.ds(ln * seg, boff)]))
        return out

    def a_run(hbm, buf, r, lo, hi):
        r0, r1 = max(r - aoff, lo), (hi if r + RT == hi else r + RT - aoff)
        return [(hbm.at[pl.ds(r0, r1 - r0)], buf.at[pl.ds(r0, r1 - r0)])]

    def retile(sl, hb):
        def f():
            w = bring[sl].reshape(128, 4, 8, DH)[:, hb]
            w2_s[hb & 1][...] = w.reshape(128, 8 * DH)
        return f

    def wq_mm(cb, hb):
        def f(hook=None):
            r = jnp.dot(xb_s[cb].astype(BF16), w2_s[hb & 1][...], preferred_element_type=F32)
            qb_s[:, 1024 * hb:1024 * hb + 1024] += r
            call(hook, r[:, 7 * DH:])
        return f

    def wuk_mm(cb, hb):
        def f(hook=None):
            for j in range(8):
                h = 8 * hb + j
                q = (qb_s[:, DH * h:DH * h + DH] * scale).astype(BF16)
                r = lax.dot_general(q, w2_s[hb & 1][:, DH * j:DH * j + DH], NT,
                                    preferred_element_type=F32)
                qabs_t[cb, 8 * h:8 * h + NB, :] = r
                if j == 0:
                    r0 = r
            call(hook, r0)
        return f

    def wuv_mm(cb, hb):
        def f(hook=None):
            for j in range(8):
                cc = cc_s[cb, pl.ds(8 * hb + j, NB, stride=NH), :].astype(BF16)
                r = jnp.dot(cc, w2_s[hb & 1][:, DH * j:DH * j + DH], preferred_element_type=F32)
                ctx_s[hb, :, DH * j:DH * j + DH] += r
            call(hook, r)
        return f

    def qabs_finish():
        for b in range(NB):
            for cb in range(4):
                qabs_s[b, :, 128 * cb:128 * cb + 128] = (
                    qabs_t[cb, pl.ds(b, NH, stride=8), :].astype(BF16))

    def c_pieces(sl):
        def cmat(b):
            return mat(bring[sl, 128 * b:128 * b + 128], 4, 0, 4)

        def qk(b):
            def f(hook=None):
                s = lax.dot_general(qabs_s[b], cmat(b), NT, preferred_element_type=F32)
                sb_s[b] = s
                call(hook, s[0:8, 0:DH])
            return f

        def sm(b):
            def f():
                s = sb_s[b]
                m_old = m_s[b]
                m_new = jnp.maximum(m_old, jnp.max(s, axis=-1, keepdims=True))
                alpha = jnp.exp(m_old - m_new)
                ps = [jnp.exp(s[:, 128 * j:128 * j + 128] - m_new) for j in range(CK // 128)]
                l_s[b] = alpha * l_s[b] + sum(ps[1:], ps[0])
                m_s[b] = m_new
                al_s[b] = alpha
                pb_s[b] = jnp.concatenate(ps, axis=-1).astype(BF16)
            return f

        def pv(b):
            def f(hook=None):
                r = jnp.dot(pb_s[b], cmat(b), preferred_element_type=F32)
                al = al_s[b]
                for j in range(4):
                    cols = slice(128 * j, 128 * j + 128)
                    acc_s[b, :, cols] = al * acc_s[b, :, cols] + r[:, cols]
                if hook is not None:
                    keep["v"] = r[0:8, 3 * DH:]
            return f

        keep = {}

        def late(f):
            def g(hook=None):
                f(hook)
                if hook is not None:
                    hook(keep["v"])
            return g

        return [qk(0), both(qk(1), sm(0)), both(qk(2), sm(1)), both(qk(3), sm(2)),
                late(both(sm(3), pv(0), pv(1), host=1)), late(both(pv(2), pv(3)))]

    def c_finish():
        for b in range(NB):
            cc = acc_s[b] / jnp.sum(l_s[b], axis=-1, keepdims=True)
            for cb in range(4):
                cc_s[cb, NH * b:NH * b + NH, :] = cc[:, 128 * cb:128 * cb + 128]

    def wob_mm(sl, cb, half):
        def f(hook=None):
            rs = []
            for i in range(2):
                c0 = 512 * half + 256 * i
                w = mat(bring[sl, c0 // 2:c0 // 2 + 128], 4, 0, 4)
                rs.append(jnp.dot(ctx_s[cb, :, c0:c0 + 256].astype(BF16), w,
                                  preferred_element_type=F32))
            out_s[1, 0:NB, :] += rs[0] + rs[1]
            call(hook, rs[0][:, 3 * DH:])
        return f

    def init():
        wait(x_copies[:1], semx.at[0])
        wait(x_copies[1:], semx.at[1])
        if not do_compute:
            return
        xb = xb_buf[...].astype(F32)
        for cb in range(4):
            xb_s[cb] = xb[:, 128 * cb:128 * cb + 128]
        qb_s[...] = jnp.zeros(qb_s.shape, F32)
        ctx_s[...] = jnp.zeros(ctx_s.shape, F32)
        out_s[...] = jnp.zeros(out_s.shape, F32)
        for r in (ma_s, la_s, acca_s):
            r[...] = jnp.zeros(r.shape, F32)
        m_s[...] = jnp.full(m_s.shape, -jnp.inf, F32)
        l_s[...] = jnp.zeros(l_s.shape, F32)
        acc_s[...] = jnp.zeros(acc_s.shape, F32)

    def wqa_mm(j):
        def f(hook=None):
            r = jnp.dot(xa_buf[...], mat(wqa_buf[...], 32, 4 * j, 4), preferred_element_type=F32) * scale
            for i in range(4):
                h = 4 * j + i
                qa_t[8 * h:8 * h + NB, :] = r[:, DH * i:DH * i + DH]
            call(hook, r[:, 0:DH])
        return f

    def a_qk(g, k):
        def f(hook=None):
            q8 = qa_t[pl.ds(64 * k + (g >> 3), 8, stride=8), :]
            s = None
            for j in range(8):
                qm = jnp.where(row8 == j, q8, 0.0).astype(BF16)
                sj = lax.dot_general(qm, kbuf[g & 1, 8 * k + j], NT, preferred_element_type=F32)
                s = sj if s is None else s + sj
                if j == 0:
                    call(hook, sj)
            sa_s[8 * k:8 * k + 8, :] = s
        return f

    def a_sm(g):
        def f():
            first = (g & 7) == 0
            s = sa_s[...]
            m_old = jnp.where(first, -jnp.inf, ma_s[...])
            m_new = jnp.maximum(m_old, jnp.max(s, axis=-1, keepdims=True))
            alpha = jnp.exp(m_old - m_new)
            p = jnp.exp(s - m_new)
            la_s[...] = jnp.where(first, p, alpha * la_s[...] + p)
            ma_s[...] = m_new
            aa_s[...] = alpha
            sa_s[...] = p
        return f

    def a_pv(g, k):
        def f(hook=None):
            first = (g & 7) == 0
            for r0 in (16 * k, 16 * k + 8):
                rows = slice(r0, r0 + 8)
                p = sa_s[rows, :].astype(BF16)
                o = None
                for j in range(8):
                    oj = jnp.dot(p, vbuf[g & 1, r0 + j], preferred_element_type=F32)
                    o = oj if o is None else jnp.where(row8 == j, oj, o)
                    if r0 % 16 == 0 and j == 4:
                        call(hook, oj)
                acca_s[rows, :] = jnp.where(first, o, aa_s[rows, :] * acca_s[rows, :] + o)
        return f

    def a_fin(g):
        def f():
            o = acca_s[...] / jnp.sum(la_s[...], axis=-1, keepdims=True)
            oa_t[pl.ds(g >> 3, NH, stride=8), :] = o
        return f

    def woa_dot(h):
        o = oa_t[8 * h:8 * h + NB, :].astype(BF16)
        return jnp.dot(o, mat(woa_buf[64 * h:64 * h + 64], 4, 0, 4), preferred_element_type=F32)

    quads = [(hs, k) for k in (3, 2, 1, 0) for hs in ((0, 4, 8, 12), (16, 20, 24, 28))]

    def quad_lhs():
        for n, (hs, k) in enumerate(quads):
            oq_s[n, 0:NB, :] = jnp.concatenate(
                [oa_t[8 * h:8 * h + NB, 32 * k:32 * k + 32] for h in hs], axis=1)

    def quad_dot(n):
        hs, k = quads[n]
        w = jnp.concatenate([woa_buf[64 * h + RT * k:64 * h + RT * k + RT] for h in hs], axis=0)
        return jnp.dot(oq_s[n, 0:NB, :].astype(BF16), mat(w, 4, 0, 4), preferred_element_type=F32)

    def woa_mm(dot, items):
        def f():
            r = dot(items[0])
            for i in items[1:]:
                r = r + dot(i)
            out_s[0, 0:NB, :] += r
        return f

    def static_ticks(waits, starts1, starts0, comp):
        for t, (descs, sem) in enumerate(waits):
            wait(descs, sem)
            for d, s in starts0.get(t, ()):
                start(d, s, 0)
            for d, s in starts1.get(t, ()):
                start(d, s, 1)
            for f in comp.get(t, ()):
                f()

    pre0 = CFG["pre0"]
    x_copies = [(xa_hbm, xa_buf), (xb_hbm, xb_buf)]
    qr = [[a_run(wqa_hbm, wqa_buf, 256 * r + RT * s, 0, 2048) for r in range(8)]
          for s in CFG["qorder"]]
    q1 = [qr[s][r] + qr[s][r + 1] for s in range(11) for r in (0, 2, 4, 6)]
    q0 = [qr[s][r] for s in range(11, 16) for r in range(8)]
    if CFG["qord"]:
        runs = sum(qr, [])
        q1 = [runs[i] + runs[i + 1] for i in range(0, 128, 3)]
        q0 = runs[2::3]
    for j in range(D1):
        start(q1[j], sem1.at[1], 1)
        if j < pre0:
            start(q0[j], sem0.at[1], 0)
    start(x_copies[:1], semx.at[0], 0)
    start(x_copies[1:], semx.at[1], 0)
    s1, s0, cm = {}, {}, {}
    for t, d in enumerate(q1[D1:]):
        at(s1, t, (d, sem1.at[1]))
    for t in range(D1):
        at(cm, len(q1) - D1 + t, lambda t=t: kv_start(k_hbm, kbuf, 0, t, sem1.at[0]))
    n0 = len(q0) - pre0
    for j in range(n0):
        at(s0, (j * len(q1)) // n0, (q0[pre0 + j], sem0.at[1]))
    at(cm, 4, init)
    static_ticks([(d, sem1.at[1]) for d in q1], s1, s0, cm)

    oruns = [a_run(woa_hbm, woa_buf, 256 * r + RT * k, 256 * r, 256 * r + 256)
             for k in range(15, -1, -1) for r in range(8)]
    o1, o0, o_end = [], [], []
    for i, pat in enumerate(CFG["opat"]):
        lo = [oruns.pop(0) for _ in pat]
        ones = [r for r, c in zip(lo, pat) if c == "1"]
        o0.append([(len(o1) + pat[:n].count("1") // 2, r)
                   for n, (r, c) in enumerate(zip(lo, pat)) if c == "0"])
        o1 += [(ones[n] + ones[n + 1], semt.at[0, i]) for n in range(0, len(ones), 2)]
        o_end.append(len(o1) - 1)
    assert not oruns

    b_slots = CFG["b_slots"]
    a_slots = CFG["a_slots"]

    def body(g, g_lo, g_hi):
        def between(lo, hi):
            if lo <= g_lo and g_hi <= hi:
                return True
            if hi < g_lo or g_hi < lo:
                return False
            if lo <= g_lo:
                return g <= hi
            if g_hi <= hi:
                return g >= lo
            return jnp.logical_and(g >= lo, g <= hi)

        def either(x, y):
            if x is True or y is True:
                return True
            if x is False or y is False:
                return y if x is False else x
            return jnp.logical_or(x, y)

        par = g & 1
        iw = g & 3
        w_stage = [(between(0, 3), wqb_hbm), (between(4, 7), wuk_hbm),
                   (between(24, 27), wuv_hbm), (between(28, 31), wob_hbm)]
        is_c = between(8, 23)
        ic = (g - 8) & 15
        last = between(NG - 1, NG - 1)
        gn = g + 1 if last is False else (g + 1) & (NG - 1)

        sl, cb = 1 - par, (g + 3) & 3
        cm = {}
        short = [qabs_finish, c_finish]
        if do_compute:
            w3 = either(between(1, 8), between(25, 28))
            for k, hb in ((0, 0), (1, 1), (4, 2), (5, 3)):
                short.append(retile(sl, hb))
                at(cm, b_slots[k], (w3, short[-1]))
            for k, hb in ((2, 0), (6, 2)):
                at(cm, b_slots[k], (between(1, 4), both(wq_mm(cb, hb), wq_mm(cb, hb + 1))))
                at(cm, b_slots[k], (between(25, 28), both(wuv_mm(cb, hb), wuv_mm(cb, hb + 1))))
            for k, hb in ((2, 0), (3, 1), (6, 2), (7, 3)):
                at(cm, b_slots[k], (between(5, 8), wuk_mm(cb, hb)))
            at(cm, b_slots[8], (between(8, 8), qabs_finish))
            for k, f in zip(CFG["c_slots"], c_pieces(sl)):
                at(cm, b_slots[k], (between(9, 24), f))
            at(cm, b_slots[8], (between(24, 24), c_finish))
            for k, half in ((3, 0), (7, 1)):
                at(cm, b_slots[k], (between(29, 31), wob_mm(sl, cb, half)))
            for k, t in enumerate(CFG["q_slots"]):
                at(cm, t, (between(0, 0), wqa_mm(k)))
            for k in range(2):
                at(cm, a_slots[k], (between(1, 31), a_pv(g - 1, k)))
            fin = either(either(between(8, 8), between(16, 16)), between(24, 24))
            short += [a_fin(g - 1), a_sm(g)]
            at(cm, a_slots[1] + 2, (fin, short[-2]))
            for k in range(4):
                at(cm, a_slots[2 + k], (True, a_qk(g, k)))
            at(cm, a_slots[6], (True, short[-1]))

        def also(x, y):
            if x is False or y is False:
                return False
            if x is True or y is True:
                return y if x is True else x
            return jnp.logical_and(x, y)

        def b_start(j, live=True):
            for cond, hbm in w_stage:
                when(also(cond, live), lambda hbm=hbm: start(
                    b_run(hbm, 2, lambda s: 512 * iw + 256 * s, par, j), sem0.at[par], 0))
            when(also(is_c, live), lambda: start(
                b_run(c_hbm, 4, lambda s: 2048 * s + 128 * ic, par, j), sem0.at[par], 0))

        def hook_for(j):
            assert is_c is True or is_c is False
            nseg = 4 if is_c else 2
            r = (512 // nseg) * (j % nseg) + RT * b_order(nseg)[j // nseg] + boff

            def hook(v):
                bring[par, r, 0:v.shape[0], :] = v.astype(BF16)
                b_start(j)
            return hook

        embed = CFG["embed"] and not isinstance(g, int)
        hosted = False
        for t in range(32):
            dst = (kbuf if t < 16 else vbuf).at[par, pl.ds(2 * (t % 16), 2)]
            pltpu.make_async_copy(dst, dst, sem1.at[t // 16]).wait()
            if hosted is not True:
                b_start(t, True if hosted is False else jnp.logical_not(hosted))
            if t < 16:
                kv_start(v_hbm, vbuf, g, t, sem1.at[1])
            else:
                if last is not True:
                    kv_start(k_hbm, kbuf, gn, t - 16, sem1.at[0], live=between(0, NG - 2))
                when(last, lambda: start(o1[t - 16][0], o1[t - 16][1], 1))
            if t == bwait:
                when(between(0, 0), lambda: wait(sum(q0, []), sem0.at[1]))
                when(between(1, 31), lambda: wait([(None, bring.at[sl])], sem0.at[sl]))
            hosted = False
            for cond, f in cm.get(t, ()):
                if embed and t < 31 and cond is not False and f not in short:
                    hosted = either(hosted, cond)
                    pl.when(g >= 0 if cond is True else cond)(
                        lambda f=f: f(hook_for(t + 1)))
                else:
                    when(cond, f)

    cuts = CFG["cuts"]
    for lo, hi in zip(cuts[:-1], cuts[1:]):
        if hi - lo == 1:
            body(lo, lo, lo)
        else:
            def loop_body(g, carry, lo=lo, hi=hi):
                body(g, lo, hi - 1)
                return carry
            lax.fori_loop(lo, hi, loop_body, 0)

    s1, s0, cm = {}, {}, {}
    nt = len(o1)
    for t in range(nt - D1):
        at(s1, t, o1[D1 + t])
    la, lb = CFG["olead"]
    for i, grp in enumerate(o0):
        for p, r in grp:
            at(s0, max(0, p - (la + ((lb - la) * p) // nt)), (r, semt.at[1, i]))
        at(cm, o_end[i], lambda i=i, grp=grp: wait(sum((r for _, r in grp), []), semt.at[1, i]))
    at(cm, 7, lambda: wait([(None, bring.at[1])], sem0.at[1]))

    def write_b():
        o_ref[:, DM:2 * DM] = out_s[1, 0:NB, :].astype(o_ref.dtype)

    if do_compute:
        at(cm, 1, a_pv(NG - 1, 0))
        at(cm, 3, a_pv(NG - 1, 1))
        at(cm, 5, a_fin(NG - 1))
        at(cm, 7, wob_mm(1, 3, 0))
        at(cm, 15, both(wob_mm(1, 3, 1), write_b))
        at(cm, 17, quad_lhs)
        for i in range(3):
            at(cm, o_end[i], woa_mm(woa_dot, tuple(range(3 - i, 16, 4))))
            at(cm, o_end[i] + 2, woa_mm(woa_dot, tuple(range(19 - i, 32, 4))))
        n = 0
        for i, pat in list(enumerate(CFG["opat"]))[3:-1]:
            at(cm, o_end[i], woa_mm(quad_dot, tuple(range(n, n + len(pat) // 4))))
            n += len(pat) // 4
    static_ticks(o1, s1, s0, cm)
    if do_compute:
        r = out_s[0, 0:NB, :]
        for i in range(n, 8):
            r = r + quad_dot(i)
        o_ref[:, 0:DM] = r.astype(o_ref.dtype)
    else:
        o_ref[...] = jnp.zeros(o_ref.shape, o_ref.dtype)


def _tiles(x):
    c = x.shape[-1]
    return x.reshape(-1, 8, c // DH, DH).transpose(0, 2, 1, 3).reshape(-1, 8, DH)


@jax.jit
def pallas_concat_heads__sliding_block_cached__compressed_kv_cla__decode_kernel(
    A_x: jax.Array,
    A_k_cache: jax.Array,
    A_v_cache: jax.Array,
    A_wq: jax.Array,
    A_wo: jax.Array,
    B_x: jax.Array,
    B_c_kv: jax.Array,
    B_w_q: jax.Array,
    B_w_uk: jax.Array,
    B_w_uv: jax.Array,
    B_w_o: jax.Array,
):
    assert A_x.shape == (NB, 1, DM) and B_x.shape == (NB, 1, DM)
    assert A_k_cache.shape == (NB, NH, SK, DH) and B_c_kv.shape == (NB, SK, DM)
    vm = pltpu.VMEM
    out = pl.pallas_call(
        _kernel,
        out_shape=jax.ShapeDtypeStruct((NB, 2 * DM), A_x.dtype),
        in_specs=[pl.BlockSpec(memory_space=pl.ANY)] * 11,
        out_specs=pl.BlockSpec(memory_space=pltpu.VMEM),
        scratch_shapes=[
            vm((NB, DM), BF16), vm((NB, DM), BF16),
            vm((2, NH, RUN, DH), BF16), vm((2, NH, RUN, DH), BF16),
            vm((2048, 8, DH), BF16), vm((2048, 8, DH), BF16),
            vm((2, 512, 8, DH), BF16),
            vm((4, NB, 128), F32),
            vm((NH * 8, DH), F32),
            vm((NH * 8, DH), F32),
            vm((NH, RUN), F32),
            vm((NH, DH), F32), vm((NH, DH), F32),
            vm((NH, DH), F32), vm((NH, DH), F32),
            vm((NB, NH * DH), F32),
            vm((4, NH * 8, 128), F32),
            vm((NB, NH, DM), BF16),
            vm((NB, NH, CK), F32),
            vm((NB, NH, CK), BF16),
            vm((NB, NH, 128), F32),
            vm((NB, NH, 128), F32), vm((NB, NH, 128), F32),
            vm((NB, NH, DM), F32),
            vm((4, NB * NH, 128), F32),
            vm((4, NB, 8 * DH), F32),
            vm((2, 8, DM), F32),
            vm((8, 8, DH), F32),
            vm((128, 8 * DH), BF16), vm((128, 8 * DH), BF16),
            pltpu.SemaphoreType.DMA((2,)), pltpu.SemaphoreType.DMA((2,)),
            pltpu.SemaphoreType.DMA((2,)), pltpu.SemaphoreType.DMA((2, len(CFG["opat"]))),
        ],
        compiler_params=pltpu.CompilerParams(
            vmem_limit_bytes=48 * 1024 * 1024,
            disable_bounds_checks=not CFG["checks"],
            disable_semaphore_checks=not CFG["checks"],
        ),
        name="concat_heads_decode",
    )(
        A_x.reshape(NB, DM), B_x.reshape(NB, DM), A_k_cache, A_v_cache,
        _tiles(A_wq), _tiles(A_wo), _tiles(B_c_kv),
        _tiles(B_w_q), _tiles(B_w_uk), _tiles(B_w_uv), _tiles(B_w_o),
    )
    return out.reshape(NB, 1, 2 * DM)
```

```python
import jax
import jax.numpy as jnp
from jax import lax
import jax.experimental.pallas as pl
import jax.experimental.pallas.tpu as pltpu

F32 = jnp.float32
BF16 = jnp.bfloat16

NB = 4
NH = 32
DH = 128
DM = 512
SK = 4096
WIN = 1024
CK = 256
NG = 32
RUN = 128
RT = 16
D1 = 16
NT = ((1,), (1,)), ((), ())

CFG = dict(compute=True, pre0=6, bwait=6, aoff=1, boff=1, embed=True,
           hbasis=(16, 15, 3, 4, 1), hoff=0, wbasis=(1, 31, 8, 5, 6), cbasis=(8, 16, 1, 3, 6), koff=1,
           qorder=(1, 2, 4, 3, 7, 8, 6, 5, 13, 14, 0, 15, 11, 12, 10, 9), qord=True, olead=(6, 6),
           opat=("110" * 10 + "11", "011" * 10 + "11", "011" * 10 + "11", "011" * 5 + "0",
                 "11011011", "1111", "1111"),
           q_slots=(6, 8, 10, 12, 14, 15, 17, 19), checks=False,
           cuts=(0, 8, 24, 32), a_slots=(1, 3, 16, 18, 20, 22, 24),
           b_slots=(6, 8, 10, 12, 14, 26, 28, 30, 31), c_slots=(0, 1, 2, 3, 5, 6))


def _xor_order(basis):
    out = [0]
    for v in basis:
        out += [x ^ v for x in out]
    assert sorted(out) == list(range(len(out)))
    return out


def _mult(x, m):
    return x if isinstance(x, int) else pl.multiple_of(x, m)


def _kernel(xa_hbm, xb_hbm, k_hbm, v_hbm, wqa_hbm, woa_hbm, c_hbm, wqb_hbm, wuk_hbm,
            wuv_hbm, wob_hbm, o_ref,
            xa_buf, xb_buf, kbuf, vbuf, wqa_buf, woa_buf, bring,
            xb_s, qa_t, oa_t, sa_s, ma_s, la_s, aa_s, acca_s, qb_s, qabs_t, qabs_s, sb_s, pb_s, al_s,
            m_s, l_s, acc_s, cc_s, ctx_s, out_s, oq_s, w2a_s, w2b_s,
            sem1, sem0, semx, semt):
    do_compute = CFG["compute"]
    aoff, boff = CFG["aoff"], CFG["boff"]
    bwait = CFG["bwait"]
    scale = DH ** -0.5
    w2_s = (w2a_s, w2b_s)
    h_order = [(x + CFG["hoff"]) % NH for x in _xor_order(CFG["hbasis"])]
    w_order = [(x + CFG["koff"]) % 32 for x in _xor_order(CFG["wbasis"])]
    c_order = [(x & 24) + (x + CFG["koff"]) % 8 for x in _xor_order(CFG["cbasis"])]
    row8 = lax.broadcasted_iota(jnp.int32, (8, DH), 0)

    def start(descs, sem, prio):
        for src, dst in descs:
            pltpu.make_async_copy(src, dst, sem).start(priority=prio)

    def wait(descs, sem):
        for _, dst in descs:
            pltpu.make_async_copy(dst, dst, sem).wait()

    def at(d, t, item):
        d.setdefault(t, []).append(item)

    def both(*fs, host=0):
        def f(hook=None):
            for i, g in enumerate(fs):
                if i == host:
                    g(hook)
                else:
                    g()
        return f

    def call(hook, v):
        if hook is not None:
            hook(v)

    def mat(w, ncol, j0, n):
        w = w.reshape(w.shape[0] // ncol, ncol, 8, DH)
        cols = [w[:, j0 + j].reshape(w.shape[0] * 8, DH) for j in range(n)]
        return jnp.concatenate(cols, axis=1)

    def when(cond, f):
        if cond is True:
            f()
        elif cond is not False:
            pl.when(cond)(f)

    def kv_start(hbm, buf, g, t, sem, live=True):
        b, sl = g >> 3, g & 7
        ko = 8 * aoff
        w0 = SK - WIN
        heads = h_order[2 * t:2 * t + 2]
        row = _mult(w0 + RUN * sl - ko, 8)
        reg = [(hbm.at[b, h, pl.ds(row, RUN)], buf.at[g & 1, h]) for h in heads]
        if ko == 0:
            when(live, lambda: start(reg, sem, 1))
            return
        fst = [(hbm.at[b, h, pl.ds(w0, RUN - ko)], buf.at[g & 1, h, pl.ds(ko, RUN - ko)])
               for h in heads]
        if t == 0:
            fst = [(hbm.at[b, :, pl.ds(SK - ko, ko)], buf.at[g & 1, :, pl.ds(0, ko)])] + fst
        if isinstance(sl, int):
            when(live, lambda: start(reg if sl else fst, sem, 1))
        else:
            pl.when(sl > 0)(lambda: start(reg, sem, 1))
            first = sl == 0
            pl.when(first if live is True else jnp.logical_and(first, live))(
                lambda: start(fst, sem, 1))

    def b_pos(nseg, t):
        return divmod((c_order if nseg == 4 else w_order)[t], 32 // nseg)

    def b_run(hbm, nseg, src, sl, t):
        seg, k = b_pos(nseg, t)
        ln = 512 // nseg
        r = boff + RT * k
        n = min(RT, ln - r)
        out = [(hbm.at[pl.ds(src(seg) + r, n)], bring.at[sl, pl.ds(ln * seg + r, n)])]
        if k == 0 and boff:
            out.append((hbm.at[pl.ds(src(seg), boff)], bring.at[sl, pl.ds(ln * seg, boff)]))
        return out

    def a_run(hbm, buf, r, lo, hi):
        r0, r1 = max(r - aoff, lo), (hi if r + RT == hi else r + RT - aoff)
        return [(hbm.at[pl.ds(r0, r1 - r0)], buf.at[pl.ds(r0, r1 - r0)])]

    def retile(sl, hb):
        def f():
            w = bring[sl].reshape(128, 4, 8, DH)[:, hb]
            w2_s[hb & 1][...] = w.reshape(128, 8 * DH)
        return f

    def wq_mm(cb, hb):
        def f(hook=None):
            r = jnp.dot(xb_s[cb].astype(BF16), w2_s[hb & 1][...], preferred_element_type=F32)
            qb_s[:, 1024 * hb:1024 * hb + 1024] += r
            call(hook, r[:, 7 * DH:])
        return f

    def wuk_mm(cb, hb):
        def f(hook=None):
            for j in range(8):
                h = 8 * hb + j
                q = (qb_s[:, DH * h:DH * h + DH] * scale).astype(BF16)
                r = lax.dot_general(q, w2_s[hb & 1][:, DH * j:DH * j + DH], NT,
                                    preferred_element_type=F32)
                qabs_t[cb, 8 * h:8 * h + NB, :] = r
                if j == 0:
                    r0 = r
            call(hook, r0)
        return f

    def wuv_mm(cb, hb):
        def f(hook=None):
            for j in range(8):
                cc = cc_s[cb, pl.ds(8 * hb + j, NB, stride=NH), :].astype(BF16)
                r = jnp.dot(cc, w2_s[hb & 1][:, DH * j:DH * j + DH], preferred_element_type=F32)
                ctx_s[hb, :, DH * j:DH * j + DH] += r
            call(hook, r)
        return f

    def qabs_finish():
        for b in range(NB):
            for cb in range(4):
                qabs_s[b, :, 128 * cb:128 * cb + 128] = (
                    qabs_t[cb, pl.ds(b, NH, stride=8), :].astype(BF16))

    def c_pieces(sl):
        def cmat(b):
            return mat(bring[sl, 128 * b:128 * b + 128], 4, 0, 4)

        def qk(b):
            def f(hook=None):
                s = lax.dot_general(qabs_s[b], cmat(b), NT, preferred_element_type=F32)
                sb_s[b] = s
                call(hook, s[0:8, 0:DH])
            return f

        def sm(b):
            def f():
                s = sb_s[b]
                m_old = m_s[b]
                m_new = jnp.maximum(m_old, jnp.max(s, axis=-1, keepdims=True))
                alpha = jnp.exp(m_old - m_new)
                ps = [jnp.exp(s[:, 128 * j:128 * j + 128] - m_new) for j in range(CK // 128)]
                l_s[b] = alpha * l_s[b] + sum(ps[1:], ps[0])
                m_s[b] = m_new
                al_s[b] = alpha
                pb_s[b] = jnp.concatenate(ps, axis=-1).astype(BF16)
            return f

        def pv(b):
            def f(hook=None):
                r = jnp.dot(pb_s[b], cmat(b), preferred_element_type=F32)
                al = al_s[b]
                for j in range(4):
                    cols = slice(128 * j, 128 * j + 128)
                    acc_s[b, :, cols] = al * acc_s[b, :, cols] + r[:, cols]
                if hook is not None:
                    keep["v"] = r[0:8, 3 * DH:]
            return f

        keep = {}

        def late(f):
            def g(hook=None):
                f(hook)
                if hook is not None:
                    hook(keep["v"])
            return g

        return [qk(0), both(qk(1), sm(0)), both(qk(2), sm(1)), both(qk(3), sm(2)),
                late(both(sm(3), pv(0), pv(1), host=1)), late(both(pv(2), pv(3)))]

    def c_finish():
        for b in range(NB):
            cc = acc_s[b] / jnp.sum(l_s[b], axis=-1, keepdims=True)
            for cb in range(4):
                cc_s[cb, NH * b:NH * b + NH, :] = cc[:, 128 * cb:128 * cb + 128]

    def wob_mm(sl, cb, half):
        def f(hook=None):
            rs = []
            for i in range(2):
                c0 = 512 * half + 256 * i
                w = mat(bring[sl, c0 // 2:c0 // 2 + 128], 4, 0, 4)
                rs.append(jnp.dot(ctx_s[cb, :, c0:c0 + 256].astype(BF16), w,
                                  preferred_element_type=F32))
            out_s[1, 0:NB, :] += rs[0] + rs[1]
            call(hook, rs[0][:, 3 * DH:])
        return f

    def init():
        wait(x_copies[:1], semx.at[0])
        wait(x_copies[1:], semx.at[1])
        if not do_compute:
            return
        xb = xb_buf[...].astype(F32)
        for cb in range(4):
            xb_s[cb] = xb[:, 128 * cb:128 * cb + 128]
        qb_s[...] = jnp.zeros(qb_s.shape, F32)
        ctx_s[...] = jnp.zeros(ctx_s.shape, F32)
        out_s[...] = jnp.zeros(out_s.shape, F32)
        for r in (ma_s, la_s, acca_s):
            r[...] = jnp.zeros(r.shape, F32)
        m_s[...] = jnp.full(m_s.shape, -jnp.inf, F32)
        l_s[...] = jnp.zeros(l_s.shape, F32)
        acc_s[...] = jnp.zeros(acc_s.shape, F32)

    def wqa_mm(j):
        def f(hook=None):
            r = jnp.dot(xa_buf[...], mat(wqa_buf[...], 32, 4 * j, 4), preferred_element_type=F32) * scale
            for i in range(4):
                h = 4 * j + i
                qa_t[8 * h:8 * h + NB, :] = r[:, DH * i:DH * i + DH]
            call(hook, r[:, 0:DH])
        return f

    def a_qk(g, k):
        def f(hook=None):
            q8 = qa_t[pl.ds(64 * k + (g >> 3), 8, stride=8), :]
            s = None
            for j in range(8):
                qm = jnp.where(row8 == j, q8, 0.0).astype(BF16)
                sj = lax.dot_general(qm, kbuf[g & 1, 8 * k + j], NT, preferred_element_type=F32)
                s = sj if s is None else s + sj
                if j == 0:
                    call(hook, sj)
            sa_s[8 * k:8 * k + 8, :] = s
        return f

    def a_sm(g):
        def f():
            first = (g & 7) == 0
            s = sa_s[...]
            m_old = jnp.where(first, -jnp.inf, ma_s[...])
            m_new = jnp.maximum(m_old, jnp.max(s, axis=-1, keepdims=True))
            alpha = jnp.exp(m_old - m_new)
            p = jnp.exp(s - m_new)
            la_s[...] = jnp.where(first, p, alpha * la_s[...] + p)
            ma_s[...] = m_new
            aa_s[...] = alpha
            sa_s[...] = p
        return f

    def a_pv(g, k):
        def f(hook=None):
            first = (g & 7) == 0
            for r0 in (16 * k, 16 * k + 8):
                rows = slice(r0, r0 + 8)
                p = sa_s[rows, :].astype(BF16)
                o = None
                for j in range(8):
                    oj = jnp.dot(p, vbuf[g & 1, r0 + j], preferred_element_type=F32)
                    o = oj if o is None else jnp.where(row8 == j, oj, o)
                    if r0 % 16 == 0 and j == 4:
                        call(hook, oj)
                acca_s[rows, :] = jnp.where(first, o, aa_s[rows, :] * acca_s[rows, :] + o)
        return f

    def a_fin(g):
        def f():
            o = acca_s[...] / jnp.sum(la_s[...], axis=-1, keepdims=True)
            oa_t[pl.ds(g >> 3, NH, stride=8), :] = o
        return f

    def woa_dot(h):
        o = oa_t[8 * h:8 * h + NB, :].astype(BF16)
        return jnp.dot(o, mat(woa_buf[64 * h:64 * h + 64], 4, 0, 4), preferred_element_type=F32)

    quads = [(hs, k) for k in (3, 2, 1, 0) for hs in ((0, 4, 8, 12), (16, 20, 24, 28))]

    def quad_lhs():
        for n, (hs, k) in enumerate(quads):
            oq_s[n, 0:NB, :] = jnp.concatenate(
                [oa_t[8 * h:8 * h + NB, 32 * k:32 * k + 32] for h in hs], axis=1)

    def quad_dot(n):
        hs, k = quads[n]
        w = jnp.concatenate([woa_buf[64 * h + RT * k:64 * h + RT * k + RT] for h in hs], axis=0)
        return jnp.dot(oq_s[n, 0:NB, :].astype(BF16), mat(w, 4, 0, 4), preferred_element_type=F32)

    def woa_mm(dot, items):
        def f():
            r = dot(items[0])
            for i in items[1:]:
                r = r + dot(i)
            out_s[0, 0:NB, :] += r
        return f

    def static_ticks(waits, starts1, starts0, comp):
        for t, (descs, sem) in enumerate(waits):
            wait(descs, sem)
            for d, s in starts0.get(t, ()):
                start(d, s, 0)
            for d, s in starts1.get(t, ()):
                start(d, s, 1)
            for f in comp.get(t, ()):
                f()

    pre0 = CFG["pre0"]
    x_copies = [(xa_hbm, xa_buf), (xb_hbm, xb_buf)]
    qr = [[a_run(wqa_hbm, wqa_buf, 256 * r + RT * s, 0, 2048) for r in range(8)]
          for s in CFG["qorder"]]
    q1 = [qr[s][r] + qr[s][r + 1] for s in range(11) for r in (0, 2, 4, 6)]
    q0 = [qr[s][r] for s in range(11, 16) for r in range(8)]
    if CFG["qord"]:
        runs = sum(qr, [])
        q1 = [runs[i] + runs[i + 1] for i in range(0, 128, 3)]
        q0 = runs[2::3]
    for j in range(D1):
        start(q1[j], sem1.at[1], 1)
        if j < pre0:
            start(q0[j], sem0.at[1], 0)
    start(x_copies[:1], semx.at[0], 0)
    start(x_copies[1:], semx.at[1], 0)
    s1, s0, cm = {}, {}, {}
    for t, d in enumerate(q1[D1:]):
        at(s1, t, (d, sem1.at[1]))
    for t in range(D1):
        at(cm, len(q1) - D1 + t, lambda t=t: kv_start(k_hbm, kbuf, 0, t, sem1.at[0]))
    n0 = len(q0) - pre0
    for j in range(n0):
        at(s0, (j * len(q1)) // n0, (q0[pre0 + j], sem0.at[1]))
    at(cm, 4, init)
    static_ticks([(d, sem1.at[1]) for d in q1], s1, s0, cm)

    oruns = [a_run(woa_hbm, woa_buf, 256 * r + RT * k, 256 * r, 256 * r + 256)
             for k in range(15, -1, -1) for r in range(8)]
    o1, o0, o_end = [], [], []
    for i, pat in enumerate(CFG["opat"]):
        lo = [oruns.pop(0) for _ in pat]
        ones = [r for r, c in zip(lo, pat) if c == "1"]
        o0.append([(len(o1) + pat[:n].count("1") // 2, r)
                   for n, (r, c) in enumerate(zip(lo, pat)) if c == "0"])
        o1 += [(ones[n] + ones[n + 1], semt.at[0, i]) for n in range(0, len(ones), 2)]
        o_end.append(len(o1) - 1)
    assert not oruns

    b_slots = CFG["b_slots"]
    a_slots = CFG["a_slots"]

    def body(g, g_lo, g_hi):
        def between(lo, hi):
            if lo <= g_lo and g_hi <= hi:
                return True
            if hi < g_lo or g_hi < lo:
                return False
            if lo <= g_lo:
                return g <= hi
            if g_hi <= hi:
                return g >= lo
            return jnp.logical_and(g >= lo, g <= hi)

        def either(x, y):
            if x is True or y is True:
                return True
            if x is False or y is False:
                return y if x is False else x
            return jnp.logical_or(x, y)

        par = g & 1
        iw = g & 3
        w_stage = [(between(0, 3), wqb_hbm), (between(4, 7), wuk_hbm),
                   (between(24, 27), wuv_hbm), (between(28, 31), wob_hbm)]
        is_c = between(8, 23)
        ic = (g - 8) & 15
        last = between(NG - 1, NG - 1)
        gn = g + 1 if last is False else (g + 1) & (NG - 1)

        sl, cb = 1 - par, (g + 3) & 3
        cm = {}
        short = [qabs_finish, c_finish]
        if do_compute:
            w3 = either(between(1, 8), between(25, 28))
            for k, hb in ((0, 0), (1, 1), (4, 2), (5, 3)):
                short.append(retile(sl, hb))
                at(cm, b_slots[k], (w3, short[-1]))
            for k, hb in ((2, 0), (6, 2)):
                at(cm, b_slots[k], (between(1, 4), both(wq_mm(cb, hb), wq_mm(cb, hb + 1))))
                at(cm, b_slots[k], (between(25, 28), both(wuv_mm(cb, hb), wuv_mm(cb, hb + 1))))
            for k, hb in ((2, 0), (3, 1), (6, 2), (7, 3)):
                at(cm, b_slots[k], (between(5, 8), wuk_mm(cb, hb)))
            at(cm, b_slots[8], (between(8, 8), qabs_finish))
            for k, f in zip(CFG["c_slots"], c_pieces(sl)):
                at(cm, b_slots[k], (between(9, 24), f))
            at(cm, b_slots[8], (between(24, 24), c_finish))
            for k, half in ((3, 0), (7, 1)):
                at(cm, b_slots[k], (between(29, 31), wob_mm(sl, cb, half)))
            for k, t in enumerate(CFG["q_slots"]):
                at(cm, t, (between(0, 0), wqa_mm(k)))
            for k in range(2):
                at(cm, a_slots[k], (between(1, 31), a_pv(g - 1, k)))
            fin = either(either(between(8, 8), between(16, 16)), between(24, 24))
            short += [a_fin(g - 1), a_sm(g)]
            at(cm, a_slots[1] + 2, (fin, short[-2]))
            for k in range(4):
                at(cm, a_slots[2 + k], (True, a_qk(g, k)))
            at(cm, a_slots[6], (True, short[-1]))

        def also(x, y):
            if x is False or y is False:
                return False
            if x is True or y is True:
                return y if x is True else x
            return jnp.logical_and(x, y)

        def b_start(j, live=True):
            for cond, hbm in w_stage:
                when(also(cond, live), lambda hbm=hbm: start(
                    b_run(hbm, 1, lambda s: 512 * iw, par, j), sem0.at[par], 0))
            when(also(is_c, live), lambda: start(
                b_run(c_hbm, 4, lambda s: 2048 * s + 128 * ic, par, j), sem0.at[par], 0))

        def hook_for(j):
            assert is_c is True or is_c is False
            seg, k = b_pos(4 if is_c else 1, j)
            r = 128 * seg + RT * k + boff

            def hook(v):
                bring[par, r, 0:v.shape[0], :] = v.astype(BF16)
                b_start(j)
            return hook

        embed = CFG["embed"] and not isinstance(g, int)
        hosted = False
        for t in range(32):
            dst = (kbuf if t < 16 else vbuf).at[par, pl.ds(2 * (t % 16), 2)]
            pltpu.make_async_copy(dst, dst, sem1.at[t // 16]).wait()
            if hosted is not True:
                b_start(t, True if hosted is False else jnp.logical_not(hosted))
            if t < 16:
                kv_start(v_hbm, vbuf, g, t, sem1.at[1])
            else:
                if last is not True:
                    kv_start(k_hbm, kbuf, gn, t - 16, sem1.at[0], live=between(0, NG - 2))
                when(last, lambda: start(o1[t - 16][0], o1[t - 16][1], 1))
            if t == bwait:
                when(between(0, 0), lambda: wait(sum(q0, []), sem0.at[1]))
                when(between(1, 31), lambda: wait([(None, bring.at[sl])], sem0.at[sl]))
            hosted = False
            for cond, f in cm.get(t, ()):
                if embed and t < 31 and cond is not False and f not in short:
                    hosted = either(hosted, cond)
                    pl.when(g >= 0 if cond is True else cond)(
                        lambda f=f: f(hook_for(t + 1)))
                else:
                    when(cond, f)

    cuts = CFG["cuts"]
    for lo, hi in zip(cuts[:-1], cuts[1:]):
        if hi - lo == 1:
            body(lo, lo, lo)
        else:
            def loop_body(g, carry, lo=lo, hi=hi):
                body(g, lo, hi - 1)
                return carry
            lax.fori_loop(lo, hi, loop_body, 0)

    s1, s0, cm = {}, {}, {}
    nt = len(o1)
    for t in range(nt - D1):
        at(s1, t, o1[D1 + t])
    la, lb = CFG["olead"]
    for i, grp in enumerate(o0):
        for p, r in grp:
            at(s0, max(0, p - (la + ((lb - la) * p) // nt)), (r, semt.at[1, i]))
        at(cm, o_end[i], lambda i=i, grp=grp: wait(sum((r for _, r in grp), []), semt.at[1, i]))
    at(cm, 7, lambda: wait([(None, bring.at[1])], sem0.at[1]))

    def write_b():
        o_ref[:, DM:2 * DM] = out_s[1, 0:NB, :].astype(o_ref.dtype)

    if do_compute:
        at(cm, 1, a_pv(NG - 1, 0))
        at(cm, 3, a_pv(NG - 1, 1))
        at(cm, 5, a_fin(NG - 1))
        at(cm, 7, wob_mm(1, 3, 0))
        at(cm, 15, both(wob_mm(1, 3, 1), write_b))
        at(cm, 17, quad_lhs)
        for i in range(3):
            at(cm, o_end[i], woa_mm(woa_dot, tuple(range(3 - i, 16, 4))))
            at(cm, o_end[i] + 2, woa_mm(woa_dot, tuple(range(19 - i, 32, 4))))
        n = 0
        for i, pat in list(enumerate(CFG["opat"]))[3:-1]:
            at(cm, o_end[i], woa_mm(quad_dot, tuple(range(n, n + len(pat) // 4))))
            n += len(pat) // 4
    static_ticks(o1, s1, s0, cm)
    if do_compute:
        r = out_s[0, 0:NB, :]
        for i in range(n, 8):
            r = r + quad_dot(i)
        o_ref[:, 0:DM] = r.astype(o_ref.dtype)
    else:
        o_ref[...] = jnp.zeros(o_ref.shape, o_ref.dtype)


def _tiles(x):
    c = x.shape[-1]
    return x.reshape(-1, 8, c // DH, DH).transpose(0, 2, 1, 3).reshape(-1, 8, DH)


@jax.jit
def pallas_concat_heads__sliding_block_cached__compressed_kv_cla__decode_kernel(
    A_x: jax.Array,
    A_k_cache: jax.Array,
    A_v_cache: jax.Array,
    A_wq: jax.Array,
    A_wo: jax.Array,
    B_x: jax.Array,
    B_c_kv: jax.Array,
    B_w_q: jax.Array,
    B_w_uk: jax.Array,
    B_w_uv: jax.Array,
    B_w_o: jax.Array,
):
    assert A_x.shape == (NB, 1, DM) and B_x.shape == (NB, 1, DM)
    assert A_k_cache.shape == (NB, NH, SK, DH) and B_c_kv.shape == (NB, SK, DM)
    vm = pltpu.VMEM
    out = pl.pallas_call(
        _kernel,
        out_shape=jax.ShapeDtypeStruct((NB, 2 * DM), A_x.dtype),
        in_specs=[pl.BlockSpec(memory_space=pl.ANY)] * 11,
        out_specs=pl.BlockSpec(memory_space=pltpu.VMEM),
        scratch_shapes=[
            vm((NB, DM), BF16), vm((NB, DM), BF16),
            vm((2, NH, RUN, DH), BF16), vm((2, NH, RUN, DH), BF16),
            vm((2048, 8, DH), BF16), vm((2048, 8, DH), BF16),
            vm((2, 512, 8, DH), BF16),
            vm((4, NB, 128), F32),
            vm((NH * 8, DH), F32),
            vm((NH * 8, DH), F32),
            vm((NH, RUN), F32),
            vm((NH, DH), F32), vm((NH, DH), F32),
            vm((NH, DH), F32), vm((NH, DH), F32),
            vm((NB, NH * DH), F32),
            vm((4, NH * 8, 128), F32),
            vm((NB, NH, DM), BF16),
            vm((NB, NH, CK), F32),
            vm((NB, NH, CK), BF16),
            vm((NB, NH, 128), F32),
            vm((NB, NH, 128), F32), vm((NB, NH, 128), F32),
            vm((NB, NH, DM), F32),
            vm((4, NB * NH, 128), F32),
            vm((4, NB, 8 * DH), F32),
            vm((2, 8, DM), F32),
            vm((8, 8, DH), F32),
            vm((128, 8 * DH), BF16), vm((128, 8 * DH), BF16),
            pltpu.SemaphoreType.DMA((2,)), pltpu.SemaphoreType.DMA((2,)),
            pltpu.SemaphoreType.DMA((2,)), pltpu.SemaphoreType.DMA((2, len(CFG["opat"]))),
        ],
        compiler_params=pltpu.CompilerParams(
            vmem_limit_bytes=48 * 1024 * 1024,
            disable_bounds_checks=not CFG["checks"],
            disable_semaphore_checks=not CFG["checks"],
        ),
        name="concat_heads_decode",
    )(
        A_x.reshape(NB, DM), B_x.reshape(NB, DM), A_k_cache, A_v_cache,
        _tiles(A_wq), _tiles(A_wo), _tiles(B_c_kv),
        _tiles(B_w_q), _tiles(B_w_uk), _tiles(B_w_uv), _tiles(B_w_o),
    )
    return out.reshape(NB, 1, 2 * DM)
```

```python
import jax
import jax.numpy as jnp
from jax import lax
import jax.experimental.pallas as pl
import jax.experimental.pallas.tpu as pltpu

F32 = jnp.float32
BF16 = jnp.bfloat16

NB = 4
NH = 32
DH = 128
DM = 512
SK = 4096
WIN = 1024
CK = 256
NG = 32
RUN = 128
RT = 16
D1 = 16
NT = ((1,), (1,)), ((), ())

CFG = dict(
    compute=True, checks=False,
    aoff=1, boff=1,
    hbasis=(16, 15, 3, 4, 1), hoff=0, wbasis=(1, 31, 8, 5, 6), cbasis=(8, 16, 1, 3, 6), koff=1,
    qbasis=(1, 86, 105, 20, 15, 100, 98), qoff=65,
    pre0=6,
    opat=("110" * 10 + "11", "011" * 10 + "11", "011" * 10 + "11", "011" * 5 + "0",
          "11011011", "1111", "1111"),
    olead=(6, 8),
    cuts=(0, 8, 24, 32),
    embed=True,
    bwait=6,
    a_slots=(1, 3, 16, 18, 20, 22, 24), b_slots=(6, 8, 10, 12, 14, 26, 28, 30, 31),
    c_slots=(0, 1, 2, 3, 5, 6), q_slots=(6, 8, 10, 12, 14, 15, 17, 19),
)


def _xor_order(basis):
    out = [0]
    for v in basis:
        out += [x ^ v for x in out]
    assert sorted(out) == list(range(len(out)))
    return out


def _mult(x, m):
    return x if isinstance(x, int) else pl.multiple_of(x, m)


def _kernel(xa_hbm, xb_hbm, k_hbm, v_hbm, wqa_hbm, woa_hbm, c_hbm, wqb_hbm, wuk_hbm,
            wuv_hbm, wob_hbm, o_ref,
            xa_buf, xb_buf, kbuf, vbuf, wqa_buf, woa_buf, bring,
            xb_s, qa_t, oa_t, sa_s, ma_s, la_s, aa_s, acca_s, qb_s, qabs_t, qabs_s, sb_s, pb_s, al_s,
            m_s, l_s, acc_s, cc_s, ctx_s, out_s, oq_s, w2a_s, w2b_s,
            sem1, sem0, semx, semt):
    do_compute = CFG["compute"]
    aoff, boff = CFG["aoff"], CFG["boff"]
    bwait = CFG["bwait"]
    scale = DH ** -0.5
    w2_s = (w2a_s, w2b_s)
    h_order = [(x + CFG["hoff"]) % NH for x in _xor_order(CFG["hbasis"])]
    w_order = [(x + CFG["koff"]) % 32 for x in _xor_order(CFG["wbasis"])]
    c_order = [(x & 24) + (x + CFG["koff"]) % 8 for x in _xor_order(CFG["cbasis"])]
    row8 = lax.broadcasted_iota(jnp.int32, (8, DH), 0)

    def start(descs, sem, prio):
        for src, dst in descs:
            pltpu.make_async_copy(src, dst, sem).start(priority=prio)

    def wait(descs, sem):
        for _, dst in descs:
            pltpu.make_async_copy(dst, dst, sem).wait()

    def at(d, t, item):
        d.setdefault(t, []).append(item)

    def both(*fs, host=0):
        def f(hook=None):
            for i, g in enumerate(fs):
                if i == host:
                    g(hook)
                else:
                    g()
        return f

    def call(hook, v):
        if hook is not None:
            hook(v)

    def mat(w, ncol, j0, n):
        w = w.reshape(w.shape[0] // ncol, ncol, 8, DH)
        cols = [w[:, j0 + j].reshape(w.shape[0] * 8, DH) for j in range(n)]
        return jnp.concatenate(cols, axis=1)

    def when(cond, f):
        if cond is True:
            f()
        elif cond is not False:
            pl.when(cond)(f)

    def kv_start(hbm, buf, g, t, sem, live=True):
        b, sl = g >> 3, g & 7
        ko = 8 * aoff
        w0 = SK - WIN
        heads = h_order[2 * t:2 * t + 2]
        row = _mult(w0 + RUN * sl - ko, 8)
        reg = [(hbm.at[b, h, pl.ds(row, RUN)], buf.at[g & 1, h]) for h in heads]
        if ko == 0:
            when(live, lambda: start(reg, sem, 1))
            return
        fst = [(hbm.at[b, h, pl.ds(w0, RUN - ko)], buf.at[g & 1, h, pl.ds(ko, RUN - ko)])
               for h in heads]
        if t == 0:
            fst = [(hbm.at[b, :, pl.ds(SK - ko, ko)], buf.at[g & 1, :, pl.ds(0, ko)])] + fst
        if isinstance(sl, int):
            when(live, lambda: start(reg if sl else fst, sem, 1))
        else:
            pl.when(sl > 0)(lambda: start(reg, sem, 1))
            first = sl == 0
            pl.when(first if live is True else jnp.logical_and(first, live))(
                lambda: start(fst, sem, 1))

    def b_pos(nseg, t):
        return divmod((c_order if nseg == 4 else w_order)[t], 32 // nseg)

    def b_run(hbm, nseg, src, sl, t):
        seg, k = b_pos(nseg, t)
        ln = 512 // nseg
        r = boff + RT * k
        n = min(RT, ln - r)
        out = [(hbm.at[pl.ds(src(seg) + r, n)], bring.at[sl, pl.ds(ln * seg + r, n)])]
        if k == 0 and boff:
            out.append((hbm.at[pl.ds(src(seg), boff)], bring.at[sl, pl.ds(ln * seg, boff)]))
        return out

    def a_run(hbm, buf, r, lo, hi):
        r0, r1 = max(r - aoff, lo), (hi if r + RT == hi else r + RT - aoff)
        return [(hbm.at[pl.ds(r0, r1 - r0)], buf.at[pl.ds(r0, r1 - r0)])]

    def retile(sl, hb):
        def f():
            w = bring[sl].reshape(128, 4, 8, DH)[:, hb]
            w2_s[hb & 1][...] = w.reshape(128, 8 * DH)
        return f

    def wq_mm(cb, hb):
        def f(hook=None):
            r = jnp.dot(xb_s[cb].astype(BF16), w2_s[hb & 1][...], preferred_element_type=F32)
            qb_s[:, 1024 * hb:1024 * hb + 1024] += r
            call(hook, r[:, 7 * DH:])
        return f

    def wuk_mm(cb, hb):
        def f(hook=None):
            for j in range(8):
                h = 8 * hb + j
                q = (qb_s[:, DH * h:DH * h + DH] * scale).astype(BF16)
                r = lax.dot_general(q, w2_s[hb & 1][:, DH * j:DH * j + DH], NT,
                                    preferred_element_type=F32)
                qabs_t[cb, 8 * h:8 * h + NB, :] = r
                if j == 0:
                    r0 = r
            call(hook, r0)
        return f

    def wuv_mm(cb, hb):
        def f(hook=None):
            for j in range(8):
                cc = cc_s[cb, pl.ds(8 * hb + j, NB, stride=NH), :].astype(BF16)
                r = jnp.dot(cc, w2_s[hb & 1][:, DH * j:DH * j + DH], preferred_element_type=F32)
                ctx_s[hb, :, DH * j:DH * j + DH] += r
            call(hook, r)
        return f

    def qabs_finish():
        for b in range(NB):
            for cb in range(4):
                qabs_s[b, :, 128 * cb:128 * cb + 128] = (
                    qabs_t[cb, pl.ds(b, NH, stride=8), :].astype(BF16))

    def c_pieces(sl):
        def cmat(b):
            return mat(bring[sl, 128 * b:128 * b + 128], 4, 0, 4)

        def qk(b):
            def f(hook=None):
                s = lax.dot_general(qabs_s[b], cmat(b), NT, preferred_element_type=F32)
                sb_s[b] = s
                call(hook, s[0:8, 0:DH])
            return f

        def sm(b):
            def f():
                s = sb_s[b]
                m_old = m_s[b]
                m_new = jnp.maximum(m_old, jnp.max(s, axis=-1, keepdims=True))
                alpha = jnp.exp(m_old - m_new)
                ps = [jnp.exp(s[:, 128 * j:128 * j + 128] - m_new) for j in range(CK // 128)]
                l_s[b] = alpha * l_s[b] + sum(ps[1:], ps[0])
                m_s[b] = m_new
                al_s[b] = alpha
                pb_s[b] = jnp.concatenate(ps, axis=-1).astype(BF16)
            return f

        def pv(b):
            def f(hook=None):
                r = jnp.dot(pb_s[b], cmat(b), preferred_element_type=F32)
                al = al_s[b]
                for j in range(4):
                    cols = slice(128 * j, 128 * j + 128)
                    acc_s[b, :, cols] = al * acc_s[b, :, cols] + r[:, cols]
                if hook is not None:
                    keep["v"] = r[0:8, 3 * DH:]
            return f

        keep = {}

        def late(f):
            def g(hook=None):
                f(hook)
                if hook is not None:
                    hook(keep["v"])
            return g

        return [qk(0), both(qk(1), sm(0)), both(qk(2), sm(1)), both(qk(3), sm(2)),
                late(both(sm(3), pv(0), pv(1), host=1)), late(both(pv(2), pv(3)))]

    def c_finish():
        for b in range(NB):
            cc = acc_s[b] / jnp.sum(l_s[b], axis=-1, keepdims=True)
            for cb in range(4):
                cc_s[cb, NH * b:NH * b + NH, :] = cc[:, 128 * cb:128 * cb + 128]

    def wob_mm(sl, cb, half):
        def f(hook=None):
            rs = []
            for i in range(2):
                c0 = 512 * half + 256 * i
                w = mat(bring[sl, c0 // 2:c0 // 2 + 128], 4, 0, 4)
                rs.append(jnp.dot(ctx_s[cb, :, c0:c0 + 256].astype(BF16), w,
                                  preferred_element_type=F32))
            out_s[1, 0:NB, :] += rs[0] + rs[1]
            call(hook, rs[0][:, 3 * DH:])
        return f

    def init():
        wait(x_copies[:1], semx.at[0])
        wait(x_copies[1:], semx.at[1])
        if not do_compute:
            return
        xb = xb_buf[...].astype(F32)
        for cb in range(4):
            xb_s[cb] = xb[:, 128 * cb:128 * cb + 128]
        qb_s[...] = jnp.zeros(qb_s.shape, F32)
        ctx_s[...] = jnp.zeros(ctx_s.shape, F32)
        out_s[...] = jnp.zeros(out_s.shape, F32)
        for r in (ma_s, la_s, acca_s):
            r[...] = jnp.zeros(r.shape, F32)
        m_s[...] = jnp.full(m_s.shape, -jnp.inf, F32)
        l_s[...] = jnp.zeros(l_s.shape, F32)
        acc_s[...] = jnp.zeros(acc_s.shape, F32)

    def wqa_mm(j):
        def f(hook=None):
            r = jnp.dot(xa_buf[...], mat(wqa_buf[...], 32, 4 * j, 4), preferred_element_type=F32) * scale
            for i in range(4):
                h = 4 * j + i
                qa_t[8 * h:8 * h + NB, :] = r[:, DH * i:DH * i + DH]
            call(hook, r[:, 0:DH])
        return f

    def a_qk(g, k):
        def f(hook=None):
            q8 = qa_t[pl.ds(64 * k + (g >> 3), 8, stride=8), :]
            s = None
            for j in range(8):
                qm = jnp.where(row8 == j, q8, 0.0).astype(BF16)
                sj = lax.dot_general(qm, kbuf[g & 1, 8 * k + j], NT, preferred_element_type=F32)
                s = sj if s is None else s + sj
                if j == 0:
                    call(hook, sj)
            sa_s[8 * k:8 * k + 8, :] = s
        return f

    def a_sm(g):
        def f():
            first = (g & 7) == 0
            s = sa_s[...]
            m_old = jnp.where(first, -jnp.inf, ma_s[...])
            m_new = jnp.maximum(m_old, jnp.max(s, axis=-1, keepdims=True))
            alpha = jnp.exp(m_old - m_new)
            p = jnp.exp(s - m_new)
            la_s[...] = jnp.where(first, p, alpha * la_s[...] + p)
            ma_s[...] = m_new
            aa_s[...] = alpha
            sa_s[...] = p
        return f

    def a_pv(g, k):
        def f(hook=None):
            first = (g & 7) == 0
            for r0 in (16 * k, 16 * k + 8):
                rows = slice(r0, r0 + 8)
                p = sa_s[rows, :].astype(BF16)
                o = None
                for j in range(8):
                    oj = jnp.dot(p, vbuf[g & 1, r0 + j], preferred_element_type=F32)
                    o = oj if o is None else jnp.where(row8 == j, oj, o)
                    if r0 % 16 == 0 and j == 4:
                        call(hook, oj)
                acca_s[rows, :] = jnp.where(first, o, aa_s[rows, :] * acca_s[rows, :] + o)
        return f

    def a_fin(g):
        def f():
            o = acca_s[...] / jnp.sum(la_s[...], axis=-1, keepdims=True)
            oa_t[pl.ds(g >> 3, NH, stride=8), :] = o
        return f

    def woa_dot(h):
        o = oa_t[8 * h:8 * h + NB, :].astype(BF16)
        return jnp.dot(o, mat(woa_buf[64 * h:64 * h + 64], 4, 0, 4), preferred_element_type=F32)

    quads = [(hs, k) for k in (3, 2, 1, 0) for hs in ((0, 4, 8, 12), (16, 20, 24, 28))]

    def quad_lhs():
        for n, (hs, k) in enumerate(quads):
            oq_s[n, 0:NB, :] = jnp.concatenate(
                [oa_t[8 * h:8 * h + NB, 32 * k:32 * k + 32] for h in hs], axis=1)

    def quad_dot(n):
        hs, k = quads[n]
        w = jnp.concatenate([woa_buf[64 * h + RT * k:64 * h + RT * k + RT] for h in hs], axis=0)
        return jnp.dot(oq_s[n, 0:NB, :].astype(BF16), mat(w, 4, 0, 4), preferred_element_type=F32)

    def woa_mm(dot, items):
        def f():
            r = dot(items[0])
            for i in items[1:]:
                r = r + dot(i)
            out_s[0, 0:NB, :] += r
        return f

    def static_ticks(waits, starts1, starts0, comp):
        for t, (descs, sem) in enumerate(waits):
            wait(descs, sem)
            for d, s in starts0.get(t, ()):
                start(d, s, 0)
            for d, s in starts1.get(t, ()):
                start(d, s, 1)
            for f in comp.get(t, ()):
                f()

    pre0 = CFG["pre0"]
    x_copies = [(xa_hbm, xa_buf), (xb_hbm, xb_buf)]
    qr = [a_run(wqa_hbm, wqa_buf, RT * ((x + CFG["qoff"]) % 128), 0, 2048)
          for x in _xor_order(CFG["qbasis"])]
    q1 = [qr[i] + qr[i + 1] for i in range(0, 128, 2) if i % 6 != 4]
    q0 = [qr[i] for i in range(128) if i % 6 >= 4]
    for j in range(D1):
        start(q1[j], sem1.at[1], 1)
        if j < pre0:
            start(q0[j], sem0.at[1], 0)
    start(x_copies[:1], semx.at[0], 0)
    start(x_copies[1:], semx.at[1], 0)
    s1, s0, cm = {}, {}, {}
    for t, d in enumerate(q1[D1:]):
        at(s1, t, (d, sem1.at[1]))
    for t in range(D1):
        at(cm, len(q1) - D1 + t, lambda t=t: kv_start(k_hbm, kbuf, 0, t, sem1.at[0]))
    n0 = len(q0) - pre0
    for j in range(n0):
        at(s0, (j * len(q1)) // n0, (q0[pre0 + j], sem0.at[1]))
    at(cm, 4, init)
    static_ticks([(d, sem1.at[1]) for d in q1], s1, s0, cm)

    oruns = [a_run(woa_hbm, woa_buf, 256 * r + RT * k, 256 * r, 256 * r + 256)
             for k in range(15, -1, -1) for r in range(8)]
    o1, o0, o_end = [], [], []
    for i, pat in enumerate(CFG["opat"]):
        lo = [oruns.pop(0) for _ in pat]
        ones = [r for r, c in zip(lo, pat) if c == "1"]
        o0.append([(len(o1) + pat[:n].count("1") // 2, r)
                   for n, (r, c) in enumerate(zip(lo, pat)) if c == "0"])
        o1 += [(ones[n] + ones[n + 1], semt.at[0, i]) for n in range(0, len(ones), 2)]
        o_end.append(len(o1) - 1)
    assert not oruns

    b_slots = CFG["b_slots"]
    a_slots = CFG["a_slots"]

    def body(g, g_lo, g_hi):
        def between(lo, hi):
            if lo <= g_lo and g_hi <= hi:
                return True
            if hi < g_lo or g_hi < lo:
                return False
            if lo <= g_lo:
                return g <= hi
            if g_hi <= hi:
                return g >= lo
            return jnp.logical_and(g >= lo, g <= hi)

        def either(x, y):
            if x is True or y is True:
                return True
            if x is False or y is False:
                return y if x is False else x
            return jnp.logical_or(x, y)

        par = g & 1
        iw = g & 3
        w_stage = [(between(0, 3), wqb_hbm), (between(4, 7), wuk_hbm),
                   (between(24, 27), wuv_hbm), (between(28, 31), wob_hbm)]
        is_c = between(8, 23)
        ic = (g - 8) & 15
        last = between(NG - 1, NG - 1)
        gn = g + 1 if last is False else (g + 1) & (NG - 1)

        sl, cb = 1 - par, (g + 3) & 3
        cm = {}
        short = [qabs_finish, c_finish]
        if do_compute:
            w3 = either(between(1, 8), between(25, 28))
            for k, hb in ((0, 0), (1, 1), (4, 2), (5, 3)):
                short.append(retile(sl, hb))
                at(cm, b_slots[k], (w3, short[-1]))
            for k, hb in ((2, 0), (6, 2)):
                at(cm, b_slots[k], (between(1, 4), both(wq_mm(cb, hb), wq_mm(cb, hb + 1))))
                at(cm, b_slots[k], (between(25, 28), both(wuv_mm(cb, hb), wuv_mm(cb, hb + 1))))
            for k, hb in ((2, 0), (3, 1), (6, 2), (7, 3)):
                at(cm, b_slots[k], (between(5, 8), wuk_mm(cb, hb)))
            at(cm, b_slots[8], (between(8, 8), qabs_finish))
            for k, f in zip(CFG["c_slots"], c_pieces(sl)):
                at(cm, b_slots[k], (between(9, 24), f))
            at(cm, b_slots[8], (between(24, 24), c_finish))
            for k, half in ((3, 0), (7, 1)):
                at(cm, b_slots[k], (between(29, 31), wob_mm(sl, cb, half)))
            for k, t in enumerate(CFG["q_slots"]):
                at(cm, t, (between(0, 0), wqa_mm(k)))
            for k in range(2):
                at(cm, a_slots[k], (between(1, 31), a_pv(g - 1, k)))
            fin = either(either(between(8, 8), between(16, 16)), between(24, 24))
            short += [a_fin(g - 1), a_sm(g)]
            at(cm, a_slots[1] + 2, (fin, short[-2]))
            for k in range(4):
                at(cm, a_slots[2 + k], (True, a_qk(g, k)))
            at(cm, a_slots[6], (True, short[-1]))

        def also(x, y):
            if x is False or y is False:
                return False
            if x is True or y is True:
                return y if x is True else x
            return jnp.logical_and(x, y)

        def b_start(j, live=True):
            for cond, hbm in w_stage:
                when(also(cond, live), lambda hbm=hbm: start(
                    b_run(hbm, 1, lambda s: 512 * iw, par, j), sem0.at[par], 0))
            when(also(is_c, live), lambda: start(
                b_run(c_hbm, 4, lambda s: 2048 * s + 128 * ic, par, j), sem0.at[par], 0))

        def hook_for(j):
            assert is_c is True or is_c is False
            seg, k = b_pos(4 if is_c else 1, j)
            r = 128 * seg + RT * k + boff

            def hook(v):
                bring[par, r, 0:v.shape[0], :] = v.astype(BF16)
                b_start(j)
            return hook

        embed = CFG["embed"] and not isinstance(g, int)
        hosted = False
        for t in range(32):
            dst = (kbuf if t < 16 else vbuf).at[par, pl.ds(2 * (t % 16), 2)]
            pltpu.make_async_copy(dst, dst, sem1.at[t // 16]).wait()
            if hosted is not True:
                b_start(t, True if hosted is False else jnp.logical_not(hosted))
            if t < 16:
                kv_start(v_hbm, vbuf, g, t, sem1.at[1])
            else:
                if last is not True:
                    kv_start(k_hbm, kbuf, gn, t - 16, sem1.at[0], live=between(0, NG - 2))
                when(last, lambda: start(o1[t - 16][0], o1[t - 16][1], 1))
            if t == bwait:
                when(between(0, 0), lambda: wait(sum(q0, []), sem0.at[1]))
                when(between(1, 31), lambda: wait([(None, bring.at[sl])], sem0.at[sl]))
            hosted = False
            for cond, f in cm.get(t, ()):
                if embed and t < 31 and cond is not False and f not in short:
                    hosted = either(hosted, cond)
                    pl.when(g >= 0 if cond is True else cond)(
                        lambda f=f: f(hook_for(t + 1)))
                else:
                    when(cond, f)

    cuts = CFG["cuts"]
    for lo, hi in zip(cuts[:-1], cuts[1:]):
        if hi - lo == 1:
            body(lo, lo, lo)
        else:
            def loop_body(g, carry, lo=lo, hi=hi):
                body(g, lo, hi - 1)
                return carry
            lax.fori_loop(lo, hi, loop_body, 0)

    s1, s0, cm = {}, {}, {}
    nt = len(o1)
    for t in range(nt - D1):
        at(s1, t, o1[D1 + t])
    la, lb = CFG["olead"]
    for i, grp in enumerate(o0):
        for p, r in grp:
            at(s0, max(0, p - (la + ((lb - la) * p) // nt)), (r, semt.at[1, i]))
        at(cm, o_end[i], lambda i=i, grp=grp: wait(sum((r for _, r in grp), []), semt.at[1, i]))
    at(cm, 7, lambda: wait([(None, bring.at[1])], sem0.at[1]))

    def write_b():
        o_ref[:, DM:2 * DM] = out_s[1, 0:NB, :].astype(o_ref.dtype)

    if do_compute:
        at(cm, 1, a_pv(NG - 1, 0))
        at(cm, 3, a_pv(NG - 1, 1))
        at(cm, 5, a_fin(NG - 1))
        at(cm, 7, wob_mm(1, 3, 0))
        at(cm, 15, both(wob_mm(1, 3, 1), write_b))
        at(cm, 17, quad_lhs)
        for i in range(3):
            at(cm, o_end[i], woa_mm(woa_dot, tuple(range(3 - i, 16, 4))))
            at(cm, o_end[i] + 2, woa_mm(woa_dot, tuple(range(19 - i, 32, 4))))
        n = 0
        for i, pat in list(enumerate(CFG["opat"]))[3:-1]:
            at(cm, o_end[i], woa_mm(quad_dot, tuple(range(n, n + len(pat) // 4))))
            n += len(pat) // 4
    static_ticks(o1, s1, s0, cm)
    if do_compute:
        r = out_s[0, 0:NB, :]
        for i in range(n, 8):
            r = r + quad_dot(i)
        o_ref[:, 0:DM] = r.astype(o_ref.dtype)
    else:
        o_ref[...] = jnp.zeros(o_ref.shape, o_ref.dtype)


def _tiles(x):
    c = x.shape[-1]
    return x.reshape(-1, 8, c // DH, DH).transpose(0, 2, 1, 3).reshape(-1, 8, DH)


@jax.jit
def pallas_concat_heads__sliding_block_cached__compressed_kv_cla__decode_kernel(
    A_x: jax.Array,
    A_k_cache: jax.Array,
    A_v_cache: jax.Array,
    A_wq: jax.Array,
    A_wo: jax.Array,
    B_x: jax.Array,
    B_c_kv: jax.Array,
    B_w_q: jax.Array,
    B_w_uk: jax.Array,
    B_w_uv: jax.Array,
    B_w_o: jax.Array,
):
    assert A_x.shape == (NB, 1, DM) and B_x.shape == (NB, 1, DM)
    assert A_k_cache.shape == (NB, NH, SK, DH) and B_c_kv.shape == (NB, SK, DM)
    vm = pltpu.VMEM
    out = pl.pallas_call(
        _kernel,
        out_shape=jax.ShapeDtypeStruct((NB, 2 * DM), A_x.dtype),
        in_specs=[pl.BlockSpec(memory_space=pl.ANY)] * 11,
        out_specs=pl.BlockSpec(memory_space=pltpu.VMEM),
        scratch_shapes=[
            vm((NB, DM), BF16), vm((NB, DM), BF16),
            vm((2, NH, RUN, DH), BF16), vm((2, NH, RUN, DH), BF16),
            vm((2048, 8, DH), BF16), vm((2048, 8, DH), BF16),
            vm((2, 512, 8, DH), BF16),
            vm((4, NB, 128), F32),
            vm((NH * 8, DH), F32),
            vm((NH * 8, DH), F32),
            vm((NH, RUN), F32),
            vm((NH, DH), F32), vm((NH, DH), F32),
            vm((NH, DH), F32), vm((NH, DH), F32),
            vm((NB, NH * DH), F32),
            vm((4, NH * 8, 128), F32),
            vm((NB, NH, DM), BF16),
            vm((NB, NH, CK), F32),
            vm((NB, NH, CK), BF16),
            vm((NB, NH, 128), F32),
            vm((NB, NH, 128), F32), vm((NB, NH, 128), F32),
            vm((NB, NH, DM), F32),
            vm((4, NB * NH, 128), F32),
            vm((4, NB, 8 * DH), F32),
            vm((2, 8, DM), F32),
            vm((8, 8, DH), F32),
            vm((128, 8 * DH), BF16), vm((128, 8 * DH), BF16),
            pltpu.SemaphoreType.DMA((2,)), pltpu.SemaphoreType.DMA((2,)),
            pltpu.SemaphoreType.DMA((2,)), pltpu.SemaphoreType.DMA((2, len(CFG["opat"]))),
        ],
        compiler_params=pltpu.CompilerParams(
            vmem_limit_bytes=48 * 1024 * 1024,
            disable_bounds_checks=not CFG["checks"],
            disable_semaphore_checks=not CFG["checks"],
        ),
        name="concat_heads_decode",
    )(
        A_x.reshape(NB, DM), B_x.reshape(NB, DM), A_k_cache, A_v_cache,
        _tiles(A_wq), _tiles(A_wo), _tiles(B_c_kv),
        _tiles(B_w_q), _tiles(B_w_uk), _tiles(B_w_uv), _tiles(B_w_o),
    )
    return out.reshape(NB, 1, 2 * DM)
```

```python
import jax
import jax.numpy as jnp
from jax import lax
import jax.experimental.pallas as pl
import jax.experimental.pallas.tpu as pltpu

F32 = jnp.float32
BF16 = jnp.bfloat16

NB = 4
NH = 32
DH = 128
DM = 512
SK = 4096
WIN = 1024
CK = 256
NG = 32
RUN = 128
RT = 16
D1 = 16
NT = ((1,), (1,)), ((), ())

CFG = dict(
    compute=True, checks=False,
    aoff=1, boff=1,
    hbasis=(16, 15, 3, 4, 1), hoff=0, wbasis=(1, 31, 8, 5, 6), cbasis=(8, 16, 1, 3, 6), koff=1,
    qbasis=(1, 86, 105, 20, 15, 100, 98), qoff=65,
    pre0=6,
    opat=("110" * 10 + "11", "011" * 10 + "11", "011" * 10 + "11", "011" * 5 + "0",
          "11011011", "1111", "1111"),
    olead=(6, 8),
    cuts=(0, 8, 24, 32),
    embed=True,
    bwait=6,
    a_slots=(1, 3, 16, 18, 20, 22, 24), b_slots=(6, 8, 10, 12, 14, 26, 28, 30, 31),
    c_slots=(0, 1, 2, 3, 5, 6), q_slots=(6, 8, 10, 12, 14, 15, 17, 19),
)


def _xor_order(basis):
    out = [0]
    for v in basis:
        out += [x ^ v for x in out]
    assert sorted(out) == list(range(len(out)))
    return out


def _mult(x, m):
    return x if isinstance(x, int) else pl.multiple_of(x, m)


def _kernel(xa_hbm, xb_hbm, k_hbm, v_hbm, wqa_hbm, woa_hbm, c_hbm, wqb_hbm, wuk_hbm,
            wuv_hbm, wob_hbm, o_ref,
            xa_buf, xb_buf, kbuf, vbuf, wqa_buf, woa_buf, bring,
            xb_s, qa_t, oa_t, sa_s, ma_s, la_s, aa_s, acca_s, qb_s, qabs_t, qabs_s, sb_s, pb_s, al_s,
            m_s, l_s, acc_s, cc_s, ctx_s, out_s, oq_s, w2a_s, w2b_s,
            sem1, sem0, semx, semt):
    do_compute = CFG["compute"]
    aoff, boff = CFG["aoff"], CFG["boff"]
    bwait = CFG["bwait"]
    scale = DH ** -0.5
    w2_s = (w2a_s, w2b_s)
    h_order = [(x + CFG["hoff"]) % NH for x in _xor_order(CFG["hbasis"])]
    w_order = [(x + CFG["koff"]) % 32 for x in _xor_order(CFG["wbasis"])]
    c_order = [(x & 24) + (x + CFG["koff"]) % 8 for x in _xor_order(CFG["cbasis"])]
    row8 = lax.broadcasted_iota(jnp.int32, (8, DH), 0)

    def start(descs, sem, prio):
        for src, dst in descs:
            pltpu.make_async_copy(src, dst, sem).start(priority=prio)

    def wait(descs, sem):
        for _, dst in descs:
            pltpu.make_async_copy(dst, dst, sem).wait()

    def at(d, t, item):
        d.setdefault(t, []).append(item)

    def both(*fs, host=0):
        def f(hook=None):
            for i, g in enumerate(fs):
                if i == host:
                    g(hook)
                else:
                    g()
        return f

    def call(hook, v):
        if hook is not None:
            hook(v)

    def mat(w, ncol, j0, n):
        w = w.reshape(w.shape[0] // ncol, ncol, 8, DH)
        cols = [w[:, j0 + j].reshape(w.shape[0] * 8, DH) for j in range(n)]
        return jnp.concatenate(cols, axis=1)

    def when(cond, f):
        if cond is True:
            f()
        elif cond is not False:
            pl.when(cond)(f)

    def kv_start(hbm, buf, g, t, sem, live=True):
        b, sl = g >> 3, g & 7
        ko = 8 * aoff
        w0 = SK - WIN
        heads = h_order[2 * t:2 * t + 2]
        row = _mult(w0 + RUN * sl - ko, 8)
        reg = [(hbm.at[b, h, pl.ds(row, RUN)], buf.at[g & 1, h]) for h in heads]
        if ko == 0:
            when(live, lambda: start(reg, sem, 1))
            return
        fst = [(hbm.at[b, h, pl.ds(w0, RUN - ko)], buf.at[g & 1, h, pl.ds(ko, RUN - ko)])
               for h in heads]
        if t == 0:
            fst = [(hbm.at[b, :, pl.ds(SK - ko, ko)], buf.at[g & 1, :, pl.ds(0, ko)])] + fst
        if isinstance(sl, int):
            when(live, lambda: start(reg if sl else fst, sem, 1))
        else:
            pl.when(sl > 0)(lambda: start(reg, sem, 1))
            first = sl == 0
            pl.when(first if live is True else jnp.logical_and(first, live))(
                lambda: start(fst, sem, 1))

    def b_pos(nseg, t):
        return divmod((c_order if nseg == 4 else w_order)[t], 32 // nseg)

    def b_run(hbm, nseg, src, sl, t):
        seg, k = b_pos(nseg, t)
        ln = 512 // nseg
        r = boff + RT * k
        n = min(RT, ln - r)
        out = [(hbm.at[pl.ds(src(seg) + r, n)], bring.at[sl, pl.ds(ln * seg + r, n)])]
        if k == 0 and boff:
            out.append((hbm.at[pl.ds(src(seg), boff)], bring.at[sl, pl.ds(ln * seg, boff)]))
        return out

    def a_run(hbm, buf, r, lo, hi):
        r0, r1 = max(r - aoff, lo), (hi if r + RT == hi else r + RT - aoff)
        return [(hbm.at[pl.ds(r0, r1 - r0)], buf.at[pl.ds(r0, r1 - r0)])]

    def retile(sl, hb):
        def f():
            w = bring[sl].reshape(128, 4, 8, DH)[:, hb]
            w2_s[hb & 1][...] = w.reshape(128, 8 * DH)
        return f

    def wq_mm(cb, hb):
        def f(hook=None):
            r = jnp.dot(xb_s[cb].astype(BF16), w2_s[hb & 1][...], preferred_element_type=F32)
            qb_s[:, 1024 * hb:1024 * hb + 1024] += r
            call(hook, r[:, 7 * DH:])
        return f

    def wuk_mm(cb, hb):
        def f(hook=None):
            for j in range(8):
                h = 8 * hb + j
                q = (qb_s[:, DH * h:DH * h + DH] * scale).astype(BF16)
                r = lax.dot_general(q, w2_s[hb & 1][:, DH * j:DH * j + DH], NT,
                                    preferred_element_type=F32)
                qabs_t[cb, 8 * h:8 * h + NB, :] = r
                if j == 0:
                    r0 = r
            call(hook, r0)
        return f

    def wuv_mm(cb, hb):
        def f(hook=None):
            for j in range(8):
                cc = cc_s[cb, pl.ds(8 * hb + j, NB, stride=NH), :].astype(BF16)
                r = jnp.dot(cc, w2_s[hb & 1][:, DH * j:DH * j + DH], preferred_element_type=F32)
                ctx_s[hb, :, DH * j:DH * j + DH] += r
            call(hook, r)
        return f

    def qabs_finish():
        for b in range(NB):
            for cb in range(4):
                qabs_s[b, :, 128 * cb:128 * cb + 128] = (
                    qabs_t[cb, pl.ds(b, NH, stride=8), :].astype(BF16))

    def c_pieces(sl):
        def cmat(b):
            return mat(bring[sl, 128 * b:128 * b + 128], 4, 0, 4)

        def qk(b):
            def f(hook=None):
                s = lax.dot_general(qabs_s[b], cmat(b), NT, preferred_element_type=F32)
                sb_s[b] = s
                call(hook, s[0:8, 0:DH])
            return f

        def sm(b):
            def f():
                s = sb_s[b]
                m_old = m_s[b]
                m_new = jnp.maximum(m_old, jnp.max(s, axis=-1, keepdims=True))
                alpha = jnp.exp(m_old - m_new)
                ps = [jnp.exp(s[:, 128 * j:128 * j + 128] - m_new) for j in range(CK // 128)]
                l_s[b] = alpha * l_s[b] + sum(ps[1:], ps[0])
                m_s[b] = m_new
                al_s[b] = alpha
                pb_s[b] = jnp.concatenate(ps, axis=-1).astype(BF16)
            return f

        def pv(b):
            def f(hook=None):
                r = jnp.dot(pb_s[b], cmat(b), preferred_element_type=F32)
                al = al_s[b]
                for j in range(4):
                    cols = slice(128 * j, 128 * j + 128)
                    acc_s[b, :, cols] = al * acc_s[b, :, cols] + r[:, cols]
                if hook is not None:
                    keep["v"] = r[0:8, 3 * DH:]
            return f

        keep = {}

        def late(f):
            def g(hook=None):
                f(hook)
                if hook is not None:
                    hook(keep["v"])
            return g

        return [qk(0), both(qk(1), sm(0)), both(qk(2), sm(1)), both(qk(3), sm(2)),
                late(both(sm(3), pv(0), pv(1), host=1)), late(both(pv(2), pv(3)))]

    def c_finish():
        for b in range(NB):
            cc = acc_s[b] / jnp.sum(l_s[b], axis=-1, keepdims=True)
            for cb in range(4):
                cc_s[cb, NH * b:NH * b + NH, :] = cc[:, 128 * cb:128 * cb + 128]

    def wob_mm(sl, cb, half):
        def f(hook=None):
            rs = []
            for i in range(2):
                c0 = 512 * half + 256 * i
                w = mat(bring[sl, c0 // 2:c0 // 2 + 128], 4, 0, 4)
                rs.append(jnp.dot(ctx_s[cb, :, c0:c0 + 256].astype(BF16), w,
                                  preferred_element_type=F32))
            out_s[1, 0:NB, :] += rs[0] + rs[1]
            call(hook, rs[0][:, 3 * DH:])
        return f

    def init():
        wait(x_copies[:1], semx.at[0])
        wait(x_copies[1:], semx.at[1])
        if not do_compute:
            return
        xb = xb_buf[...].astype(F32)
        for cb in range(4):
            xb_s[cb] = xb[:, 128 * cb:128 * cb + 128]
        qb_s[...] = jnp.zeros(qb_s.shape, F32)
        ctx_s[...] = jnp.zeros(ctx_s.shape, F32)
        out_s[...] = jnp.zeros(out_s.shape, F32)
        for r in (ma_s, la_s, acca_s):
            r[...] = jnp.zeros(r.shape, F32)
        m_s[...] = jnp.full(m_s.shape, -jnp.inf, F32)
        l_s[...] = jnp.zeros(l_s.shape, F32)
        acc_s[...] = jnp.zeros(acc_s.shape, F32)

    def wqa_mm(j):
        def f(hook=None):
            w = mat(wqa_buf[...], 32, 4 * j, 4)
            r = jnp.dot(xa_buf[...], w, preferred_element_type=F32) * scale
            for i in range(4):
                h = 4 * j + i
                qa_t[8 * h:8 * h + NB, :] = r[:, DH * i:DH * i + DH]
            call(hook, r[:, 0:DH])
        return f

    def a_qk(g, k):
        def f(hook=None):
            q8 = qa_t[pl.ds(64 * k + (g >> 3), 8, stride=8), :]
            s = None
            for j in range(8):
                qm = jnp.where(row8 == j, q8, 0.0).astype(BF16)
                sj = lax.dot_general(qm, kbuf[g & 1, 8 * k + j], NT, preferred_element_type=F32)
                s = sj if s is None else s + sj
                if j == 0:
                    call(hook, sj)
            sa_s[8 * k:8 * k + 8, :] = s
        return f

    def a_sm(g):
        def f():
            first = (g & 7) == 0
            s = sa_s[...]
            m_old = jnp.where(first, -jnp.inf, ma_s[...])
            m_new = jnp.maximum(m_old, jnp.max(s, axis=-1, keepdims=True))
            alpha = jnp.exp(m_old - m_new)
            p = jnp.exp(s - m_new)
            la_s[...] = jnp.where(first, p, alpha * la_s[...] + p)
            ma_s[...] = m_new
            aa_s[...] = alpha
            sa_s[...] = p
        return f

    def a_pv(g, k):
        def f(hook=None):
            first = (g & 7) == 0
            for r0 in (16 * k, 16 * k + 8):
                rows = slice(r0, r0 + 8)
                p = sa_s[rows, :].astype(BF16)
                o = None
                for j in range(8):
                    oj = jnp.dot(p, vbuf[g & 1, r0 + j], preferred_element_type=F32)
                    o = oj if o is None else jnp.where(row8 == j, oj, o)
                    if r0 % 16 == 0 and j == 4:
                        call(hook, oj)
                acca_s[rows, :] = jnp.where(first, o, aa_s[rows, :] * acca_s[rows, :] + o)
        return f

    def a_fin(g):
        def f():
            o = acca_s[...] / jnp.sum(la_s[...], axis=-1, keepdims=True)
            oa_t[pl.ds(g >> 3, NH, stride=8), :] = o
        return f

    def woa_dot(h):
        o = oa_t[8 * h:8 * h + NB, :].astype(BF16)
        return jnp.dot(o, mat(woa_buf[64 * h:64 * h + 64], 4, 0, 4), preferred_element_type=F32)

    quads = [(hs, k) for k in (3, 2, 1, 0) for hs in ((0, 4, 8, 12), (16, 20, 24, 28))]

    def quad_lhs():
        for n, (hs, k) in enumerate(quads):
            oq_s[n, 0:NB, :] = jnp.concatenate(
                [oa_t[8 * h:8 * h + NB, 32 * k:32 * k + 32] for h in hs], axis=1)

    def quad_dot(n):
        hs, k = quads[n]
        w = jnp.concatenate([woa_buf[64 * h + RT * k:64 * h + RT * k + RT] for h in hs], axis=0)
        return jnp.dot(oq_s[n, 0:NB, :].astype(BF16), mat(w, 4, 0, 4), preferred_element_type=F32)

    def woa_mm(dot, items):
        def f():
            r = dot(items[0])
            for i in items[1:]:
                r = r + dot(i)
            out_s[0, 0:NB, :] += r
        return f

    def static_ticks(waits, starts1, starts0, comp):
        for t, (descs, sem) in enumerate(waits):
            wait(descs, sem)
            for d, s in starts0.get(t, ()):
                start(d, s, 0)
            for d, s in starts1.get(t, ()):
                start(d, s, 1)
            for f in comp.get(t, ()):
                f()

    pre0 = CFG["pre0"]
    x_copies = [(xa_hbm, xa_buf), (xb_hbm, xb_buf)]
    qr = [a_run(wqa_hbm, wqa_buf, RT * ((x + CFG["qoff"]) % 128), 0, 2048)
          for x in _xor_order(CFG["qbasis"])]
    q1 = [qr[i] + qr[i + 1] for i in range(0, 128, 2) if i % 6 != 4]
    q0 = [qr[i] for i in range(128) if i % 6 >= 4]
    for j in range(D1):
        start(q1[j], sem1.at[1], 1)
        if j < pre0:
            start(q0[j], sem0.at[1], 0)
    start(x_copies[:1], semx.at[0], 0)
    start(x_copies[1:], semx.at[1], 0)
    s1, s0, cm = {}, {}, {}
    for t, d in enumerate(q1[D1:]):
        at(s1, t, (d, sem1.at[1]))
    for t in range(D1):
        at(cm, len(q1) - D1 + t, lambda t=t: kv_start(k_hbm, kbuf, 0, t, sem1.at[0]))
    n0 = len(q0) - pre0
    for j in range(n0):
        at(s0, (j * len(q1)) // n0, (q0[pre0 + j], sem0.at[1]))
    at(cm, 4, init)
    static_ticks([(d, sem1.at[1]) for d in q1], s1, s0, cm)

    oruns = [a_run(woa_hbm, woa_buf, 256 * r + RT * k, 256 * r, 256 * r + 256)
             for k in range(15, -1, -1) for r in range(8)]
    o1, o0, o_end = [], [], []
    for i, pat in enumerate(CFG["opat"]):
        lo = [oruns.pop(0) for _ in pat]
        ones = [r for r, c in zip(lo, pat) if c == "1"]
        o0.append([(len(o1) + pat[:n].count("1") // 2, r)
                   for n, (r, c) in enumerate(zip(lo, pat)) if c == "0"])
        o1 += [(ones[n] + ones[n + 1], semt.at[0, i]) for n in range(0, len(ones), 2)]
        o_end.append(len(o1) - 1)
    assert not oruns

    b_slots = CFG["b_slots"]
    a_slots = CFG["a_slots"]

    def body(g, g_lo, g_hi):
        def between(lo, hi):
            if lo <= g_lo and g_hi <= hi:
                return True
            if hi < g_lo or g_hi < lo:
                return False
            if lo <= g_lo:
                return g <= hi
            if g_hi <= hi:
                return g >= lo
            return jnp.logical_and(g >= lo, g <= hi)

        def either(x, y):
            if x is True or y is True:
                return True
            if x is False or y is False:
                return y if x is False else x
            return jnp.logical_or(x, y)

        par = g & 1
        iw = g & 3
        w_stage = [(between(0, 3), wqb_hbm), (between(4, 7), wuk_hbm),
                   (between(24, 27), wuv_hbm), (between(28, 31), wob_hbm)]
        is_c = between(8, 23)
        ic = (g - 8) & 15
        last = between(NG - 1, NG - 1)
        gn = g + 1 if last is False else (g + 1) & (NG - 1)

        sl, cb = 1 - par, (g + 3) & 3
        cm = {}
        short = [qabs_finish, c_finish]
        if do_compute:
            w3 = either(between(1, 8), between(25, 28))
            for k, hb in ((0, 0), (1, 1), (4, 2), (5, 3)):
                short.append(retile(sl, hb))
                at(cm, b_slots[k], (w3, short[-1]))
            for k, hb in ((2, 0), (6, 2)):
                at(cm, b_slots[k], (between(1, 4), both(wq_mm(cb, hb), wq_mm(cb, hb + 1))))
                at(cm, b_slots[k], (between(25, 28), both(wuv_mm(cb, hb), wuv_mm(cb, hb + 1))))
            for k, hb in ((2, 0), (3, 1), (6, 2), (7, 3)):
                at(cm, b_slots[k], (between(5, 8), wuk_mm(cb, hb)))
            at(cm, b_slots[8], (between(8, 8), qabs_finish))
            for k, f in zip(CFG["c_slots"], c_pieces(sl)):
                at(cm, b_slots[k], (between(9, 24), f))
            at(cm, b_slots[8], (between(24, 24), c_finish))
            for k, half in ((3, 0), (7, 1)):
                at(cm, b_slots[k], (between(29, 31), wob_mm(sl, cb, half)))
            for k, t in enumerate(CFG["q_slots"]):
                at(cm, t, (between(0, 0), wqa_mm(k)))
            for k in range(2):
                at(cm, a_slots[k], (between(1, 31), a_pv(g - 1, k)))
            fin = either(either(between(8, 8), between(16, 16)), between(24, 24))
            short += [a_fin(g - 1), a_sm(g)]
            at(cm, a_slots[1] + 2, (fin, short[-2]))
            for k in range(4):
                at(cm, a_slots[2 + k], (True, a_qk(g, k)))
            at(cm, a_slots[6], (True, short[-1]))

        def also(x, y):
            if x is False or y is False:
                return False
            if x is True or y is True:
                return y if x is True else x
            return jnp.logical_and(x, y)

        def b_start(j, live=True):
            for cond, hbm in w_stage:
                when(also(cond, live), lambda hbm=hbm: start(
                    b_run(hbm, 1, lambda s: 512 * iw, par, j), sem0.at[par], 0))
            when(also(is_c, live), lambda: start(
                b_run(c_hbm, 4, lambda s: 2048 * s + 128 * ic, par, j), sem0.at[par], 0))

        def hook_for(j):
            assert is_c is True or is_c is False
            seg, k = b_pos(4 if is_c else 1, j)
            r = 128 * seg + RT * k + boff

            def hook(v):
                bring[par, r, 0:v.shape[0], :] = v.astype(BF16)
                b_start(j)
            return hook

        embed = CFG["embed"] and not isinstance(g, int)
        hosted = False
        for t in range(32):
            dst = (kbuf if t < 16 else vbuf).at[par, pl.ds(2 * (t % 16), 2)]
            pltpu.make_async_copy(dst, dst, sem1.at[t // 16]).wait()
            if hosted is not True:
                b_start(t, True if hosted is False else jnp.logical_not(hosted))
            if t < 16:
                kv_start(v_hbm, vbuf, g, t, sem1.at[1])
            else:
                if last is not True:
                    kv_start(k_hbm, kbuf, gn, t - 16, sem1.at[0], live=between(0, NG - 2))
                when(last, lambda: start(o1[t - 16][0], o1[t - 16][1], 1))
            if t == bwait:
                when(between(0, 0), lambda: wait(sum(q0, []), sem0.at[1]))
                when(between(1, 31), lambda: wait([(None, bring.at[sl])], sem0.at[sl]))
            hosted = False
            for cond, f in cm.get(t, ()):
                if embed and t < 31 and cond is not False and f not in short:
                    hosted = either(hosted, cond)
                    pl.when(g >= 0 if cond is True else cond)(
                        lambda f=f: f(hook_for(t + 1)))
                else:
                    when(cond, f)

    cuts = CFG["cuts"]
    for lo, hi in zip(cuts[:-1], cuts[1:]):
        if hi - lo == 1:
            body(lo, lo, lo)
        else:
            def loop_body(g, carry, lo=lo, hi=hi):
                body(g, lo, hi - 1)
                return carry
            lax.fori_loop(lo, hi, loop_body, 0)

    s1, s0, cm = {}, {}, {}
    nt = len(o1)
    for t in range(nt - D1):
        at(s1, t, o1[D1 + t])
    la, lb = CFG["olead"]
    for i, grp in enumerate(o0):
        for p, r in grp:
            at(s0, max(0, p - (la + ((lb - la) * p) // nt)), (r, semt.at[1, i]))
        at(cm, o_end[i], lambda i=i, grp=grp: wait(sum((r for _, r in grp), []), semt.at[1, i]))
    at(cm, 7, lambda: wait([(None, bring.at[1])], sem0.at[1]))

    def write_b():
        o_ref[:, DM:2 * DM] = out_s[1, 0:NB, :].astype(o_ref.dtype)

    if do_compute:
        at(cm, 1, a_pv(NG - 1, 0))
        at(cm, 3, a_pv(NG - 1, 1))
        at(cm, 5, a_fin(NG - 1))
        at(cm, 7, wob_mm(1, 3, 0))
        at(cm, 15, both(wob_mm(1, 3, 1), write_b))
        at(cm, 17, quad_lhs)
        for i in range(3):
            at(cm, o_end[i], woa_mm(woa_dot, tuple(range(3 - i, 16, 4))))
            at(cm, o_end[i] + 2, woa_mm(woa_dot, tuple(range(19 - i, 32, 4))))
        n = 0
        for i, pat in list(enumerate(CFG["opat"]))[3:-1]:
            at(cm, o_end[i], woa_mm(quad_dot, tuple(range(n, n + len(pat) // 4))))
            n += len(pat) // 4
    static_ticks(o1, s1, s0, cm)
    if do_compute:
        r = out_s[0, 0:NB, :]
        for i in range(n, 8):
            r = r + quad_dot(i)
        o_ref[:, 0:DM] = r.astype(o_ref.dtype)
    else:
        o_ref[...] = jnp.zeros(o_ref.shape, o_ref.dtype)


def _tiles(x):
    c = x.shape[-1]
    return x.reshape(-1, 8, c // DH, DH).transpose(0, 2, 1, 3).reshape(-1, 8, DH)


def _compiler_params():
    kw = dict(vmem_limit_bytes=48 * 1024 * 1024, disable_bounds_checks=not CFG["checks"])
    try:
        return pltpu.CompilerParams(disable_semaphore_checks=not CFG["checks"], **kw)
    except TypeError:
        return pltpu.CompilerParams(**kw)


@jax.jit
def pallas_concat_heads__sliding_block_cached__compressed_kv_cla__decode_kernel(
    A_x: jax.Array,
    A_k_cache: jax.Array,
    A_v_cache: jax.Array,
    A_wq: jax.Array,
    A_wo: jax.Array,
    B_x: jax.Array,
    B_c_kv: jax.Array,
    B_w_q: jax.Array,
    B_w_uk: jax.Array,
    B_w_uv: jax.Array,
    B_w_o: jax.Array,
):
    assert A_x.shape == (NB, 1, DM) and B_x.shape == (NB, 1, DM)
    assert A_k_cache.shape == (NB, NH, SK, DH) and B_c_kv.shape == (NB, SK, DM)
    vm = pltpu.VMEM
    out = pl.pallas_call(
        _kernel,
        out_shape=jax.ShapeDtypeStruct((NB, 2 * DM), A_x.dtype),
        in_specs=[pl.BlockSpec(memory_space=pl.ANY)] * 11,
        out_specs=pl.BlockSpec(memory_space=pltpu.VMEM),
        scratch_shapes=[
            vm((NB, DM), BF16), vm((NB, DM), BF16),
            vm((2, NH, RUN, DH), BF16), vm((2, NH, RUN, DH), BF16),
            vm((2048, 8, DH), BF16), vm((2048, 8, DH), BF16),
            vm((2, 512, 8, DH), BF16),
            vm((4, NB, 128), F32),
            vm((NH * 8 + 8, DH), F32),
            vm((NH * 8 + 8, DH), F32),
            vm((NH, RUN), F32),
            vm((NH, DH), F32), vm((NH, DH), F32),
            vm((NH, DH), F32), vm((NH, DH), F32),
            vm((NB, NH * DH), F32),
            vm((4, NH * 8 + 8, 128), F32),
            vm((NB, NH, DM), BF16),
            vm((NB, NH, CK), F32),
            vm((NB, NH, CK), BF16),
            vm((NB, NH, 128), F32),
            vm((NB, NH, 128), F32), vm((NB, NH, 128), F32),
            vm((NB, NH, DM), F32),
            vm((4, NB * NH + NH, 128), F32),
            vm((4, NB, 8 * DH), F32),
            vm((2, 8, DM), F32),
            vm((8, 8, DH), F32),
            vm((128, 8 * DH), BF16), vm((128, 8 * DH), BF16),
            pltpu.SemaphoreType.DMA((2,)), pltpu.SemaphoreType.DMA((2,)),
            pltpu.SemaphoreType.DMA((2,)), pltpu.SemaphoreType.DMA((2, len(CFG["opat"]))),
        ],
        compiler_params=_compiler_params(),
        name="concat_heads_decode",
    )(
        A_x.reshape(NB, DM), B_x.reshape(NB, DM), A_k_cache, A_v_cache,
        _tiles(A_wq), _tiles(A_wo), _tiles(B_c_kv),
        _tiles(B_w_q), _tiles(B_w_uk), _tiles(B_w_uv), _tiles(B_w_o),
    )
    return out.reshape(NB, 1, 2 * DM)
```

```python
import jax
import jax.numpy as jnp
from jax import lax
import jax.experimental.pallas as pl
import jax.experimental.pallas.tpu as pltpu

F32 = jnp.float32
BF16 = jnp.bfloat16

NB = 4
NH = 32
DH = 128
DM = 512
SK = 4096
WIN = 1024
CK = 256
NG = 32
RUN = 128
RT = 16
D1 = 16
NT = ((1,), (1,)), ((), ())

CFG = dict(
    compute=True, checks=False,
    aoff=1, boff=1,
    hbasis=(15, 3, 4, 1), wbasis=(1, 31, 8, 5, 6), cbasis=(8, 16, 1, 3, 6), koff=1,
    qbasis=(1, 86, 105, 20, 15, 100, 98), qoff=65,
    pre0=6,
    opat=("110" * 10 + "11", "011" * 10 + "11", "011" * 10 + "11", "011" * 5 + "0",
          "11011011", "1111", "1111"),
    olead=(6, 8),
    cuts=(0, 8, 24, 32),
    embed=True,
    bwait=6,
    a_slots=(1, 3, 16, 18, 20, 22, 24), b_slots=(6, 8, 10, 12, 14, 26, 28, 30, 31),
    c_slots=(0, 1, 2, 3, 5, 6), q_slots=(6, 8, 10, 12, 14, 15, 17, 19),
)


def _xor_order(basis):
    out = [0]
    for v in basis:
        out += [x ^ v for x in out]
    assert sorted(out) == list(range(len(out)))
    return out


def _mult(x, m):
    return x if isinstance(x, int) else pl.multiple_of(x, m)


def _kernel(xa_hbm, xb_hbm, k_hbm, v_hbm, wqa_hbm, woa_hbm, c_hbm, wqb_hbm, wuk_hbm,
            wuv_hbm, wob_hbm, o_ref,
            xa_buf, xb_buf, kbuf, vbuf, wqa_buf, woa_buf, bring,
            xb_s, qa_t, oa_t, sa_s, ma_s, la_s, aa_s, acca_s, qb_s, qabs_t, qabs_s, sb_s, pb_s, al_s,
            m_s, l_s, acc_s, cc_s, ctx_s, out_s, oq_s, w2a_s, w2b_s,
            sem1, sem0, semx, semt):
    do_compute = CFG["compute"]
    aoff, boff = CFG["aoff"], CFG["boff"]
    bwait = CFG["bwait"]
    scale = DH ** -0.5
    w2_s = (w2a_s, w2b_s)
    h_order = _xor_order(CFG["hbasis"])
    w_order = [(x + CFG["koff"]) % 32 for x in _xor_order(CFG["wbasis"])]
    c_order = [(x & 24) + (x + CFG["koff"]) % 8 for x in _xor_order(CFG["cbasis"])]
    row8 = lax.broadcasted_iota(jnp.int32, (8, DH), 0)

    def start(descs, sem, prio):
        for src, dst in descs:
            pltpu.make_async_copy(src, dst, sem).start(priority=prio)

    def wait(descs, sem):
        for _, dst in descs:
            pltpu.make_async_copy(dst, dst, sem).wait()

    def at(d, t, item):
        d.setdefault(t, []).append(item)

    def both(*fs, host=0):
        def f(hook=None):
            for i, g in enumerate(fs):
                if i == host:
                    g(hook)
                else:
                    g()
        return f

    def call(hook, v):
        if hook is not None:
            hook(v)

    def mat(w, ncol, j0, n):
        w = w.reshape(w.shape[0] // ncol, ncol, 8, DH)
        cols = [w[:, j0 + j].reshape(w.shape[0] * 8, DH) for j in range(n)]
        return jnp.concatenate(cols, axis=1)

    def when(cond, f):
        if cond is True:
            f()
        elif cond is not False:
            pl.when(cond)(f)

    def kv_start(hbm, buf, g, t, sem, live=True):
        b, sl = g >> 3, g & 7
        ko = 8 * aoff
        w0 = SK - WIN
        h = h_order[t]
        row = _mult(w0 + RUN * sl - ko, 8)
        reg = [(hbm.at[b, :, h, pl.ds(row, RUN)], buf.at[g & 1, :, h])]
        if ko == 0:
            when(live, lambda: start(reg, sem, 1))
            return
        fst = [(hbm.at[b, :, h, pl.ds(w0, RUN - ko)], buf.at[g & 1, :, h, pl.ds(ko, RUN - ko)])]
        if t < 2:
            fst = [(hbm.at[b, t, :, pl.ds(SK - ko, ko)], buf.at[g & 1, t, :, pl.ds(0, ko)])] + fst
        if isinstance(sl, int):
            when(live, lambda: start(reg if sl else fst, sem, 1))
        else:
            pl.when(sl > 0)(lambda: start(reg, sem, 1))
            first = sl == 0
            pl.when(first if live is True else jnp.logical_and(first, live))(
                lambda: start(fst, sem, 1))

    def b_pos(nseg, t):
        return divmod((c_order if nseg == 4 else w_order)[t], 32 // nseg)

    def b_run(hbm, nseg, src, sl, t):
        seg, k = b_pos(nseg, t)
        ln = 512 // nseg
        r = boff + RT * k
        n = min(RT, ln - r)
        out = [(hbm.at[pl.ds(src(seg) + r, n)], bring.at[sl, pl.ds(ln * seg + r, n)])]
        if k == 0 and boff:
            out.append((hbm.at[pl.ds(src(seg), boff)], bring.at[sl, pl.ds(ln * seg, boff)]))
        return out

    def a_run(hbm, buf, r, lo, hi):
        r0, r1 = max(r - aoff, lo), (hi if r + RT == hi else r + RT - aoff)
        return [(hbm.at[pl.ds(r0, r1 - r0)], buf.at[pl.ds(r0, r1 - r0)])]

    def retile(sl, hb):
        def f():
            w = bring[sl].reshape(128, 4, 8, DH)[:, hb]
            w2_s[hb & 1][...] = w.reshape(128, 8 * DH)
        return f

    def wq_mm(cb, hb):
        def f(hook=None):
            r = jnp.dot(xb_s[cb].astype(BF16), w2_s[hb & 1][...], preferred_element_type=F32)
            qb_s[:, 1024 * hb:1024 * hb + 1024] += r
            call(hook, r[:, 7 * DH:])
        return f

    def wuk_mm(cb, hb):
        def f(hook=None):
            for j in range(8):
                h = 8 * hb + j
                q = (qb_s[:, DH * h:DH * h + DH] * scale).astype(BF16)
                r = lax.dot_general(q, w2_s[hb & 1][:, DH * j:DH * j + DH], NT,
                                    preferred_element_type=F32)
                qabs_t[cb, 8 * h:8 * h + NB, :] = r
                if j == 0:
                    r0 = r
            call(hook, r0)
        return f

    def wuv_mm(cb, hb):
        def f(hook=None):
            for j in range(8):
                cc = cc_s[cb, pl.ds(8 * hb + j, NB, stride=NH), :].astype(BF16)
                r = jnp.dot(cc, w2_s[hb & 1][:, DH * j:DH * j + DH], preferred_element_type=F32)
                ctx_s[hb, :, DH * j:DH * j + DH] += r
            call(hook, r)
        return f

    def qabs_finish():
        for b in range(NB):
            for cb in range(4):
                qabs_s[b, :, 128 * cb:128 * cb + 128] = (
                    qabs_t[cb, pl.ds(b, NH, stride=8), :].astype(BF16))

    def c_pieces(sl):
        def cmat(b):
            return mat(bring[sl, 128 * b:128 * b + 128], 4, 0, 4)

        def qk(b):
            def f(hook=None):
                s = lax.dot_general(qabs_s[b], cmat(b), NT, preferred_element_type=F32)
                sb_s[b] = s
                call(hook, s[0:8, 0:DH])
            return f

        def sm(b):
            def f():
                s = sb_s[b]
                m_old = m_s[b]
                m_new = jnp.maximum(m_old, jnp.max(s, axis=-1, keepdims=True))
                alpha = jnp.exp(m_old - m_new)
                ps = [jnp.exp(s[:, 128 * j:128 * j + 128] - m_new) for j in range(CK // 128)]
                l_s[b] = alpha * l_s[b] + sum(ps[1:], ps[0])
                m_s[b] = m_new
                al_s[b] = alpha
                pb_s[b] = jnp.concatenate(ps, axis=-1).astype(BF16)
            return f

        def pv(b):
            def f(hook=None):
                r = jnp.dot(pb_s[b], cmat(b), preferred_element_type=F32)
                al = al_s[b]
                for j in range(4):
                    cols = slice(128 * j, 128 * j + 128)
                    acc_s[b, :, cols] = al * acc_s[b, :, cols] + r[:, cols]
                if hook is not None:
                    keep["v"] = r[0:8, 3 * DH:]
            return f

        keep = {}

        def late(f):
            def g(hook=None):
                f(hook)
                if hook is not None:
                    hook(keep["v"])
            return g

        return [qk(0), both(qk(1), sm(0)), both(qk(2), sm(1)), both(qk(3), sm(2)),
                late(both(sm(3), pv(0), pv(1), host=1)), late(both(pv(2), pv(3)))]

    def c_finish():
        for b in range(NB):
            cc = acc_s[b] / jnp.sum(l_s[b], axis=-1, keepdims=True)
            for cb in range(4):
                cc_s[cb, NH * b:NH * b + NH, :] = cc[:, 128 * cb:128 * cb + 128]

    def wob_mm(sl, cb, half):
        def f(hook=None):
            rs = []
            for i in range(2):
                c0 = 512 * half + 256 * i
                w = mat(bring[sl, c0 // 2:c0 // 2 + 128], 4, 0, 4)
                rs.append(jnp.dot(ctx_s[cb, :, c0:c0 + 256].astype(BF16), w,
                                  preferred_element_type=F32))
            out_s[1, 0:NB, :] += rs[0] + rs[1]
            call(hook, rs[0][:, 3 * DH:])
        return f

    def init():
        wait(x_copies[:1], semx.at[0])
        wait(x_copies[1:], semx.at[1])
        if not do_compute:
            return
        xb = xb_buf[...].astype(F32)
        for cb in range(4):
            xb_s[cb] = xb[:, 128 * cb:128 * cb + 128]
        qb_s[...] = jnp.zeros(qb_s.shape, F32)
        ctx_s[...] = jnp.zeros(ctx_s.shape, F32)
        out_s[...] = jnp.zeros(out_s.shape, F32)
        for r in (ma_s, la_s, acca_s):
            r[...] = jnp.zeros(r.shape, F32)
        m_s[...] = jnp.full(m_s.shape, -jnp.inf, F32)
        l_s[...] = jnp.zeros(l_s.shape, F32)
        acc_s[...] = jnp.zeros(acc_s.shape, F32)

    def wqa_mm(j):
        def f(hook=None):
            w = mat(wqa_buf[...], 32, 4 * j, 4)
            r = jnp.dot(xa_buf[...], w, preferred_element_type=F32) * scale
            for i in range(4):
                h = 4 * j + i
                qa_t[8 * h:8 * h + NB, :] = r[:, DH * i:DH * i + DH]
            call(hook, r[:, 0:DH])
        return f

    def a_qk(g, k):
        def f(hook=None):
            q8 = qa_t[pl.ds(64 * k + (g >> 3), 8, stride=8), :]
            s = None
            for j in range(8):
                qm = jnp.where(row8 == j, q8, 0.0).astype(BF16)
                sj = lax.dot_general(qm, kbuf[g & 1, k // 2, 8 * (k % 2) + j], NT,
                                     preferred_element_type=F32)
                s = sj if s is None else s + sj
                if j == 0:
                    call(hook, sj)
            sa_s[8 * k:8 * k + 8, :] = s
        return f

    def a_sm(g):
        def f():
            first = (g & 7) == 0
            s = sa_s[...]
            m_old = jnp.where(first, -jnp.inf, ma_s[...])
            m_new = jnp.maximum(m_old, jnp.max(s, axis=-1, keepdims=True))
            alpha = jnp.exp(m_old - m_new)
            p = jnp.exp(s - m_new)
            la_s[...] = jnp.where(first, p, alpha * la_s[...] + p)
            ma_s[...] = m_new
            aa_s[...] = alpha
            sa_s[...] = p
        return f

    def a_pv(g, k):
        def f(hook=None):
            first = (g & 7) == 0
            for r0 in (16 * k, 16 * k + 8):
                rows = slice(r0, r0 + 8)
                p = sa_s[rows, :].astype(BF16)
                o = None
                for j in range(8):
                    oj = jnp.dot(p, vbuf[g & 1, k, r0 % 16 + j], preferred_element_type=F32)
                    o = oj if o is None else jnp.where(row8 == j, oj, o)
                    if r0 % 16 == 0 and j == 4:
                        call(hook, oj)
                acca_s[rows, :] = jnp.where(first, o, aa_s[rows, :] * acca_s[rows, :] + o)
        return f

    def a_fin(g):
        def f():
            o = acca_s[...] / jnp.sum(la_s[...], axis=-1, keepdims=True)
            oa_t[pl.ds(g >> 3, NH, stride=8), :] = o
        return f

    def woa_dot(h):
        o = oa_t[8 * h:8 * h + NB, :].astype(BF16)
        return jnp.dot(o, mat(woa_buf[64 * h:64 * h + 64], 4, 0, 4), preferred_element_type=F32)

    quads = [(hs, k) for k in (3, 2, 1, 0) for hs in ((0, 4, 8, 12), (16, 20, 24, 28))]

    def quad_lhs():
        for n, (hs, k) in enumerate(quads):
            oq_s[n, 0:NB, :] = jnp.concatenate(
                [oa_t[8 * h:8 * h + NB, 32 * k:32 * k + 32] for h in hs], axis=1)

    def quad_dot(n):
        hs, k = quads[n]
        w = jnp.concatenate([woa_buf[64 * h + RT * k:64 * h + RT * k + RT] for h in hs], axis=0)
        return jnp.dot(oq_s[n, 0:NB, :].astype(BF16), mat(w, 4, 0, 4), preferred_element_type=F32)

    def woa_mm(dot, items):
        def f():
            r = dot(items[0])
            for i in items[1:]:
                r = r + dot(i)
            out_s[0, 0:NB, :] += r
        return f

    def static_ticks(waits, starts1, starts0, comp):
        for t, (descs, sem) in enumerate(waits):
            wait(descs, sem)
            for d, s in starts0.get(t, ()):
                start(d, s, 0)
            for d, s in starts1.get(t, ()):
                start(d, s, 1)
            for f in comp.get(t, ()):
                f()

    pre0 = CFG["pre0"]
    x_copies = [(xa_hbm, xa_buf), (xb_hbm, xb_buf)]
    qr = [a_run(wqa_hbm, wqa_buf, RT * ((x + CFG["qoff"]) % 128), 0, 2048)
          for x in _xor_order(CFG["qbasis"])]
    q1 = [qr[i] + qr[i + 1] for i in range(0, 128, 2) if i % 6 != 4]
    q0 = [qr[i] for i in range(128) if i % 6 >= 4]
    for j in range(D1):
        start(q1[j], sem1.at[1], 1)
        if j < pre0:
            start(q0[j], sem0.at[1], 0)
    start(x_copies[:1], semx.at[0], 0)
    start(x_copies[1:], semx.at[1], 0)
    s1, s0, cm = {}, {}, {}
    for t, d in enumerate(q1[D1:]):
        at(s1, t, (d, sem1.at[1]))
    for t in range(D1):
        at(cm, len(q1) - D1 + t, lambda t=t: kv_start(k_hbm, kbuf, 0, t, sem1.at[0]))
    n0 = len(q0) - pre0
    for j in range(n0):
        at(s0, (j * len(q1)) // n0, (q0[pre0 + j], sem0.at[1]))
    at(cm, 4, init)
    static_ticks([(d, sem1.at[1]) for d in q1], s1, s0, cm)

    oruns = [a_run(woa_hbm, woa_buf, 256 * r + RT * k, 256 * r, 256 * r + 256)
             for k in range(15, -1, -1) for r in range(8)]
    o1, o0, o_end = [], [], []
    for i, pat in enumerate(CFG["opat"]):
        lo = [oruns.pop(0) for _ in pat]
        ones = [r for r, c in zip(lo, pat) if c == "1"]
        o0.append([(len(o1) + pat[:n].count("1") // 2, r)
                   for n, (r, c) in enumerate(zip(lo, pat)) if c == "0"])
        o1 += [(ones[n] + ones[n + 1], semt.at[0, i]) for n in range(0, len(ones), 2)]
        o_end.append(len(o1) - 1)
    assert not oruns

    b_slots = CFG["b_slots"]
    a_slots = CFG["a_slots"]

    def body(g, g_lo, g_hi):
        def between(lo, hi):
            if lo <= g_lo and g_hi <= hi:
                return True
            if hi < g_lo or g_hi < lo:
                return False
            if lo <= g_lo:
                return g <= hi
            if g_hi <= hi:
                return g >= lo
            return jnp.logical_and(g >= lo, g <= hi)

        def either(x, y):
            if x is True or y is True:
                return True
            if x is False or y is False:
                return y if x is False else x
            return jnp.logical_or(x, y)

        par = g & 1
        iw = g & 3
        w_stage = [(between(0, 3), wqb_hbm), (between(4, 7), wuk_hbm),
                   (between(24, 27), wuv_hbm), (between(28, 31), wob_hbm)]
        is_c = between(8, 23)
        ic = (g - 8) & 15
        last = between(NG - 1, NG - 1)
        gn = g + 1 if last is False else (g + 1) & (NG - 1)

        sl, cb = 1 - par, (g + 3) & 3
        cm = {}
        short = [qabs_finish, c_finish]
        if do_compute:
            w3 = either(between(1, 8), between(25, 28))
            for k, hb in ((0, 0), (1, 1), (4, 2), (5, 3)):
                short.append(retile(sl, hb))
                at(cm, b_slots[k], (w3, short[-1]))
            for k, hb in ((2, 0), (6, 2)):
                at(cm, b_slots[k], (between(1, 4), both(wq_mm(cb, hb), wq_mm(cb, hb + 1))))
                at(cm, b_slots[k], (between(25, 28), both(wuv_mm(cb, hb), wuv_mm(cb, hb + 1))))
            for k, hb in ((2, 0), (3, 1), (6, 2), (7, 3)):
                at(cm, b_slots[k], (between(5, 8), wuk_mm(cb, hb)))
            at(cm, b_slots[8], (between(8, 8), qabs_finish))
            for k, f in zip(CFG["c_slots"], c_pieces(sl)):
                at(cm, b_slots[k], (between(9, 24), f))
            at(cm, b_slots[8], (between(24, 24), c_finish))
            for k, half in ((3, 0), (7, 1)):
                at(cm, b_slots[k], (between(29, 31), wob_mm(sl, cb, half)))
            for k, t in enumerate(CFG["q_slots"]):
                at(cm, t, (between(0, 0), wqa_mm(k)))
            for k in range(2):
                at(cm, a_slots[k], (between(1, 31), a_pv(g - 1, k)))
            fin = either(either(between(8, 8), between(16, 16)), between(24, 24))
            short += [a_fin(g - 1), a_sm(g)]
            at(cm, a_slots[1] + 2, (fin, short[-2]))
            for k in range(4):
                at(cm, a_slots[2 + k], (True, a_qk(g, k)))
            at(cm, a_slots[6], (True, short[-1]))

        def also(x, y):
            if x is False or y is False:
                return False
            if x is True or y is True:
                return y if x is True else x
            return jnp.logical_and(x, y)

        def b_start(j, live=True):
            for cond, hbm in w_stage:
                when(also(cond, live), lambda hbm=hbm: start(
                    b_run(hbm, 1, lambda s: 512 * iw, par, j), sem0.at[par], 0))
            when(also(is_c, live), lambda: start(
                b_run(c_hbm, 4, lambda s: 2048 * s + 128 * ic, par, j), sem0.at[par], 0))

        def hook_for(j):
            assert is_c is True or is_c is False
            seg, k = b_pos(4 if is_c else 1, j)
            r = 128 * seg + RT * k + boff

            def hook(v):
                bring[par, r, 0:v.shape[0], :] = v.astype(BF16)
                b_start(j)
            return hook

        embed = CFG["embed"] and not isinstance(g, int)
        hosted = False
        for t in range(32):
            dst = (kbuf if t < 16 else vbuf).at[par, :, h_order[t % 16]]
            pltpu.make_async_copy(dst, dst, sem1.at[t // 16]).wait()
            if hosted is not True:
                b_start(t, True if hosted is False else jnp.logical_not(hosted))
            if t < 16:
                kv_start(v_hbm, vbuf, g, t, sem1.at[1])
            else:
                if last is not True:
                    kv_start(k_hbm, kbuf, gn, t - 16, sem1.at[0], live=between(0, NG - 2))
                when(last, lambda: start(o1[t - 16][0], o1[t - 16][1], 1))
            if t == bwait:
                when(between(0, 0), lambda: wait(sum(q0, []), sem0.at[1]))
                when(between(1, 31), lambda: wait([(None, bring.at[sl])], sem0.at[sl]))
            hosted = False
            for cond, f in cm.get(t, ()):
                if embed and t < 31 and cond is not False and f not in short:
                    hosted = either(hosted, cond)
                    pl.when(g >= 0 if cond is True else cond)(
                        lambda f=f: f(hook_for(t + 1)))
                else:
                    when(cond, f)

    cuts = CFG["cuts"]
    for lo, hi in zip(cuts[:-1], cuts[1:]):
        if hi - lo == 1:
            body(lo, lo, lo)
        else:
            def loop_body(g, carry, lo=lo, hi=hi):
                body(g, lo, hi - 1)
                return carry
            lax.fori_loop(lo, hi, loop_body, 0)

    s1, s0, cm = {}, {}, {}
    nt = len(o1)
    for t in range(nt - D1):
        at(s1, t, o1[D1 + t])
    la, lb = CFG["olead"]
    for i, grp in enumerate(o0):
        for p, r in grp:
            at(s0, max(0, p - (la + ((lb - la) * p) // nt)), (r, semt.at[1, i]))
        at(cm, o_end[i], lambda i=i, grp=grp: wait(sum((r for _, r in grp), []), semt.at[1, i]))
    at(cm, 7, lambda: wait([(None, bring.at[1])], sem0.at[1]))

    def write_b():
        o_ref[:, DM:2 * DM] = out_s[1, 0:NB, :].astype(o_ref.dtype)

    if do_compute:
        at(cm, 1, a_pv(NG - 1, 0))
        at(cm, 3, a_pv(NG - 1, 1))
        at(cm, 5, a_fin(NG - 1))
        at(cm, 7, wob_mm(1, 3, 0))
        at(cm, 15, both(wob_mm(1, 3, 1), write_b))
        at(cm, 17, quad_lhs)
        for i in range(3):
            at(cm, o_end[i], woa_mm(woa_dot, tuple(range(3 - i, 16, 4))))
            at(cm, o_end[i] + 2, woa_mm(woa_dot, tuple(range(19 - i, 32, 4))))
        n = 0
        for i, pat in list(enumerate(CFG["opat"]))[3:-1]:
            at(cm, o_end[i], woa_mm(quad_dot, tuple(range(n, n + len(pat) // 4))))
            n += len(pat) // 4
    static_ticks(o1, s1, s0, cm)
    if do_compute:
        r = out_s[0, 0:NB, :]
        for i in range(n, 8):
            r = r + quad_dot(i)
        o_ref[:, 0:DM] = r.astype(o_ref.dtype)
    else:
        o_ref[...] = jnp.zeros(o_ref.shape, o_ref.dtype)


def _tiles(x):
    c = x.shape[-1]
    return x.reshape(-1, 8, c // DH, DH).transpose(0, 2, 1, 3).reshape(-1, 8, DH)


def _compiler_params():
    kw = dict(vmem_limit_bytes=48 * 1024 * 1024, disable_bounds_checks=not CFG["checks"])
    try:
        return pltpu.CompilerParams(disable_semaphore_checks=not CFG["checks"], **kw)
    except TypeError:
        return pltpu.CompilerParams(**kw)


@jax.jit
def pallas_concat_heads__sliding_block_cached__compressed_kv_cla__decode_kernel(
    A_x: jax.Array,
    A_k_cache: jax.Array,
    A_v_cache: jax.Array,
    A_wq: jax.Array,
    A_wo: jax.Array,
    B_x: jax.Array,
    B_c_kv: jax.Array,
    B_w_q: jax.Array,
    B_w_uk: jax.Array,
    B_w_uv: jax.Array,
    B_w_o: jax.Array,
):
    assert A_x.shape == (NB, 1, DM) and B_x.shape == (NB, 1, DM)
    assert A_k_cache.shape == (NB, NH, SK, DH) and B_c_kv.shape == (NB, SK, DM)
    vm = pltpu.VMEM
    out = pl.pallas_call(
        _kernel,
        out_shape=jax.ShapeDtypeStruct((NB, 2 * DM), A_x.dtype),
        in_specs=[pl.BlockSpec(memory_space=pl.ANY)] * 11,
        out_specs=pl.BlockSpec(memory_space=pltpu.VMEM),
        scratch_shapes=[
            vm((NB, DM), BF16), vm((NB, DM), BF16),
            vm((2, 2, 16, RUN, DH), BF16), vm((2, 2, 16, RUN, DH), BF16),
            vm((2048, 8, DH), BF16), vm((2048, 8, DH), BF16),
            vm((2, 512, 8, DH), BF16),
            vm((4, NB, 128), F32),
            vm((NH * 8 + 8, DH), F32),
            vm((NH * 8 + 8, DH), F32),
            vm((NH, RUN), F32),
            vm((NH, DH), F32), vm((NH, DH), F32),
            vm((NH, DH), F32), vm((NH, DH), F32),
            vm((NB, NH * DH), F32),
            vm((4, NH * 8 + 8, 128), F32),
            vm((NB, NH, DM), BF16),
            vm((NB, NH, CK), F32),
            vm((NB, NH, CK), BF16),
            vm((NB, NH, 128), F32),
            vm((NB, NH, 128), F32), vm((NB, NH, 128), F32),
            vm((NB, NH, DM), F32),
            vm((4, NB * NH + NH, 128), F32),
            vm((4, NB, 8 * DH), F32),
            vm((2, 8, DM), F32),
            vm((8, 8, DH), F32),
            vm((128, 8 * DH), BF16), vm((128, 8 * DH), BF16),
            pltpu.SemaphoreType.DMA((2,)), pltpu.SemaphoreType.DMA((2,)),
            pltpu.SemaphoreType.DMA((2,)), pltpu.SemaphoreType.DMA((2, len(CFG["opat"]))),
        ],
        compiler_params=_compiler_params(),
        name="concat_heads_decode",
    )(
        A_x.reshape(NB, DM), B_x.reshape(NB, DM),
        A_k_cache.reshape(NB, 2, 16, SK, DH), A_v_cache.reshape(NB, 2, 16, SK, DH),
        _tiles(A_wq), _tiles(A_wo), _tiles(B_c_kv),
        _tiles(B_w_q), _tiles(B_w_uk), _tiles(B_w_uv), _tiles(B_w_o),
    )
    return out.reshape(NB, 1, 2 * DM)
```
